```python
import jax
import jax.numpy as jnp

def _softmax(x, axis=-1):
    return jax.nn.softmax(x, axis=axis)

def _gelu(x):
    return jax.nn.gelu(x, approximate=True)

def _silu(x):
    return jax.nn.silu(x)

def _sigmoid(x):
    return jax.nn.sigmoid(x)

def _layernorm(x, axis=-1, eps=1e-05):
    m = jnp.mean(x, axis=axis, keepdims=True)
    v = jnp.var(x, axis=axis, keepdims=True)
    return (x - m) / jnp.sqrt(v + eps)

def _scatter_add(tgt, idx, src, axis=0):
    return tgt.at[idx].add(src)

def _segment_sum(src, seg, n):
    return jax.ops.segment_sum(src, seg, n)

class _Rng:

    def __init__(self, key):
        self._k = key

    def _next(self):
        self._k, sub = jax.random.split(self._k)
        return sub

    def normal(self, shape):
        return jax.random.normal(self._next(), shape, dtype=jnp.bfloat16)

    def randint(self, lo, hi, shape):
        return jax.random.randint(self._next(), shape, lo, hi, dtype=jnp.int32)

    def uniform(self, shape, lo=0.0, hi=1.0):
        return jax.random.uniform(self._next(), shape, jnp.bfloat16, lo, hi)

    def permutation(self, n):
        return jax.random.permutation(self._next(), n)
kernel_name = 'gated_mix__memory_aug_recurrent_mem_tr__moe_arch_mod__prompt'

def setup_inputs():
    _rng = _Rng(jax.random.key(int.from_bytes(__import__("os").urandom(4), "little")))
    _w = lambda a: (lambda t: t.astype(jnp.bfloat16) if jnp.issubdtype(t.dtype, jnp.floating) else t)(jnp.asarray(a))

    def _A_setup():
        B, S, Dm = (1, 2048, 1024)
        H, Dh = (32, 128)
        M, seg = (8, 32)
        seg = min(seg, S)
        S = S // seg * seg
        return {'x': _w((lambda *s: _rng.normal(s) * 0.05)(B, S, Dm)), 'mem0': _w((lambda *s: _rng.normal(s) * 0.05)(B, M, Dm)), 'Wq': _w((lambda *s: _rng.normal(s) * 0.05)(Dm, H, Dh) * Dm ** (-0.5)), 'Wk': _w((lambda *s: _rng.normal(s) * 0.05)(Dm, H, Dh) * Dm ** (-0.5)), 'Wv': _w((lambda *s: _rng.normal(s) * 0.05)(Dm, H, Dh) * Dm ** (-0.5)), 'Wo': _w((lambda *s: _rng.normal(s) * 0.05)(H, Dh, Dm) * (H * Dh) ** (-0.5)), 'seg_len': seg}
    _A_in = _A_setup()

    def _B_setup():
        B, S, D, F, C = (1, 2048, 1024, 3584, 8)
        return {'x': _w((lambda *s: _rng.normal(s) * 0.05)(B, S, D)), 'w_r': _w((lambda *s: _rng.normal(s) * 0.05)(D)), 'w_gate': _w((lambda *s: _rng.normal(s) * 0.05)(D, F)), 'w_up': _w((lambda *s: _rng.normal(s) * 0.05)(D, F)), 'w_down': _w((lambda *s: _rng.normal(s) * 0.05)(F, D))}
    _B_in = _B_setup()
    return {'A_x': _A_in['x'], 'A_mem0': _A_in['mem0'], 'A_Wq': _A_in['Wq'], 'A_Wk': _A_in['Wk'], 'A_Wv': _A_in['Wv'], 'A_Wo': _A_in['Wo'], 'A_seg_len': _A_in['seg_len'], 'B_x': _B_in['x'], 'B_w_r': _B_in['w_r'], 'B_w_gate': _B_in['w_gate'], 'B_w_up': _B_in['w_up'], 'B_w_down': _B_in['w_down'], 'gate_w': _w((lambda *s: _rng.normal(s) * 0.05)(1024))}

def reference(A_x, A_mem0, A_Wq, A_Wk, A_Wv, A_Wo, A_seg_len, B_x, B_w_r, B_w_gate, B_w_up, B_w_down, gate_w):

    def _A_ref(x, mem0, Wq, Wk, Wv, Wo, seg_len):
        B, S, Dm = x.shape
        H, Dh = (Wq.shape[1], Wq.shape[2])
        M = mem0.shape[1]
        scale = Dh ** (-0.5)
        n_seg = S // seg_len
        L = M + seg_len
        idx = jnp.arange(L)
        mask = (idx[:, None] < M) | (idx[:, None] >= idx[None, :])
        mem = mem0
        outs = []
        for s in range(n_seg):
            xs = x[:, s * seg_len:(s + 1) * seg_len, :].copy()
            h = jnp.concatenate([mem, xs], axis=1)
            q = jnp.einsum('btd,dhe->bhte', h, Wq)
            k = jnp.einsum('btd,dhe->bhte', h, Wk)
            v = jnp.einsum('btd,dhe->bhte', h, Wv)
            scores = jnp.einsum('bhqe,bhke->bhqk', q, k) * scale
            scores = jnp.where(mask[None, None], scores, -1000000000.0)
            p = _softmax(scores, axis=-1)
            o = jnp.einsum('bhqk,bhke->bhqe', p, v)
            o = jnp.einsum('bhte,hed->btd', o, Wo)
            mem = o[:, :M, :].copy()
            outs.append(o[:, M:, :])
        return jnp.concatenate(outs, axis=1)

    def _B_ref(x, w_r, w_gate, w_up, w_down):
        B, S, D = x.shape
        C = 8
        r = x @ w_r
        idx = jnp.argsort(-r, axis=-1)[:, :C]
        idx_e = jnp.repeat(idx.reshape(B, C, 1), D, axis=2)
        x_sel = jnp.take_along_axis(x, idx_e, axis=1)
        g = _silu(x_sel @ w_gate)
        u = x_sel @ w_up
        y = g * u @ w_down
        r_sel = _sigmoid(jnp.take_along_axis(r, idx, axis=1))
        y = y * r_sel.reshape(B, C, 1)
        b_off = (jnp.arange(B) * S).reshape(B, 1)
        flat_idx = (idx + b_off).reshape(B * C)
        zero = (x * 0.0).reshape(B * S, D)
        upd = _scatter_add(zero, flat_idx, y.reshape(B * C, D), axis=0)
        return x + upd.reshape(B, S, D)
    x = A_x
    g = _sigmoid((x * gate_w).sum(-1, keepdims=True))
    a = _A_ref(x, A_mem0, A_Wq, A_Wk, A_Wv, A_Wo, A_seg_len)
    b = _B_ref(x, B_w_r, B_w_gate, B_w_up, B_w_down)
    return g * a + (1 - g) * b
```

```python
import functools

import jax
import jax.numpy as jnp
import numpy as np
from jax import lax
from jax.experimental import pallas as pl
from jax.experimental.pallas import tpu as pltpu

BF16, F32, U32, I32 = jnp.bfloat16, jnp.float32, jnp.uint32, jnp.int32
LANES = 128
TOP_C = 8
W_AHEAD = 2
OUT_SEGS = 8
INT_MIN = -(2 ** 31)


def _dot(a, b):
    return jnp.dot(a, b, preferred_element_type=F32)


def _as_bf16(words):
    return pltpu.bitcast(words, BF16)


def _sigmoid(v):
    return 1.0 / (1.0 + jnp.exp(-v))


def _score_fill(n_mem, seg):
    shape = (2 * (n_mem + seg), LANES)

    def decode(i):
        tail = i >= 2 * seg
        head = jnp.where(tail, (i - 2 * seg) >> 3, i >> 5)
        r = i & (seg - 1)
        pos = jnp.where(tail, n_mem + (i & 7), jnp.where(r < n_mem, r, r + n_mem))
        return head, pos

    rh, rp = decode(lax.broadcasted_iota(I32, shape, 0))
    ch, cp = decode(lax.broadcasted_iota(I32, shape, 1))
    visible = (rp < n_mem) | (rp >= cp)
    return jnp.where(rh == ch, jnp.where(visible, 0.0, -1e9), -jnp.inf).astype(F32)


def _kernel(x_hbm, mem0_ref, wq_hbm, wk_hbm, wv_hbm, wo_hbm, wr_ref, wg_hbm, wu_hbm,
            wd_hbm, gw_ref, out_hbm,
            x_v, wqkv, wo_v, qkv0, o0, a_v, g_v, mem, fill_v, key_v, wg_v, wu_v, wd_v,
            out_v, idx_s, sem_w, sem_x, sem_wo, sem_f, sem_out):
    n_seg, seg, dm = x_v.shape
    n_mem = mem.shape[0]
    n_pair = wqkv.shape[1]
    n_head = 2 * n_pair
    nk = dm // LANES
    nf = wg_v.shape[0]
    scale = LANES ** -0.5
    w_hbm = (wq_hbm, wk_hbm, wv_hbm)

    def w_copy(m, p):
        return pltpu.make_async_copy(
            w_hbm[m].bitcast(U32).at[:, p, :], wqkv.at[m, p], sem_w.at[m, p])

    def col_copy(src, dst, n, sem):
        cols = pl.ds(pl.multiple_of(n * LANES, LANES), LANES)
        return pltpu.make_async_copy(src.bitcast(U32).at[:, cols], dst.at[n], sem)

    def wait_whole(dst, sem):
        pltpu.make_async_copy(dst, dst, sem).wait()

    x_head = pltpu.make_async_copy(
        x_hbm.at[:, pl.ds(0, n_mem), :], x_v.at[:, pl.ds(0, n_mem), :], sem_x.at[0])
    x_tail = pltpu.make_async_copy(
        x_hbm.at[:, pl.ds(n_mem, seg - n_mem), :], x_v.at[:, pl.ds(n_mem, seg - n_mem), :],
        sem_x.at[1])

    x_head.start()
    for p in range(W_AHEAD):
        for m in range(3):
            w_copy(m, p).start()

    fill_v[...] = _score_fill(n_mem, seg)
    key_v[...] = jnp.full(key_v.shape, INT_MIN, I32)
    mem[...] = mem0_ref[...].astype(F32)

    def head_weights(m, p):
        w = wqkv[m, p].reshape(dm // 16, 2, 8, LANES)
        return [_as_bf16(w[:, j].reshape(dm // 2, LANES)) for j in range(2)]

    x_head.wait()

    def prologue(p, carry):
        @pl.when(p + W_AHEAD < n_pair)
        def _():
            for m in range(3):
                w_copy(m, p + W_AHEAD).start()

        @pl.when(p < nk)
        def _():
            col_copy(wo_hbm, wo_v, p, sem_wo.at[0]).start()

        @pl.when(p == nk)
        def _():
            x_tail.start()

        for m in range(3):
            wait_whole(wqkv.at[m, p], sem_w.at[m, p])
        x0 = x_v[:, 0:n_mem, :].reshape(n_seg * n_mem, dm)
        for m in range(3):
            even = wqkv[m, p, pl.ds(0, dm // 2, stride=2), :]
            odd = wqkv[m, p, pl.ds(1, dm // 2, stride=2), :]
            wa = (even & np.uint32(0xFFFF)) | (odd << 16)
            wb = (even >> 16) | (odd & np.uint32(0xFFFF0000))
            wqkv[m, p] = jnp.concatenate(
                [wa.reshape(dm // 16, 8, LANES), wb.reshape(dm // 16, 8, LANES)],
                axis=1).reshape(dm, LANES)
            ra = _dot(x0, _as_bf16(wa)).reshape(n_seg, n_mem, LANES)
            rb = _dot(x0, _as_bf16(wb)).reshape(n_seg, n_mem, LANES)
            r = jnp.concatenate([ra, rb], axis=1).reshape(n_seg * 2 * n_mem, LANES)
            qkv0[m, p] = pltpu.bitcast(r.astype(BF16), U32)
        return carry

    lax.fori_loop(0, n_pair, prologue, 0)

    x_tail.wait()
    wait_whole(wo_v, sem_wo.at[0])

    def row_dot(rows, w):
        acc = rows[:, 0:LANES] * w[0:1, :]
        for n in range(1, nk):
            acc = acc + rows[:, n * LANES:(n + 1) * LANES] * w[n:n + 1, :]
        return jnp.sum(acc, axis=-1, keepdims=True)

    def step(s, carry):
        @pl.when(s < nf)
        def _():
            col_copy(wg_hbm, wg_v, s, sem_f.at[0]).start()
            col_copy(wu_hbm, wu_v, s, sem_f.at[1]).start()

        @pl.when(s < nk)
        def _():
            col_copy(wd_hbm, wd_v, s, sem_f.at[2]).start()

        xs = x_v[s]
        xf = xs.astype(F32)
        h = jnp.concatenate([mem[...], xf[n_mem:2 * n_mem]], axis=0).astype(BF16)
        h = jnp.concatenate([h, xs[2 * n_mem:]], axis=0)
        rows0 = pl.ds(pl.multiple_of(s * n_mem, n_mem), n_mem)
        pad = jnp.zeros((LANES - 2 * (seg + n_mem), LANES), BF16)

        def project(m, p):
            wa, wb = head_weights(m, p)
            return jnp.concatenate(
                [_dot(h, wa).astype(BF16), _dot(h, wb).astype(BF16),
                 _as_bf16(qkv0[m, p, rows0, :])], axis=0)

        def probabilities(q, k):
            sc = lax.dot_general(q, jnp.concatenate([k, pad], axis=0),
                                 (((1,), (1,)), ((), ())), preferred_element_type=F32)
            fill = fill_v[...]
            sc = jnp.where(fill == 0.0, sc * scale, fill)
            e = jnp.exp(sc - jnp.max(sc, axis=-1, keepdims=True))
            den = jnp.sum(e, axis=-1, keepdims=True)
            inv = pl.reciprocal(den, approx=True)
            inv = inv * (2.0 - den * inv)
            return (e * inv).astype(BF16)

        def attend(prob, v, p):
            o = _dot(prob, jnp.concatenate([v, pad], axis=0))
            o0[2 * p, rows0, :] = o[2 * seg:2 * seg + n_mem]
            o0[2 * p + 1, rows0, :] = o[2 * seg + n_mem:]
            ob = o[0:2 * seg].astype(BF16)
            return ob[0:seg], ob[seg:]

        def out_proj(heads, lo, hi, n):
            lhs = jnp.concatenate([heads[i] for i in range(lo, hi)], axis=1)
            return _dot(lhs, _as_bf16(wo_v[n, lo * (LANES // 2):hi * (LANES // 2), :]))

        q, k, v, prob, heads, part = {}, {}, {}, {}, {}, []
        half = n_head // 2
        for p in range(n_pair + 2):
            if p < n_pair:
                k[p] = project(1, p)
                q[p] = project(0, p)
            if 0 <= p - 1 < n_pair:
                prob[p - 1] = probabilities(q[p - 1], k[p - 1])
            if p < n_pair:
                v[p] = project(2, p)
            else:
                first = (p - n_pair) * (nk // 2)
                part += [out_proj(heads, 0, half, n) for n in range(first, first + nk // 2)]
            if 0 <= p - 2 < n_pair:
                heads[2 * p - 4], heads[2 * p - 3] = attend(prob[p - 2], v[p - 2], p - 2)
        for n in range(nk):
            r = out_proj(heads, half, n_head, n) + part[n]
            mem[:, n * LANES:(n + 1) * LANES] = r[0:n_mem]
            a_v[s, n_mem:, n * LANES:(n + 1) * LANES] = r[n_mem:]

        gate = _sigmoid(row_dot(xf, gw_ref[...].astype(F32)))
        g_v[s] = jnp.broadcast_to(gate, (seg, LANES))
        score = row_dot(xf, wr_ref[...].astype(F32)).astype(BF16).astype(F32)
        score = jnp.broadcast_to(score, (seg, LANES))
        bits = pltpu.bitcast(jnp.where(score == 0.0, 0.0, score), I32)
        order = jnp.where(bits < 0, bits ^ np.int32(0x7FFFFFFF), bits)
        order = jnp.where(score != score, INT_MIN, order)
        token = s * seg + lax.broadcasted_iota(I32, (seg, LANES), 0)
        key = (order & np.int32(-65536)) | (65535 - token)
        lane = lax.broadcasted_iota(I32, (seg, LANES), 1)
        key_v[...] = jnp.where(lane == s, key, key_v[...])
        return carry

    lax.fori_loop(0, n_seg, step, 0)

    def first_tokens_out(c):
        rows = pl.ds(pl.multiple_of(c * (OUT_SEGS * n_mem), OUT_SEGS * n_mem), OUT_SEGS * n_mem)
        lhs = jnp.concatenate([o0[i, rows, :].astype(BF16) for i in range(n_head)], axis=1)
        for n in range(nk):
            r = _dot(lhs, _as_bf16(wo_v[n])).reshape(OUT_SEGS, n_mem, LANES)
            a_v[pl.ds(c * OUT_SEGS, OUT_SEGS), 0:n_mem, n * LANES:(n + 1) * LANES] = r

    def mix(c):
        segs = pl.ds(c * OUT_SEGS, OUT_SEGS)
        gate = g_v[segs]
        for n in range(nk):
            cols = slice(n * LANES, (n + 1) * LANES)
            b = x_v[segs, :, cols].astype(F32)
            out_v[segs, :, cols] = (gate * a_v[segs, :, cols] + (1.0 - gate) * b).astype(BF16)

    def out_copy(c):
        segs = pl.ds(c * OUT_SEGS, OUT_SEGS)
        return pltpu.make_async_copy(out_v.at[segs], out_hbm.at[segs], sem_out.at[0])

    for i, w in enumerate((wg_v, wu_v, wd_v)):
        wait_whole(w, sem_f.at[i])

    first_tokens_out(0)
    keys = key_v[...]
    for i in range(TOP_C):
        best = jnp.max(keys)
        idx_s[i] = 65535 - (best & 65535)
        keys = jnp.where(keys == best, INT_MIN, keys)

    row = lax.broadcasted_iota(I32, (seg, dm), 0)
    slot = lax.broadcasted_iota(I32, (2 * TOP_C, dm), 0)
    x_sel = jnp.zeros((2 * TOP_C, dm), F32)
    for i in range(TOP_C):
        t = idx_s[i]
        picked = jnp.where(row == (t & (seg - 1)), x_v[t // seg].astype(F32), 0.0)
        x_sel = jnp.where(slot == i, jnp.sum(picked, axis=0, keepdims=True), x_sel)
    r_sel = _sigmoid(row_dot(x_sel, wr_ref[...].astype(F32)))
    lhs = x_sel.astype(BF16)
    hidden = []
    for n in range(nf):
        gt = _dot(lhs, _as_bf16(wg_v[n]))
        up = _dot(lhs, _as_bf16(wu_v[n]))
        hidden.append((gt * _sigmoid(gt) * up).astype(BF16))
    hidden = jnp.concatenate(hidden, axis=1)
    y = jnp.concatenate([_dot(hidden, _as_bf16(wd_v[n])) for n in range(nk)], axis=1) * r_sel
    for i in range(TOP_C):
        t = idx_s[i]
        upd = jnp.where(row == (t & (seg - 1)), y[i:i + 1, :], 0.0)
        x_v[t // seg] = (x_v[t // seg].astype(F32) + upd).astype(BF16)

    n_chunk = n_seg // OUT_SEGS

    def epilogue(c, carry):
        mix(c)
        first_tokens_out(c + 1)
        out_copy(c).start()
        return carry

    lax.fori_loop(0, n_chunk - 1, epilogue, 0)
    mix(n_chunk - 1)
    out_copy(n_chunk - 1).start()
    pltpu.make_async_copy(out_v, out_hbm, sem_out.at[0]).wait()


@functools.partial(jax.jit, static_argnames=("A_seg_len",))
def pallas_gated_mix__memory_aug_recurrent_mem_tr__moe_arch_mod__prompt_kernel(
    A_x, A_mem0, A_Wq, A_Wk, A_Wv, A_Wo, A_seg_len, B_x, B_w_r, B_w_gate, B_w_up,
    B_w_down, gate_w,
):
    del B_x
    batch, n_tok, dm = A_x.shape
    n_mem = A_mem0.shape[1]
    n_head, dh = A_Wq.shape[1:]
    d_ff = B_w_gate.shape[1]
    seg = int(A_seg_len)
    n_seg = n_tok // seg
    assert (batch, n_mem, seg, dh) == (1, 8, 32, LANES)
    assert n_head % 4 == 0 and dm % 256 == 0 and d_ff % LANES == 0
    assert n_tok % (seg * OUT_SEGS) == 0 and n_seg <= LANES
    n_pair, nk, nf = n_head // 2, dm // LANES, d_ff // LANES
    assert nk < n_pair and max(nk, nf) <= n_seg

    hbm = pl.BlockSpec(memory_space=pl.ANY)
    vmem = pl.BlockSpec(memory_space=pltpu.VMEM)
    out = pl.pallas_call(
        _kernel,
        out_shape=jax.ShapeDtypeStruct((n_seg, seg, dm), A_x.dtype),
        in_specs=[hbm, vmem, hbm, hbm, hbm, hbm, vmem, hbm, hbm, hbm, vmem],
        out_specs=hbm,
        scratch_shapes=[
            pltpu.VMEM((n_seg, seg, dm), BF16),
            pltpu.VMEM((3, n_pair, dm, LANES), U32),
            pltpu.VMEM((nk, n_head * dh // 2, LANES), U32),
            pltpu.VMEM((3, n_pair, n_seg * n_mem, LANES), U32),
            pltpu.VMEM((n_head, n_seg * n_mem, LANES), F32),
            pltpu.VMEM((n_seg, seg, dm), F32),
            pltpu.VMEM((n_seg, seg, LANES), F32),
            pltpu.VMEM((n_mem, dm), F32),
            pltpu.VMEM((2 * (n_mem + seg), LANES), F32),
            pltpu.VMEM((seg, LANES), I32),
            pltpu.VMEM((nf, dm // 2, LANES), U32),
            pltpu.VMEM((nf, dm // 2, LANES), U32),
            pltpu.VMEM((nk, d_ff // 2, LANES), U32),
            pltpu.VMEM((n_seg, seg, dm), BF16),
            pltpu.SMEM((TOP_C,), I32),
            pltpu.SemaphoreType.DMA((3, n_pair)),
            pltpu.SemaphoreType.DMA((2,)),
            pltpu.SemaphoreType.DMA((1,)),
            pltpu.SemaphoreType.DMA((3,)),
            pltpu.SemaphoreType.DMA((1,)),
        ],
        compiler_params=pltpu.CompilerParams(vmem_limit_bytes=112 * 1024 * 1024),
        name="gated_mix_rmt_mod",
    )(
        A_x.reshape(n_seg, seg, dm), A_mem0.reshape(n_mem, dm), A_Wq, A_Wk, A_Wv,
        A_Wo.reshape(n_head * dh, dm), B_w_r.reshape(nk, LANES), B_w_gate, B_w_up, B_w_down,
        gate_w.reshape(nk, LANES),
    )
    return out.reshape(batch, n_tok, dm)
```

```python
import functools

import jax
import jax.numpy as jnp
import numpy as np
from jax import lax
from jax.experimental import pallas as pl
from jax.experimental.pallas import tpu as pltpu

BF16, F32, U32, I32 = jnp.bfloat16, jnp.float32, jnp.uint32, jnp.int32
LANES = 128
TOP_C = 8
INT_MIN = -(2 ** 31)
HI16 = np.uint32(0xFFFF0000)

PRO_PAIRS = 2
RAMP = (0, 1, 3)
STEP_UNROLL = 2
QK_LAG, PV_LAG = 3, 4
ROUTE_SLOTS = 8
EARLY_HALVES = 6


def _dot(a, b):
    return jnp.dot(a, b, preferred_element_type=F32)


def _as_bf16(words):
    return pltpu.bitcast(words, BF16)


def _to_words(v):
    return pltpu.bitcast(v.astype(BF16), U32)


def _split_words(words):
    return pltpu.bitcast(words << 16, F32), pltpu.bitcast(words & HI16, F32)


def _join_words(lo, hi):
    return pltpu.pack_elementwise([lo, hi], packed_dtype=BF16)


def _sigmoid(v):
    return 1.0 / (1.0 + jnp.exp(-v))


def _mix(gate, a, b):
    return (gate * a + (1.0 - gate) * b).astype(BF16)


def _lhs_terms(a, b, c, d):
    return [c + d, a, a + b, d, a + d, c - a, b - d]


def _rhs_terms(e, f, g, h):
    return [e, f - h, h, g - e, e + h, e + f, g + h]


def _combine(m):
    return [m[3] - m[2] + m[4] + m[6], m[1] + m[2], m[0] + m[3], m[1] - m[0] + m[4] + m[5]]


def _score_fill(n_mem, seg):
    shape = (2 * (n_mem + seg), LANES)

    def decode(i):
        tail = i >= 2 * seg
        head = jnp.where(tail, (i - 2 * seg) >> 3, i >> 5)
        r = i & (seg - 1)
        pos = jnp.where(tail, n_mem + (i & 7), jnp.where(r < n_mem, r, r + n_mem))
        return head, pos

    rh, rp = decode(lax.broadcasted_iota(I32, shape, 0))
    ch, cp = decode(lax.broadcasted_iota(I32, shape, 1))
    visible = (rp < n_mem) | (rp >= cp)
    return jnp.where(rh == ch, jnp.where(visible, 0.0, -1e9), -jnp.inf).astype(F32)


def _kernel(x_hbm, mem0_ref, wq_hbm, wk_hbm, wv_hbm, wo_hbm, wr_ref, wg_hbm, wu_hbm,
            wd_hbm, gw_ref, out_hbm,
            x_v, x_terms, wqkv, wo_v, qkv0, o_terms, a_v, g_v, mem, fill_v, key_v,
            wg_v, wu_v, wd_v, out_v, idx_s, sem_w, sem_x, sem_wo, sem_f, sem_out):
    n_seg, seg, dm = x_v.shape
    n_mem = mem.shape[0]
    n_pair = wqkv.shape[1]
    n_head = 2 * n_pair
    nk = dm // LANES
    nf = wg_v.shape[0]
    scale = LANES ** -0.5
    w_hbm = (wq_hbm, wk_hbm, wv_hbm)
    first, rest = pl.ds(0, n_mem), pl.ds(n_mem, seg - n_mem)

    def lanes(n):
        return slice(n * LANES, (n + 1) * LANES)

    def w_copy(m, p):
        return pltpu.make_async_copy(
            w_hbm[m].bitcast(U32).at[:, p, :], wqkv.at[m, p], sem_w.at[m, p])

    def col_copy(src, dst, n, sem):
        start = n * LANES if isinstance(n, int) else pl.multiple_of(n * LANES, LANES)
        cols = pl.ds(start, LANES)
        return pltpu.make_async_copy(src.bitcast(U32).at[:, cols], dst.at[n], sem)

    def wait_whole(dst, sem):
        pltpu.make_async_copy(dst, dst, sem).wait()

    x_first = pltpu.make_async_copy(x_hbm.at[:, first, :], x_v.at[:, first, :], sem_x.at[0])
    x_rest = pltpu.make_async_copy(x_hbm.at[:, rest, :], x_v.at[:, rest, :], sem_x.at[1])

    units = [(m, j) for j in range(PRO_PAIRS) for m in range(3)]
    x_first.start()
    w_copy(*units[0]).start()

    fill_v[...] = _score_fill(n_mem, seg)
    key_v[...] = jnp.full(key_v.shape, INT_MIN, I32)
    mem[...] = mem0_ref[...].astype(F32)

    half_rows = n_seg * n_mem // 2
    x_first.wait()
    for n in range(nk // 2):
        lo, hi = (x_v[:, 0:n_mem, lanes(n + i * nk // 2)].astype(F32).reshape(2, half_rows, LANES)
                  for i in range(2))
        for i, t in enumerate(_lhs_terms(lo[0], hi[0], lo[1], hi[1])):
            x_terms[i, n] = _to_words(t)

    def project_first(m, p):
        even = wqkv[m, p, pl.ds(0, dm // 2, stride=2), :]
        odd = wqkv[m, p, pl.ds(1, dm // 2, stride=2), :]
        wa = (even & np.uint32(0xFFFF)) | (odd << 16)
        wb = (even >> 16) | (odd & HI16)
        wqkv[m, p] = jnp.concatenate(
            [wa.reshape(dm // 16, 8, LANES), wb.reshape(dm // 16, 8, LANES)],
            axis=1).reshape(dm, LANES)
        halves = []
        for words in (even, odd):
            (e, f), (g, h) = _split_words(words[:dm // 4]), _split_words(words[dm // 4:])
            halves.append(_rhs_terms(e, f, g, h))
        terms = [_join_words(lo, hi) for lo, hi in zip(*halves)]
        terms[0], terms[2] = wa[:dm // 4], wb[dm // 4:]
        prods = []
        for i in range(7):
            lhs = jnp.concatenate([_as_bf16(x_terms[i, n]) for n in range(nk // 2)], axis=1)
            prods.append(_dot(lhs, _as_bf16(terms[i])))
        c = [t.reshape(n_seg // 2, n_mem, LANES) for t in _combine(prods)]
        for i in range(2):
            both = jnp.concatenate(c[2 * i:2 * i + 2], axis=1).reshape(2 * half_rows, LANES)
            qkv0[m, p, i * half_rows:(i + 1) * half_rows, :] = _to_words(both)

    def project_block(block, p0):
        for m, j in block:
            wait_whole(wqkv.at[m, p0 + j], sem_w.at[m, p0 + j])
        for m, j in block:
            project_first(m, p0 + j)

    n_pro = n_pair // PRO_PAIRS
    wo_per_it = nk // n_pro

    ramp = [units[a:b] for a, b in zip(RAMP, RAMP[1:] + (len(units),))]
    for i, block in enumerate(ramp):
        if i + 1 < len(ramp):
            for m, j in ramp[i + 1]:
                w_copy(m, j).start()
        else:
            for m, j in units:
                w_copy(m, PRO_PAIRS + j).start()
        project_block(block, 0)
    for n in range(wo_per_it):
        col_copy(wo_hbm, wo_v, n, sem_wo.at[0]).start()

    def prologue(it, carry):
        p0 = it * PRO_PAIRS

        @pl.when(it + 1 < n_pro)
        def _():
            for m, j in units:
                w_copy(m, p0 + PRO_PAIRS + j).start()

        for n in range(wo_per_it):
            col_copy(wo_hbm, wo_v, it * wo_per_it + n, sem_wo.at[0]).start()

        @pl.when(it == n_pro // 2)
        def _():
            x_rest.start()

        project_block(units, p0)
        return carry

    lax.fori_loop(1, n_pro, prologue, 0)

    x_rest.wait()
    wait_whole(wo_v, sem_wo.at[0])

    def row_dot(rows, w):
        acc = rows[:, lanes(0)] * w[0:1, :]
        for n in range(1, nk):
            acc = acc + rows[:, lanes(n)] * w[n:n + 1, :]
        return jnp.sum(acc, axis=-1, keepdims=True)

    def head_weights(m, hd, lo, hi):
        w = wqkv[m, hd // 2, lo * LANES:hi * LANES, :].reshape(-1, 2, 8, LANES)
        return _as_bf16(w[:, hd % 2].reshape(-1, LANES))

    def segment(s, mem_cols, mem_is_late):
        xs = x_v[s]
        xf = xs.astype(F32)
        h_cols = [
            jnp.concatenate(
                [jnp.concatenate([mem_cols[n], xf[n_mem:2 * n_mem, lanes(n)]], axis=0).astype(BF16),
                 xs[2 * n_mem:, lanes(n)]], axis=0)
            for n in range(nk)]
        rows0 = pl.ds(pl.multiple_of(s * n_mem, n_mem), n_mem)
        pad = jnp.zeros((LANES - 2 * (seg + n_mem), LANES), BF16)

        def partial_proj(m, hd, lo, hi):
            return _dot(jnp.concatenate(h_cols[lo:hi], axis=1), head_weights(m, hd, lo, hi))

        early = {}
        if mem_is_late:
            order = [(m, 2 * p + j) for p in range(n_pair) for m in (1, 0, 2) for j in range(2)]
            for m, hd in order[:EARLY_HALVES]:
                early[m, hd] = partial_proj(m, hd, 0, nk // 2)

        def project(m, p):
            out = []
            for hd in (2 * p, 2 * p + 1):
                if (m, hd) in early:
                    r = partial_proj(m, hd, nk // 2, nk) + early[m, hd]
                else:
                    r = partial_proj(m, hd, 0, nk)
                out.append(r.astype(BF16))
            return jnp.concatenate(out + [_as_bf16(qkv0[m, p, rows0, :])], axis=0)

        def probabilities(q, k):
            sc = lax.dot_general(q, jnp.concatenate([k, pad], axis=0),
                                 (((1,), (1,)), ((), ())), preferred_element_type=F32)
            fill = fill_v[...]
            sc = jnp.where(fill == 0.0, sc * scale, fill)
            e = jnp.exp(sc - jnp.max(sc, axis=-1, keepdims=True))
            den = jnp.sum(e, axis=-1, keepdims=True)
            inv = pl.reciprocal(den, approx=True)
            inv = inv * (2.0 - den * inv)
            return (e * inv).astype(BF16)

        def out_proj(lo, hi, n):
            lhs = jnp.concatenate([heads[i] for i in range(lo, hi)], axis=1)
            return _dot(lhs, _as_bf16(wo_v[n, lo * (LANES // 2):hi * (LANES // 2), :]))

        slots = [(m, p) for p in range(n_pair) for m in (1, 0, 2)] + [(3, n) for n in range(nk)]
        res, prob, heads, o_first = {}, {}, {}, {}
        for i, (m, j) in enumerate(slots):
            res[m, j] = project(m, j) if m < 3 else out_proj(0, n_pair, j)
            for p in range(n_pair):
                if i == 3 * p + 1 + QK_LAG:
                    prob[p] = probabilities(res[0, p], res[1, p])
                if i == min(3 * p + 1 + QK_LAG + PV_LAG, len(slots) - 1):
                    o = _dot(prob[p], jnp.concatenate([res[2, p], pad], axis=0))
                    ob = o[0:2 * seg].astype(BF16)
                    heads[2 * p], heads[2 * p + 1] = ob[0:seg], ob[seg:]
                    o_first[2 * p] = o[2 * seg:2 * seg + n_mem]
                    o_first[2 * p + 1] = o[2 * seg + n_mem:]
        gate = jnp.broadcast_to(_sigmoid(row_dot(xf, gw_ref[...].astype(F32))), (seg, LANES))
        g_v[s] = gate
        new_mem = []
        for n in range(nk):
            r = out_proj(n_pair, n_head, n) + res[3, n]
            new_mem.append(r[0:n_mem])
            a_v[s, :, lanes(n)] = r[n_mem:]
            out_v[s, rest, lanes(n)] = _mix(gate[n_mem:], r[n_mem:], xf[n_mem:, lanes(n)])

        score = row_dot(xf, wr_ref[...].astype(F32)).astype(BF16).astype(F32)
        score = jnp.broadcast_to(score, (seg, LANES))
        bits = pltpu.bitcast(jnp.where(score == 0.0, 0.0, score), I32)
        order = jnp.where(bits < 0, bits ^ np.int32(0x7FFFFFFF), bits)
        order = jnp.where(score != score, INT_MIN, order)
        token = s * seg + lax.broadcasted_iota(I32, (seg, LANES), 0)
        key = (order & np.int32(-65536)) | (65535 - token)
        lane = lax.broadcasted_iota(I32, (seg, LANES), 1)
        key_v[...] = jnp.where(lane == s, key, key_v[...])
        return new_mem, o_first

    n_step = n_seg // STEP_UNROLL

    def step(it, carry):
        for dst, src, sem in ((wg_v, wg_hbm, 0), (wu_v, wu_hbm, 1), (wd_v, wd_hbm, 2)):
            per_step = pl.cdiv(dst.shape[0], n_step)
            for i in range(per_step):
                @pl.when(it * per_step + i < dst.shape[0])
                def _():
                    col_copy(src, dst, it * per_step + i, sem_f.at[sem]).start()

        mem_cols = [mem[:, lanes(n)] for n in range(nk)]
        for u0 in range(0, STEP_UNROLL, 2):
            o = []
            for u in (u0, u0 + 1):
                mem_cols, o_first = segment(it * STEP_UNROLL + u, mem_cols, u > 0)
                o.append(o_first)
            rows = pl.ds(pl.multiple_of((it * STEP_UNROLL + u0) * 2, 4), 4)
            for hd in range(n_pair):
                a, b, c, d = (o[i][j] for i in range(2) for j in (hd, hd + n_pair))
                for i, t in enumerate(_lhs_terms(a, b, c, d)):
                    o_terms[i, hd, rows, :] = _to_words(jnp.concatenate([t, t], axis=0))[0:4]
        for n in range(nk):
            mem[:, lanes(n)] = mem_cols[n]
        return carry

    lax.fori_loop(0, n_step, step, 0)

    def out_copy(rows, cols):
        return pltpu.make_async_copy(
            out_v.at[:, rows, cols], out_hbm.at[:, rows, cols], sem_out.at[0])

    def routed_ffn():
        keys = key_v[...]
        for i in range(TOP_C):
            best = jnp.max(keys)
            idx_s[i] = 65535 - (best & 65535)
            keys = jnp.where(keys == best, INT_MIN, keys)
        row = lax.broadcasted_iota(I32, (seg, dm), 0)
        slot = lax.broadcasted_iota(I32, (2 * TOP_C, dm), 0)
        x_sel = jnp.zeros((2 * TOP_C, dm), F32)
        for i in range(TOP_C):
            t = idx_s[i]
            picked = jnp.where(row == (t & (seg - 1)), x_v[t // seg].astype(F32), 0.0)
            x_sel = jnp.where(slot == i, jnp.sum(picked, axis=0, keepdims=True), x_sel)
        r_sel = _sigmoid(row_dot(x_sel, wr_ref[...].astype(F32)))
        lhs = x_sel.astype(BF16)
        for _ in range(ROUTE_SLOTS):
            yield
        hidden = []
        for n in range(nf):
            gt = _dot(lhs, _as_bf16(wg_v[n]))
            yield
            up = _dot(lhs, _as_bf16(wu_v[n]))
            hidden.append((gt * _sigmoid(gt) * up).astype(BF16))
            yield
        y = [None] * nk
        for lo, hi in ((0, nf // 2), (nf // 2, nf)):
            lhs = jnp.concatenate(hidden[lo:hi], axis=1)
            for n in range(nk):
                part = _dot(lhs, _as_bf16(wd_v[n, lo * (LANES // 2):hi * (LANES // 2), :]))
                y[n] = part if y[n] is None else part + y[n]
                yield
        y = jnp.concatenate(y, axis=1) * r_sel
        for i in range(TOP_C):
            t = idx_s[i]
            s = t // seg
            upd = jnp.where(row == (t & (seg - 1)), y[i:i + 1, :], 0.0)
            b = (x_v[s].astype(F32) + upd).astype(BF16)
            x_v[s] = b
            gate = g_v[s, rest, :]
            for n in range(nk):
                out_v[s, rest, lanes(n)] = _mix(
                    gate, a_v[s, :, lanes(n)], b.astype(F32)[n_mem:, lanes(n)])

    def out_first(u, filler):
        k_half = wo_v.shape[1] // 2
        blocks = [wo_v[2 * u + j, i * k_half:(i + 1) * k_half, :]
                  for i in range(2) for j in range(2)]
        e, f, g, h = (_split_words(w) for w in blocks)
        terms = [_join_words(lo, hi) for lo, hi in
                 zip(*(_rhs_terms(e[i], f[i], g[i], h[i]) for i in range(2)))]
        terms[0], terms[2] = blocks[0], blocks[3]
        prods = []
        for i in range(7):
            acc = None
            for lo in range(0, n_pair, 4):
                lhs = jnp.concatenate(
                    [_as_bf16(o_terms[i, hd]) for hd in range(lo, lo + 4)], axis=1)
                part = _dot(lhs, _as_bf16(terms[i][lo * (LANES // 2):(lo + 4) * (LANES // 2)]))
                acc = part if acc is None else part + acc
                next(filler, None)
            prods.append(acc)
        c = [t.reshape(n_seg // 2, 1, n_mem, LANES) for t in _combine(prods)]
        return [jnp.concatenate([c[j], c[j + 2]], axis=1).reshape(n_seg, n_mem, LANES)
                for j in range(2)]

    def mix_first(a, n):
        out_v[:, first, lanes(n)] = _mix(
            g_v[:, first, :], a, x_v[:, first, lanes(n)].astype(F32))

    for i, w in enumerate((wg_v, wu_v, wd_v)):
        wait_whole(w, sem_f.at[i])

    ffn = routed_ffn()
    a_first = []
    for u in range(nk // 2 - 1):
        a_first += out_first(u, ffn)
    for _ in ffn:
        pass
    out_copy(rest, pl.ds(0, dm)).start()
    a_first += out_first(nk // 2 - 1, ffn)
    for n in range(nk - 2):
        mix_first(a_first[n], n)
    out_copy(first, pl.ds(0, dm - 2 * LANES)).start()
    for n in range(nk - 2, nk):
        mix_first(a_first[n], n)
    out_copy(first, pl.ds(dm - 2 * LANES, 2 * LANES)).start()
    pltpu.make_async_copy(out_v, out_hbm, sem_out.at[0]).wait()


@functools.partial(jax.jit, static_argnames=("A_seg_len",))
def pallas_gated_mix__memory_aug_recurrent_mem_tr__moe_arch_mod__prompt_kernel(
    A_x, A_mem0, A_Wq, A_Wk, A_Wv, A_Wo, A_seg_len, B_x, B_w_r, B_w_gate, B_w_up,
    B_w_down, gate_w,
):
    del B_x
    batch, n_tok, dm = A_x.shape
    n_mem = A_mem0.shape[1]
    n_head, dh = A_Wq.shape[1:]
    d_ff = B_w_gate.shape[1]
    seg = int(A_seg_len)
    n_seg = n_tok // seg
    n_pair, nk, nf = n_head // 2, dm // LANES, d_ff // LANES
    assert (batch, n_mem, seg, dh) == (1, 8, 32, LANES)
    assert dm % (4 * LANES) == 0 and d_ff % LANES == 0 and n_pair % PRO_PAIRS == 0
    assert n_tok % (seg * STEP_UNROLL) == 0 and n_seg <= LANES
    assert nk % (n_pair // PRO_PAIRS) == 0

    hbm = pl.BlockSpec(memory_space=pl.ANY)
    vmem = pl.BlockSpec(memory_space=pltpu.VMEM)
    out = pl.pallas_call(
        _kernel,
        out_shape=jax.ShapeDtypeStruct((n_seg, seg, dm), A_x.dtype),
        in_specs=[hbm, vmem, hbm, hbm, hbm, hbm, vmem, hbm, hbm, hbm, vmem],
        out_specs=hbm,
        scratch_shapes=[
            pltpu.VMEM((n_seg, seg, dm), BF16),
            pltpu.VMEM((7, nk // 2, n_seg * n_mem // 4, LANES), U32),
            pltpu.VMEM((3, n_pair, dm, LANES), U32),
            pltpu.VMEM((nk, n_head * dh // 2, LANES), U32),
            pltpu.VMEM((3, n_pair, n_seg * n_mem, LANES), U32),
            pltpu.VMEM((7, n_pair, n_seg * n_mem // 4, LANES), U32),
            pltpu.VMEM((n_seg, seg - n_mem, dm), F32),
            pltpu.VMEM((n_seg, seg, LANES), F32),
            pltpu.VMEM((n_mem, dm), F32),
            pltpu.VMEM((2 * (n_mem + seg), LANES), F32),
            pltpu.VMEM((seg, LANES), I32),
            pltpu.VMEM((nf, dm // 2, LANES), U32),
            pltpu.VMEM((nf, dm // 2, LANES), U32),
            pltpu.VMEM((nk, d_ff // 2, LANES), U32),
            pltpu.VMEM((n_seg, seg, dm), BF16),
            pltpu.SMEM((TOP_C,), I32),
            pltpu.SemaphoreType.DMA((3, n_pair)),
            pltpu.SemaphoreType.DMA((2,)),
            pltpu.SemaphoreType.DMA((1,)),
            pltpu.SemaphoreType.DMA((3,)),
            pltpu.SemaphoreType.DMA((1,)),
        ],
        compiler_params=pltpu.CompilerParams(vmem_limit_bytes=116 * 1024 * 1024),
        name="gated_mix_rmt_mod",
    )(
        A_x.reshape(n_seg, seg, dm), A_mem0.reshape(n_mem, dm), A_Wq, A_Wk, A_Wv,
        A_Wo.reshape(n_head * dh, dm), B_w_r.reshape(nk, LANES), B_w_gate, B_w_up, B_w_down,
        gate_w.reshape(nk, LANES),
    )
    return out.reshape(batch, n_tok, dm)
```

```python
import functools

import jax
import jax.numpy as jnp
import numpy as np
from jax import lax
from jax.experimental import pallas as pl
from jax.experimental.pallas import tpu as pltpu

BF16, F32, U32, I32 = jnp.bfloat16, jnp.float32, jnp.uint32, jnp.int32
LANES = 128
TOP_C = 8
N_FIXED_SEMS = 11
INT_MIN = -(2 ** 31)
HI16 = np.uint32(0xFFFF0000)

PRO_PAIRS = 2
STEP_UNROLL = 2
QK_LAG, PV_LAG = 3, 4
FIRST_LAG = 0
ROUTE_SLOTS = 8
EARLY_HALVES = 6


def _dot(a, b):
    return jnp.dot(a, b, preferred_element_type=F32)


def _as_bf16(words):
    return pltpu.bitcast(words, BF16)


def _to_words(v):
    return pltpu.bitcast(v.astype(BF16), U32)


def _split_words(words):
    return pltpu.bitcast(words << 16, F32), pltpu.bitcast(words & HI16, F32)


def _join_words(lo, hi):
    return pltpu.pack_elementwise([lo, hi], packed_dtype=BF16)


def _sigmoid(v):
    return 1.0 / (1.0 + jnp.exp(-v))


def _mix(gate, a, b):
    return (gate * a + (1.0 - gate) * b).astype(BF16)


def _lhs_terms(a, b, c, d):
    return [c + d, a, a + b, d, a + d, c - a, b - d]


RHS_TERMS = (((0, 0),), ((0, 1), jnp.subtract, (1, 1)), ((1, 1),), ((1, 0), jnp.subtract, (0, 0)),
             ((0, 0), jnp.add, (1, 1)), ((0, 0), jnp.add, (0, 1)), ((1, 0), jnp.add, (1, 1)))


def _rhs_term(i, block):
    term = RHS_TERMS[i]
    rows = block(i, *term[0])
    if len(term) > 1:
        rows = [term[1](u, v) for u, v in zip(rows, block(i, *term[2]))]
    return _as_bf16(_join_words(*rows))


def _opaque_zero(count, i):
    return count >> (16 + i)


def _combine(m):
    return [m[3] - m[2] + m[4] + m[6], m[1] + m[2], m[0] + m[3], m[1] - m[0] + m[4] + m[5]]


def _score_fill(n_mem, seg):
    shape = (2 * (n_mem + seg), LANES)

    def decode(i):
        tail = i >= 2 * seg
        head = jnp.where(tail, (i - 2 * seg) >> 3, i >> 5)
        r = i & (seg - 1)
        pos = jnp.where(tail, n_mem + (i & 7), jnp.where(r < n_mem, r, r + n_mem))
        return head, pos

    rh, rp = decode(lax.broadcasted_iota(I32, shape, 0))
    ch, cp = decode(lax.broadcasted_iota(I32, shape, 1))
    visible = (rp < n_mem) | (rp >= cp)
    return jnp.where(rh == ch, jnp.where(visible, 0.0, -1e9), -jnp.inf).astype(F32)


def _kernel(x_hbm, mem0_hbm, wq_hbm, wk_hbm, wv_hbm, wo_hbm, wr_hbm, wg_hbm, wu_hbm,
            wd_hbm, gw_hbm, out_hbm,
            x_v, x_terms, wqkv, wo_v, qkv0, o_terms, a_v, g_v, mem, fill_v, key_v,
            mem0_ref, wr_ref, gw_ref, wg_v, wu_v, wd_v, out_v, idx_s,
            sems):
    n_seg, seg, dm = x_v.shape
    n_mem = mem.shape[0]
    n_pair = wqkv.shape[0] // 3
    n_head = 2 * n_pair
    nk = dm // LANES
    nf = wg_v.shape[0]
    scale = LANES ** -0.5
    w_hbm = (wq_hbm, wk_hbm, wv_hbm)
    first, rest = pl.ds(0, n_mem), pl.ds(n_mem, seg - n_mem)

    def lanes(n):
        return slice(n * LANES, (n + 1) * LANES)

    fixed = [sems.at[i] for i in range(N_FIXED_SEMS)]
    sem_x, sem_small, sem_ffn, sem_wo, sem_out = (
        fixed[0:2], fixed[2:5], fixed[5:8], fixed[8], fixed[9:11])

    def w_copy(m, p):
        return pltpu.make_async_copy(
            w_hbm[m].bitcast(U32).at[:, p, :], wqkv.at[3 * p + m],
            sems.at[N_FIXED_SEMS + 3 * p + m])

    def col_copy(src, dst, n, sem):
        start = n * LANES if isinstance(n, int) else pl.multiple_of(n * LANES, LANES)
        cols = pl.ds(start, LANES)
        return pltpu.make_async_copy(src.bitcast(U32).at[:, cols], dst.at[n], sem)

    def wait_whole(dst, sem):
        pltpu.make_async_copy(dst, dst, sem).wait()

    x_first = pltpu.make_async_copy(x_hbm.at[:, first, :], x_v.at[:, first, :], sem_x[0])
    x_rest = pltpu.make_async_copy(x_hbm.at[:, rest, :], x_v.at[:, rest, :], sem_x[1])

    units = [(m, j) for j in range(PRO_PAIRS) for m in range(3)]
    small = [pltpu.make_async_copy(src, dst, sem_small[i]) for i, (src, dst) in
             enumerate(((mem0_hbm, mem0_ref), (wr_hbm, wr_ref), (gw_hbm, gw_ref)))]
    x_first.start()
    for p0 in (0, PRO_PAIRS):
        for m, j in units:
            w_copy(m, p0 + j).start()
    for copy in small:
        copy.start()

    fill_v[...] = _score_fill(n_mem, seg)
    key_v[...] = jnp.full(key_v.shape, INT_MIN, I32)

    half_rows = n_seg * n_mem // 2
    x_first.wait()
    for n in range(nk // 2):
        lo, hi = (x_v[:, 0:n_mem, lanes(n + i * nk // 2)].astype(F32).reshape(2, half_rows, LANES)
                  for i in range(2))
        for i, t in enumerate(_lhs_terms(lo[0], hi[0], lo[1], hi[1])):
            x_terms[i, n] = _to_words(t)

    def regroup(w, piece, n_piece):
        groups = dm // 16
        for r in range(groups * piece // n_piece * 16, groups * (piece + 1) // n_piece * 16, 16):
            even = wqkv[w, pl.ds(r, 8, stride=2), :]
            odd = wqkv[w, pl.ds(r + 1, 8, stride=2), :]
            wqkv[w, r:r + 8, :] = (even & np.uint32(0xFFFF)) | (odd << 16)
            wqkv[w, r + 8:r + 16, :] = (even >> 16) | (odd & HI16)

    def project_first(w, regroup_previous):
        def block(i, row, col):
            at = w + _opaque_zero(w, i)
            return [_split_words(wqkv[at, pl.ds(row * (dm // 2) + r, dm // 4, stride=2), :])[col]
                    for r in range(2)]

        prods = []
        for i in range(7):
            lhs = jnp.concatenate([_as_bf16(x_terms[i, n]) for n in range(nk // 2)], axis=1)
            prods.append(_dot(lhs, _rhs_term(i, block)))
            if regroup_previous:
                regroup(w - 1, i, 7)
        c = [t.reshape(n_seg // 2, n_mem, LANES) for t in _combine(prods)]
        for i in range(2):
            both = jnp.concatenate(c[2 * i:2 * i + 2], axis=1).reshape(2 * half_rows, LANES)
            qkv0[w, i * half_rows:(i + 1) * half_rows, :] = _to_words(both)

    def wait_weights(w):
        wait_whole(wqkv.at[w], sems.at[N_FIXED_SEMS + w])

    n_pro = n_pair // PRO_PAIRS
    wo_per_it = nk // n_pro

    def ramp(w, carry):
        @pl.when(w > 0)
        def _():
            regroup(w - 1, 0, 1)

        wait_weights(w)
        project_first(w, False)
        return carry

    lax.fori_loop(0, len(units), ramp, 0)
    for n in range(wo_per_it):
        col_copy(wo_hbm, wo_v, n, sem_wo).start()

    def prologue(it, carry):
        p0 = it * PRO_PAIRS

        @pl.when(it + 1 < n_pro)
        def _():
            for m, j in units:
                w_copy(m, p0 + PRO_PAIRS + j).start()

        for n in range(wo_per_it):
            col_copy(wo_hbm, wo_v, it * wo_per_it + n, sem_wo).start()

        @pl.when(it == n_pro // 2)
        def _():
            x_rest.start()

        for u in range(len(units)):
            wait_weights(3 * p0 + u)
        for u in range(len(units)):
            project_first(3 * p0 + u, True)
        return carry

    lax.fori_loop(1, n_pro, prologue, 0)

    regroup(3 * n_pair - 1, 0, 1)
    x_rest.wait()
    for copy in small:
        copy.wait()
    mem[...] = mem0_ref[...].astype(F32)
    wait_whole(wo_v, sem_wo)

    def row_dot(rows, w):
        acc = rows[:, lanes(0)] * w[0:1, :]
        for n in range(1, nk):
            acc = acc + rows[:, lanes(n)] * w[n:n + 1, :]
        return jnp.sum(acc, axis=-1, keepdims=True)

    def head_weights(m, hd, lo, hi):
        w = wqkv[3 * (hd // 2) + m, lo * LANES:hi * LANES, :].reshape(-1, 2, 8, LANES)
        return _as_bf16(w[:, hd % 2].reshape(-1, LANES))

    def segment(s, mem_cols, mem_is_late):
        xs = x_v[s]
        xf = xs.astype(F32)
        h_cols = [
            jnp.concatenate(
                [jnp.concatenate([mem_cols[n], xf[n_mem:2 * n_mem, lanes(n)]], axis=0).astype(BF16),
                 xs[2 * n_mem:, lanes(n)]], axis=0)
            for n in range(nk)]
        rows0 = pl.ds(pl.multiple_of(s * n_mem, n_mem), n_mem)
        pad = jnp.zeros((LANES - 2 * (seg + n_mem), LANES), BF16)

        def partial_proj(m, hd, lo, hi):
            return _dot(jnp.concatenate(h_cols[lo:hi], axis=1), head_weights(m, hd, lo, hi))

        early = {}
        if mem_is_late:
            order = [(m, 2 * p + j) for p in range(n_pair) for m in (1, 0, 2) for j in range(2)]
            for m, hd in order[:EARLY_HALVES]:
                early[m, hd] = partial_proj(m, hd, 0, nk // 2)

        def project(m, p):
            out = []
            for hd in (2 * p, 2 * p + 1):
                if (m, hd) in early:
                    r = partial_proj(m, hd, nk // 2, nk) + early[m, hd]
                else:
                    r = partial_proj(m, hd, 0, nk)
                out.append(r.astype(BF16))
            return jnp.concatenate(out + [_as_bf16(qkv0[3 * p + m, rows0, :])], axis=0)

        def probabilities(q, k):
            sc = lax.dot_general(q, jnp.concatenate([k, pad], axis=0),
                                 (((1,), (1,)), ((), ())), preferred_element_type=F32)
            fill = fill_v[...]
            sc = jnp.where(fill == 0.0, sc * scale, fill)
            e = jnp.exp(sc - jnp.max(sc, axis=-1, keepdims=True))
            den = jnp.sum(e, axis=-1, keepdims=True)
            inv = pl.reciprocal(den, approx=True)
            inv = inv * (2.0 - den * inv)
            return (e * inv).astype(BF16)

        def out_proj(lo, hi, n):
            lhs = jnp.concatenate([heads[i] for i in range(lo, hi)], axis=1)
            return _dot(lhs, _as_bf16(wo_v[n, lo * (LANES // 2):hi * (LANES // 2), :]))

        slots = [(m, p) for p in range(n_pair) for m in (1, 0, 2)] + [(3, n) for n in range(nk)]
        res, prob, heads, o_first = {}, {}, {}, {}
        for i, (m, j) in enumerate(slots):
            res[m, j] = project(m, j) if m < 3 else out_proj(0, n_pair, j)
            for p in range(n_pair):
                extra = 0 if mem_is_late else max(FIRST_LAG - p, 0)
                if i == 3 * p + 1 + QK_LAG:
                    prob[p] = probabilities(res[0, p], res[1, p])
                if i == min(3 * p + 1 + QK_LAG + PV_LAG + extra, len(slots) - 1):
                    o = _dot(prob[p], jnp.concatenate([res[2, p], pad], axis=0))
                    ob = o[0:2 * seg].astype(BF16)
                    heads[2 * p], heads[2 * p + 1] = ob[0:seg], ob[seg:]
                    o_first[2 * p] = o[2 * seg:2 * seg + n_mem]
                    o_first[2 * p + 1] = o[2 * seg + n_mem:]
        gate = jnp.broadcast_to(_sigmoid(row_dot(xf, gw_ref[...].astype(F32))), (seg, LANES))
        g_v[s] = gate
        new_mem = []
        for n in range(nk):
            r = out_proj(n_pair, n_head, n) + res[3, n]
            new_mem.append(r[0:n_mem])
            a_v[s, rest, lanes(n)] = r[n_mem:]
            out_v[s, rest, lanes(n)] = _mix(gate[n_mem:], r[n_mem:], xf[n_mem:, lanes(n)])

        score = row_dot(xf, wr_ref[...].astype(F32)).astype(BF16).astype(F32)
        score = jnp.broadcast_to(score, (seg, LANES))
        bits = pltpu.bitcast(jnp.where(score == 0.0, 0.0, score), I32)
        order = jnp.where(bits < 0, bits ^ np.int32(0x7FFFFFFF), bits)
        order = jnp.where(score != score, INT_MIN, order)
        token = s * seg + lax.broadcasted_iota(I32, (seg, LANES), 0)
        key = (order & np.int32(-65536)) | (65535 - token)
        lane = lax.broadcasted_iota(I32, (seg, LANES), 1)
        key_v[...] = jnp.where(lane == s, key, key_v[...])
        return new_mem, o_first

    n_step = n_seg // STEP_UNROLL

    def step(it, carry):
        for dst, src, sem in ((wg_v, wg_hbm, 0), (wu_v, wu_hbm, 1), (wd_v, wd_hbm, 2)):
            per_step = pl.cdiv(dst.shape[0], n_step)
            for i in range(per_step):
                @pl.when(it * per_step + i < dst.shape[0])
                def _():
                    col_copy(src, dst, it * per_step + i, sem_ffn[sem]).start()

        mem_cols = [mem[:, lanes(n)] for n in range(nk)]
        for u0 in range(0, STEP_UNROLL, 2):
            o = []
            for u in (u0, u0 + 1):
                mem_cols, o_first = segment(it * STEP_UNROLL + u, mem_cols, u > 0)
                o.append(o_first)
            rows = pl.ds(pl.multiple_of((it * STEP_UNROLL + u0) * 2, 4), 4)
            for hd in range(n_pair):
                a, b, c, d = (o[i][j] for i in range(2) for j in (hd, hd + n_pair))
                for i, t in enumerate(_lhs_terms(a, b, c, d)):
                    o_terms[i, hd, rows, :] = _to_words(jnp.concatenate([t, t], axis=0))[0:4]
        for n in range(nk):
            mem[:, lanes(n)] = mem_cols[n]
        return carry + 1

    steps = lax.fori_loop(0, n_step, step, 0)

    def out_copy(segs, rows, cols, sem):
        return pltpu.make_async_copy(
            out_v.at[segs, rows, cols], out_hbm.at[segs, rows, cols], sem)

    every_seg, every_col = pl.ds(0, n_seg), pl.ds(0, dm)
    rest_copy = out_copy(every_seg, rest, every_col, sem_out[0])
    first_copies = [out_copy(every_seg, first, pl.ds(0, dm - 2 * LANES), sem_out[1]),
                    out_copy(every_seg, first, pl.ds(dm - 2 * LANES, 2 * LANES), sem_out[1])]

    def for_routed_segments(fn):
        segs = [idx_s[i] // seg for i in range(TOP_C)]
        for i, s in enumerate(segs):
            new = functools.reduce(jnp.logical_and, [s != t for t in segs[:i]], True)
            pl.when(new)(lambda: fn(out_copy(pl.ds(s, 1), rest, every_col, sem_out[0])))

    row = lax.broadcasted_iota(I32, (n_mem, dm), 0)

    def routed_ffn():
        keys = key_v[...]
        for i in range(TOP_C):
            best = jnp.max(keys)
            idx_s[i] = 65535 - (best & 65535)
            keys = jnp.where(keys == best, INT_MIN, keys)
        slot = lax.broadcasted_iota(I32, (2 * TOP_C, dm), 0)
        x_sel = jnp.zeros((2 * TOP_C, dm), F32)
        for i in range(TOP_C):
            t = idx_s[i]
            rows = pl.ds(pl.multiple_of(t & (seg - n_mem), n_mem), n_mem)
            picked = jnp.where(row == (t & (n_mem - 1)), x_v[t // seg, rows, :].astype(F32), 0.0)
            x_sel = jnp.where(slot == i, jnp.sum(picked, axis=0, keepdims=True), x_sel)
        r_sel = _sigmoid(row_dot(x_sel, wr_ref[...].astype(F32)))
        lhs = x_sel.astype(BF16)
        for _ in range(ROUTE_SLOTS):
            yield
        hidden = []
        for n in range(nf):
            gt = _dot(lhs, _as_bf16(wg_v[n]))
            yield
            up = _dot(lhs, _as_bf16(wu_v[n]))
            hidden.append((gt * _sigmoid(gt) * up).astype(BF16))
            yield
        y = [None] * nk
        for lo in range(0, nf, nk):
            hi = min(lo + nk, nf)
            lhs = jnp.concatenate(hidden[lo:hi], axis=1)
            for n in range(nk):
                part = _dot(lhs, _as_bf16(wd_v[n, lo * (LANES // 2):hi * (LANES // 2), :]))
                y[n] = part if y[n] is None else part + y[n]
                if (n + 1) * (hi - lo) % nk < hi - lo:
                    yield
        y = jnp.concatenate(y, axis=1) * r_sel
        rest_copy.wait()
        for i in range(TOP_C):
            yield
            t = idx_s[i]
            s, r0 = t // seg, pl.multiple_of(t & (seg - n_mem), n_mem)
            rows = pl.ds(r0, n_mem)
            upd = jnp.where(row == (t & (n_mem - 1)), y[i:i + 1, :], 0.0)
            b = (x_v[s, rows, :].astype(F32) + upd).astype(BF16)
            x_v[s, rows, :] = b
            later = pl.ds(pl.multiple_of(jnp.maximum(r0, n_mem), n_mem), n_mem)
            gate, b = g_v[s, rows, :], b.astype(F32)
            for n in range(nk):
                a = a_v[s, rows if n < nk - 2 else later, lanes(n)]
                out_v[s, rows, lanes(n)] = _mix(gate, a, b[:, lanes(n)])
        yield
        first_copies[0].start()
        for_routed_segments(lambda copy: copy.start())

    def out_first(u, filler):
        prods = []
        for i in range(7):
            acc = None
            for lo in range(0, n_pair, 4):
                lhs = jnp.concatenate(
                    [_as_bf16(o_terms[i, hd]) for hd in range(lo, lo + 4)], axis=1)

                def block(i, row, col):
                    r0 = row * (wo_v.shape[1] // 2) + lo * (LANES // 2)
                    return wo_v[2 * u + col + _opaque_zero(steps, i), r0:r0 + 2 * LANES, :]

                if len(RHS_TERMS[i]) == 1:
                    rhs = _as_bf16(block(i, *RHS_TERMS[i][0]))
                else:
                    rhs = _rhs_term(i, lambda *at: _split_words(block(*at)))
                part = _dot(lhs, rhs)
                acc = part if acc is None else part + acc
                next(filler, None)
            prods.append(acc)
        c = [t.reshape(n_seg // 2, 1, n_mem, LANES) for t in _combine(prods)]
        return [jnp.concatenate([c[j], c[j + 2]], axis=1).reshape(n_seg, n_mem, LANES)
                for j in range(2)]

    def mix_first(u, blocks):
        for n, a in enumerate(blocks, 2 * u):
            a_v[:, first, lanes(n)] = a
            out_v[:, first, lanes(n)] = _mix(
                g_v[:, first, :], a, x_v[:, first, lanes(n)].astype(F32))

    for i, w in enumerate((wg_v, wu_v, wd_v)):
        wait_whole(w, sem_ffn[i])

    rest_copy.start()
    ffn = routed_ffn()
    for u in range(nk // 2):
        blocks = out_first(u, ffn)
        if u == nk // 2 - 1:
            for _ in ffn:
                pass
        mix_first(u, blocks)
    first_copies[1].start()
    for_routed_segments(lambda copy: copy.wait())
    for copy in first_copies:
        copy.wait()


@functools.partial(jax.jit, static_argnames=("A_seg_len",))
def pallas_gated_mix__memory_aug_recurrent_mem_tr__moe_arch_mod__prompt_kernel(
    A_x, A_mem0, A_Wq, A_Wk, A_Wv, A_Wo, A_seg_len, B_x, B_w_r, B_w_gate, B_w_up,
    B_w_down, gate_w,
):
    del B_x
    batch, n_tok, dm = A_x.shape
    n_mem = A_mem0.shape[1]
    n_head, dh = A_Wq.shape[1:]
    d_ff = B_w_gate.shape[1]
    seg = int(A_seg_len)
    n_seg = n_tok // seg
    n_pair, nk, nf = n_head // 2, dm // LANES, d_ff // LANES
    assert (batch, n_mem, seg, dh) == (1, 8, 32, LANES)
    assert dm % (4 * LANES) == 0 and d_ff % LANES == 0 and n_pair % PRO_PAIRS == 0
    assert n_tok % (seg * STEP_UNROLL) == 0 and n_seg <= LANES
    assert nk % (n_pair // PRO_PAIRS) == 0
    assert ROUTE_SLOTS + 3 * nf > (nk // 2 - 1) * 7 * (n_pair // 4)

    hbm = pl.BlockSpec(memory_space=pl.ANY)
    out = pl.pallas_call(
        _kernel,
        out_shape=jax.ShapeDtypeStruct((n_seg, seg, dm), A_x.dtype),
        in_specs=[hbm] * 11,
        out_specs=hbm,
        scratch_shapes=[
            pltpu.VMEM((n_seg, seg, dm), BF16),
            pltpu.VMEM((7, nk // 2, n_seg * n_mem // 4, LANES), U32),
            pltpu.VMEM((3 * n_pair, dm, LANES), U32),
            pltpu.VMEM((nk, n_head * dh // 2, LANES), U32),
            pltpu.VMEM((3 * n_pair, n_seg * n_mem, LANES), U32),
            pltpu.VMEM((7, n_pair, n_seg * n_mem // 4, LANES), U32),
            pltpu.VMEM((n_seg, seg, dm), F32),
            pltpu.VMEM((n_seg, seg, LANES), F32),
            pltpu.VMEM((n_mem, dm), F32),
            pltpu.VMEM((2 * (n_mem + seg), LANES), F32),
            pltpu.VMEM((seg, LANES), I32),
            pltpu.VMEM((n_mem, dm), BF16),
            pltpu.VMEM((nk, LANES), BF16),
            pltpu.VMEM((nk, LANES), BF16),
            pltpu.VMEM((nf, dm // 2, LANES), U32),
            pltpu.VMEM((nf, dm // 2, LANES), U32),
            pltpu.VMEM((nk, d_ff // 2, LANES), U32),
            pltpu.VMEM((n_seg, seg, dm), BF16),
            pltpu.SMEM((TOP_C,), I32),
            pltpu.SemaphoreType.DMA((N_FIXED_SEMS + 3 * n_pair,)),
        ],
        compiler_params=pltpu.CompilerParams(
            vmem_limit_bytes=116 * 1024 * 1024, disable_bounds_checks=True),
        name="gated_mix_rmt_mod",
    )(
        A_x.reshape(n_seg, seg, dm), A_mem0.reshape(n_mem, dm), A_Wq, A_Wk, A_Wv,
        A_Wo.reshape(n_head * dh, dm), B_w_r.reshape(nk, LANES), B_w_gate, B_w_up, B_w_down,
        gate_w.reshape(nk, LANES),
    )
    return out.reshape(batch, n_tok, dm)
```

```python
import functools

import jax
import jax.numpy as jnp
import numpy as np
from jax import lax
from jax.experimental import pallas as pl
from jax.experimental.pallas import tpu as pltpu

BF16, F32, U32, I32 = jnp.bfloat16, jnp.float32, jnp.uint32, jnp.int32
LANES = 128
TOP_C = 8
INT_MIN = -(2 ** 31)
HI16 = np.uint32(0xFFFF0000)

FLAGS = None
PRO_PAIRS = 2
STEP_UNROLL = 2
QK_LAG, PV_LAG = 3, 4
FIRST_LAG = 0
ROUTE_SLOTS = 8
EARLY_HALVES = 6


def _dot(a, b):
    return jnp.dot(a, b, preferred_element_type=F32)


def _as_bf16(words):
    return pltpu.bitcast(words, BF16)


def _to_words(v):
    return pltpu.bitcast(v.astype(BF16), U32)


def _split_words(words):
    return pltpu.bitcast(words << 16, F32), pltpu.bitcast(words & HI16, F32)


def _sigmoid(v):
    return 1.0 / (1.0 + jnp.exp(-v))


def _mix(gate, a, b):
    return (gate * a + (1.0 - gate) * b).astype(BF16)


def _lhs_terms(a, b, c, d):
    return [c + d, a, a + b, d, a + d, c - a, b - d]


RHS_TERMS = (((0, 0),), ((0, 1), jnp.subtract, (1, 1)), ((1, 1),), ((1, 0), jnp.subtract, (0, 0)),
             ((0, 0), jnp.add, (1, 1)), ((0, 0), jnp.add, (0, 1)), ((1, 0), jnp.add, (1, 1)))


def _rhs_term(i, block):
    term = RHS_TERMS[i]
    out = block(i, *term[0])
    if len(term) > 1:
        out = term[1](out.astype(F32), block(i, *term[2]).astype(F32))
    return out.astype(BF16)


def _opaque_zero(count, i):
    return count >> (16 + i)


def _combine(m):
    return [m[3] - m[2] + m[4] + m[6], m[1] + m[2], m[0] + m[3], m[1] - m[0] + m[4] + m[5]]


def _score_fill(n_mem, seg):
    shape = (2 * (n_mem + seg), LANES)

    def decode(i):
        tail = i >= 2 * seg
        head = jnp.where(tail, (i - 2 * seg) >> 3, i >> 5)
        r = i & (seg - 1)
        pos = jnp.where(tail, n_mem + (i & 7), jnp.where(r < n_mem, r, r + n_mem))
        return head, pos

    rh, rp = decode(lax.broadcasted_iota(I32, shape, 0))
    ch, cp = decode(lax.broadcasted_iota(I32, shape, 1))
    visible = (rp < n_mem) | (rp >= cp)
    return jnp.where(rh == ch, jnp.where(visible, 0.0, -1e9), -jnp.inf).astype(F32)


def _kernel(x_hbm, mem0_hbm, wq_hbm, wk_hbm, wv_hbm, wo_hbm, wr_hbm, wg_hbm, wu_hbm,
            wd_hbm, gw_hbm, out_hbm,
            x_v, x_terms, wqkv, wo_v, qkv0, o_terms, a_v, g_v, mem, fill_v, key_v,
            mem0_ref, wr_ref, gw_ref, wg_v, wu_v, wd_v, out_v, idx_s,
            sems):
    n_seg, seg, dm = x_v.shape
    n_mem = mem.shape[0]
    n_pair = wqkv.shape[0] // 3
    n_head = 2 * n_pair
    nk = dm // LANES
    nf = wg_v.shape[0]
    scale = LANES ** -0.5
    w_hbm = (wq_hbm, wk_hbm, wv_hbm)
    first, rest = pl.ds(0, n_mem), pl.ds(n_mem, seg - n_mem)

    def lanes(n):
        return slice(n * LANES, (n + 1) * LANES)

    sem_a, sem_b = sems.at[0], sems.at[1]

    def w_copy(m, p, sem):
        return pltpu.make_async_copy(w_hbm[m].bitcast(U32).at[:, p, :], wqkv.at[3 * p + m], sem)

    def col_copy(src, dst, n, sem):
        start = n * LANES if isinstance(n, int) else pl.multiple_of(n * LANES, LANES)
        cols = pl.ds(start, LANES)
        return pltpu.make_async_copy(src.bitcast(U32).at[:, cols], dst.at[n], sem)

    def wait_whole(dst, sem):
        pltpu.make_async_copy(dst, dst, sem).wait()

    x_first = pltpu.make_async_copy(x_hbm.at[:, first, :], x_v.at[:, first, :], sem_a)
    x_rest = pltpu.make_async_copy(x_hbm.at[:, rest, :], x_v.at[:, rest, :], sem_b)

    units = [(m, j) for j in range(PRO_PAIRS) for m in range(3)]
    small = [pltpu.make_async_copy(src, dst, sem_b)
             for src, dst in ((mem0_hbm, mem0_ref), (wr_hbm, wr_ref), (gw_hbm, gw_ref))]

    def group_sem(it):
        return sems.at[2 + (it & 1)]

    x_first.start()
    for u, (m, j) in enumerate(units):
        w_copy(m, j, sems.at[4 + u]).start()
    for m, j in units:
        w_copy(m, PRO_PAIRS + j, group_sem(1)).start()

    fill_v[...] = _score_fill(n_mem, seg)
    key_v[...] = jnp.full(key_v.shape, INT_MIN, I32)
    spare = 3 * n_pair
    wqkv[spare] = jnp.zeros((dm, LANES), U32)

    half_rows = n_seg * n_mem // 2
    x_first.wait()
    for n in range(nk // 2):
        lo, hi = (x_v[:, 0:n_mem, lanes(n + i * nk // 2)].astype(F32).reshape(2, half_rows, LANES)
                  for i in range(2))
        for i, t in enumerate(_lhs_terms(lo[0], hi[0], lo[1], hi[1])):
            x_terms[i, n] = _to_words(t)

    def regroup(w, piece, n_piece):
        groups = dm // 16
        for r in range(groups * piece // n_piece * 16, groups * (piece + 1) // n_piece * 16, 16):
            even = wqkv[w, pl.ds(r, 8, stride=2), :]
            odd = wqkv[w, pl.ds(r + 1, 8, stride=2), :]
            wqkv[w, r:r + 8, :] = (even & np.uint32(0xFFFF)) | (odd << 16)
            wqkv[w, r + 8:r + 16, :] = (even >> 16) | (odd & HI16)

    def project_first(w, previous):
        def block(i, row, col):
            words = wqkv[w + _opaque_zero(w, i), row * (dm // 2):(row + 1) * (dm // 2), :]
            return _split_words(words)[col]

        prods = []
        for i in range(7):
            lhs = jnp.concatenate([_as_bf16(x_terms[i, n]) for n in range(nk // 2)], axis=1)
            prods.append(_dot(lhs, _rhs_term(i, block)))
            regroup(previous, i, 7)
        c = [t.reshape(n_seg // 2, n_mem, LANES) for t in _combine(prods)]
        for i in range(2):
            both = jnp.concatenate(c[2 * i:2 * i + 2], axis=1).reshape(2 * half_rows, LANES)
            qkv0[w, i * half_rows:(i + 1) * half_rows, :] = _to_words(both)

    n_pro = n_pair // PRO_PAIRS
    wo_per_it = nk // n_pro

    def ramp(w, carry):
        wait_whole(wqkv.at[w], sems.at[4 + w])
        project_first(w, jnp.where(w > 0, w - 1, spare))
        return carry

    lax.fori_loop(0, len(units), ramp, 0)
    for copy in small:
        copy.start()
    for n in range(wo_per_it):
        col_copy(wo_hbm, wo_v, n, sem_b).start()

    def prologue(it, carry):
        p0 = it * PRO_PAIRS

        @pl.when(it + 1 < n_pro)
        def _():
            for m, j in units:
                w_copy(m, p0 + PRO_PAIRS + j, group_sem(it + 1)).start()

        for n in range(wo_per_it):
            col_copy(wo_hbm, wo_v, it * wo_per_it + n, sem_b).start()

        @pl.when(it == n_pro // 2)
        def _():
            x_rest.start()

        wait_whole(wqkv.at[pl.ds(3 * p0, len(units))], group_sem(it))
        for u in range(len(units)):
            project_first(3 * p0 + u, 3 * p0 + u - 1)
        return carry

    lax.fori_loop(1, n_pro, prologue, 0)

    regroup(3 * n_pair - 1, 0, 1)
    x_rest.wait()
    wait_whole(wo_v, sem_b)
    for copy in small:
        copy.wait()
    mem[...] = mem0_ref[...].astype(F32)

    def row_dot(rows, w):
        acc = rows[:, lanes(0)] * w[0:1, :]
        for n in range(1, nk):
            acc = acc + rows[:, lanes(n)] * w[n:n + 1, :]
        return jnp.sum(acc, axis=-1, keepdims=True)

    def head_weights(m, hd, lo, hi):
        w = wqkv[3 * (hd // 2) + m, lo * LANES:hi * LANES, :].reshape(-1, 2, 8, LANES)
        return _as_bf16(w[:, hd % 2].reshape(-1, LANES))

    def segment(s, mem_cols, mem_is_late):
        xs = x_v[s]
        xf = xs.astype(F32)
        h_cols = [
            jnp.concatenate(
                [jnp.concatenate([mem_cols[n], xf[n_mem:2 * n_mem, lanes(n)]], axis=0).astype(BF16),
                 xs[2 * n_mem:, lanes(n)]], axis=0)
            for n in range(nk)]
        rows0 = pl.ds(pl.multiple_of(s * n_mem, n_mem), n_mem)
        pad = jnp.zeros((LANES - 2 * (seg + n_mem), LANES), F32)

        def partial_proj(m, hd, lo, hi):
            return _dot(jnp.concatenate(h_cols[lo:hi], axis=1), head_weights(m, hd, lo, hi))

        early = {}
        if mem_is_late:
            order = [(m, 2 * p + j) for p in range(n_pair) for m in (1, 0, 2) for j in range(2)]
            for m, hd in order[:EARLY_HALVES]:
                early[m, hd] = partial_proj(m, hd, 0, nk // 2)

        def project(m, p):
            out = []
            for hd in (2 * p, 2 * p + 1):
                if (m, hd) in early:
                    r = partial_proj(m, hd, nk // 2, nk) + early[m, hd]
                else:
                    r = partial_proj(m, hd, 0, nk)
                out.append(r)
            out.append(_as_bf16(qkv0[3 * p + m, rows0, :]).astype(F32))
            return jnp.concatenate(out + [pad] * (m > 0), axis=0).astype(BF16)

        def probabilities(q, k):
            sc = lax.dot_general(q, k, (((1,), (1,)), ((), ())), preferred_element_type=F32)
            fill = fill_v[...]
            sc = jnp.where(fill == 0.0, sc * scale, fill)
            e = jnp.exp(sc - jnp.max(sc, axis=-1, keepdims=True))
            den = jnp.sum(e, axis=-1, keepdims=True)
            inv = pl.reciprocal(den, approx=True)
            inv = inv * (2.0 - den * inv)
            return (e * inv).astype(BF16)

        def out_proj(lo, hi, n):
            lhs = jnp.concatenate([heads[i] for i in range(lo, hi)], axis=1)
            return _dot(lhs, _as_bf16(wo_v[n, lo * (LANES // 2):hi * (LANES // 2), :]))

        slots = [(m, p) for p in range(n_pair) for m in (1, 0, 2)] + [(3, n) for n in range(nk)]
        res, prob, heads, o_first = {}, {}, {}, {}
        for i, (m, j) in enumerate(slots):
            res[m, j] = project(m, j) if m < 3 else out_proj(0, n_pair, j)
            for p in range(n_pair):
                extra = 0 if mem_is_late else max(FIRST_LAG - p, 0)
                if i == 3 * p + 1 + QK_LAG:
                    prob[p] = probabilities(res[0, p], res[1, p])
                if i == min(3 * p + 1 + QK_LAG + PV_LAG + extra, len(slots) - 1):
                    o = _dot(prob[p], res[2, p])
                    ob = o[0:2 * seg].astype(BF16)
                    heads[2 * p], heads[2 * p + 1] = ob[0:seg], ob[seg:]
                    o_first[2 * p] = o[2 * seg:2 * seg + n_mem]
                    o_first[2 * p + 1] = o[2 * seg + n_mem:]
        gate = jnp.broadcast_to(_sigmoid(row_dot(xf, gw_ref[...].astype(F32))), (seg, LANES))
        g_v[s] = gate
        new_mem = []
        for n in range(nk):
            r = out_proj(n_pair, n_head, n) + res[3, n]
            new_mem.append(r[0:n_mem])
            a_v[s, rest, lanes(n)] = r[n_mem:]
            out_v[s, rest, lanes(n)] = _mix(gate[n_mem:], r[n_mem:], xf[n_mem:, lanes(n)])

        score = row_dot(xf, wr_ref[...].astype(F32)).astype(BF16).astype(F32)
        score = jnp.broadcast_to(score, (seg, LANES))
        bits = pltpu.bitcast(jnp.where(score == 0.0, 0.0, score), I32)
        order = jnp.where(bits < 0, bits ^ np.int32(0x7FFFFFFF), bits)
        order = jnp.where(score != score, INT_MIN, order)
        token = s * seg + lax.broadcasted_iota(I32, (seg, LANES), 0)
        key = (order & np.int32(-65536)) | (65535 - token)
        lane = lax.broadcasted_iota(I32, (seg, LANES), 1)
        key_v[...] = jnp.where(lane == s, key, key_v[...])
        return new_mem, o_first

    n_step = n_seg // STEP_UNROLL

    def out_copy(segs, rows, cols, sem):
        return pltpu.make_async_copy(
            out_v.at[segs, rows, cols], out_hbm.at[segs, rows, cols], sem)

    every_seg, every_col = pl.ds(0, n_seg), pl.ds(0, dm)
    def step(it, carry):
        @pl.when(it > 0)
        def _():
            done = pl.ds((it - 1) * STEP_UNROLL, STEP_UNROLL)
            out_copy(done, rest, every_col, sem_b).start()

        for dst, src in ((wg_v, wg_hbm), (wu_v, wu_hbm), (wd_v, wd_hbm)):
            per_step = pl.cdiv(dst.shape[0], n_step)
            for i in range(per_step):
                @pl.when(it * per_step + i < dst.shape[0])
                def _():
                    col_copy(src, dst, it * per_step + i, sem_a).start()

        mem_cols = [mem[:, lanes(n)] for n in range(nk)]
        for u0 in range(0, STEP_UNROLL, 2):
            o = []
            for u in (u0, u0 + 1):
                mem_cols, o_first = segment(it * STEP_UNROLL + u, mem_cols, u > 0)
                o.append(o_first)
            rows = pl.ds(pl.multiple_of((it * STEP_UNROLL + u0) * 2, 4), 4)
            for hd in range(n_pair):
                a, b, c, d = (o[i][j] for i in range(2) for j in (hd, hd + n_pair))
                for i, t in enumerate(_lhs_terms(a, b, c, d)):
                    o_terms[i, hd, rows, :] = _to_words(jnp.concatenate([t, t], axis=0))[0:4]
        for n in range(nk):
            mem[:, lanes(n)] = mem_cols[n]
        return carry + 1

    steps = lax.fori_loop(0, n_step, step, 0)

    last_copy = out_copy(pl.ds(n_seg - STEP_UNROLL, STEP_UNROLL), rest, every_col, sem_a)
    first_copies = [out_copy(every_seg, first, pl.ds(0, dm - 2 * LANES), sem_a),
                    out_copy(every_seg, first, pl.ds(dm - 2 * LANES, 2 * LANES), sem_a)]

    def for_routed_segments(fn):
        segs = [idx_s[i] // seg for i in range(TOP_C)]
        for i, s in enumerate(segs):
            new = functools.reduce(jnp.logical_and, [s != t for t in segs[:i]], s < n_early)
            pl.when(new)(lambda: fn(out_copy(pl.ds(s, 1), rest, every_col, sem_b)))

    row = lax.broadcasted_iota(I32, (n_mem, dm), 0)

    def routed_ffn():
        keys = key_v[...]
        for i in range(TOP_C):
            best = jnp.max(keys)
            idx_s[i] = 65535 - (best & 65535)
            keys = jnp.where(keys == best, INT_MIN, keys)
        slot = lax.broadcasted_iota(I32, (2 * TOP_C, dm), 0)
        x_sel = jnp.zeros((2 * TOP_C, dm), F32)
        for i in range(TOP_C):
            t = idx_s[i]
            rows = pl.ds(pl.multiple_of(t & (seg - n_mem), n_mem), n_mem)
            picked = jnp.where(row == (t & (n_mem - 1)), x_v[t // seg, rows, :].astype(F32), 0.0)
            x_sel = jnp.where(slot == i, jnp.sum(picked, axis=0, keepdims=True), x_sel)
        r_sel = _sigmoid(row_dot(x_sel, wr_ref[...].astype(F32)))
        lhs = x_sel.astype(BF16)
        for _ in range(ROUTE_SLOTS):
            yield
        hidden = []
        for n in range(nf):
            gt = _dot(lhs, _as_bf16(wg_v[n]))
            yield
            up = _dot(lhs, _as_bf16(wu_v[n]))
            hidden.append((gt * _sigmoid(gt) * up).astype(BF16))
            yield
        y = [None] * nk
        for lo in range(0, nf, nk):
            hi = min(lo + nk, nf)
            lhs = jnp.concatenate(hidden[lo:hi], axis=1)
            for n in range(nk):
                part = _dot(lhs, _as_bf16(wd_v[n, lo * (LANES // 2):hi * (LANES // 2), :]))
                y[n] = part if y[n] is None else part + y[n]
                if (n + 1) * (hi - lo) % nk < hi - lo:
                    yield
        y = jnp.concatenate(y, axis=1) * r_sel
        for i in range(TOP_C):
            yield
            t = idx_s[i]
            s, r0 = t // seg, pl.multiple_of(t & (seg - n_mem), n_mem)
            rows = pl.ds(r0, n_mem)
            upd = jnp.where(row == (t & (n_mem - 1)), y[i:i + 1, :], 0.0)
            b = (x_v[s, rows, :].astype(F32) + upd).astype(BF16)
            x_v[s, rows, :] = b
            later = pl.ds(pl.multiple_of(jnp.maximum(r0, n_mem), n_mem), n_mem)
            gate, b = g_v[s, rows, :], b.astype(F32)
            for n in range(nk):
                a = a_v[s, rows if n < nk - 2 else later, lanes(n)]
                out_v[s, rows, lanes(n)] = _mix(gate, a, b[:, lanes(n)])
        yield
        first_copies[0].start()
        last_copy.start()
        for_routed_segments(lambda copy: copy.start())

    def out_first(u, filler):
        prods = []
        for i in range(7):
            acc = None
            for lo in range(0, n_pair, 4):
                lhs = jnp.concatenate(
                    [_as_bf16(o_terms[i, hd]) for hd in range(lo, lo + 4)], axis=1)

                def block(i, row, col):
                    r0 = row * (wo_v.shape[1] // 2) + lo * (LANES // 2)
                    return _as_bf16(
                        wo_v[2 * u + col + _opaque_zero(steps, i), r0:r0 + 2 * LANES, :])

                part = _dot(lhs, _rhs_term(i, block))
                acc = part if acc is None else part + acc
                next(filler, None)
            prods.append(acc)
        c = [t.reshape(n_seg // 2, 1, n_mem, LANES) for t in _combine(prods)]
        return [jnp.concatenate([c[j], c[j + 2]], axis=1).reshape(n_seg, n_mem, LANES)
                for j in range(2)]

    def mix_first(u, blocks):
        for n, a in enumerate(blocks, 2 * u):
            a_v[:, first, lanes(n)] = a
            out_v[:, first, lanes(n)] = _mix(
                g_v[:, first, :], a, x_v[:, first, lanes(n)].astype(F32))

    for w in (wg_v, wu_v, wd_v):
        wait_whole(w, sem_a)
    n_early = n_seg - STEP_UNROLL
    out_copy(pl.ds(0, n_early), rest, every_col, sem_b).wait()

    ffn = routed_ffn()
    for u in range(nk // 2):
        blocks = out_first(u, ffn)
        if u == nk // 2 - 1:
            for _ in ffn:
                pass
        mix_first(u, blocks)
    first_copies[1].start()
    for_routed_segments(lambda copy: copy.wait())
    for copy in first_copies + [last_copy]:
        copy.wait()


@functools.partial(jax.jit, static_argnames=("A_seg_len",))
def pallas_gated_mix__memory_aug_recurrent_mem_tr__moe_arch_mod__prompt_kernel(
    A_x, A_mem0, A_Wq, A_Wk, A_Wv, A_Wo, A_seg_len, B_x, B_w_r, B_w_gate, B_w_up,
    B_w_down, gate_w,
):
    del B_x
    batch, n_tok, dm = A_x.shape
    n_mem = A_mem0.shape[1]
    n_head, dh = A_Wq.shape[1:]
    d_ff = B_w_gate.shape[1]
    seg = int(A_seg_len)
    n_seg = n_tok // seg
    n_pair, nk, nf = n_head // 2, dm // LANES, d_ff // LANES
    assert (batch, n_mem, seg, dh) == (1, 8, 32, LANES)
    assert dm % (4 * LANES) == 0 and d_ff % LANES == 0 and n_pair % PRO_PAIRS == 0
    assert n_tok % (seg * STEP_UNROLL) == 0 and n_seg <= LANES
    assert nk % (n_pair // PRO_PAIRS) == 0
    assert ROUTE_SLOTS + 3 * nf > (nk // 2 - 1) * 7 * (n_pair // 4)

    hbm = pl.BlockSpec(memory_space=pl.ANY)
    out = pl.pallas_call(
        _kernel,
        out_shape=jax.ShapeDtypeStruct((n_seg, seg, dm), A_x.dtype),
        in_specs=[hbm] * 11,
        out_specs=hbm,
        scratch_shapes=[
            pltpu.VMEM((n_seg, seg, dm), BF16),
            pltpu.VMEM((7, nk // 2, n_seg * n_mem // 4, LANES), U32),
            pltpu.VMEM((3 * n_pair + 1, dm, LANES), U32),
            pltpu.VMEM((nk, n_head * dh // 2, LANES), U32),
            pltpu.VMEM((3 * n_pair, n_seg * n_mem, LANES), U32),
            pltpu.VMEM((7, n_pair, n_seg * n_mem // 4, LANES), U32),
            pltpu.VMEM((n_seg, seg, dm), F32),
            pltpu.VMEM((n_seg, seg, LANES), F32),
            pltpu.VMEM((n_mem, dm), F32),
            pltpu.VMEM((2 * (n_mem + seg), LANES), F32),
            pltpu.VMEM((seg, LANES), I32),
            pltpu.VMEM((n_mem, dm), BF16),
            pltpu.VMEM((nk, LANES), BF16),
            pltpu.VMEM((nk, LANES), BF16),
            pltpu.VMEM((nf, dm // 2, LANES), U32),
            pltpu.VMEM((nf, dm // 2, LANES), U32),
            pltpu.VMEM((nk, d_ff // 2, LANES), U32),
            pltpu.VMEM((n_seg, seg, dm), BF16),
            pltpu.SMEM((TOP_C,), I32),
            pltpu.SemaphoreType.DMA((4 + 3 * PRO_PAIRS,)),
        ],
        compiler_params=pltpu.CompilerParams(
            vmem_limit_bytes=116 * 1024 * 1024, disable_bounds_checks=True, flags=FLAGS),
        name="gated_mix_rmt_mod",
    )(
        A_x.reshape(n_seg, seg, dm), A_mem0.reshape(n_mem, dm), A_Wq, A_Wk, A_Wv,
        A_Wo.reshape(n_head * dh, dm), B_w_r.reshape(nk, LANES), B_w_gate, B_w_up, B_w_down,
        gate_w.reshape(nk, LANES),
    )
    return out.reshape(batch, n_tok, dm)
```

```python
import functools

import jax
import jax.numpy as jnp
import numpy as np
from jax import lax
from jax.experimental import pallas as pl
from jax.experimental.pallas import tpu as pltpu

BF16, F32, U32, I32 = jnp.bfloat16, jnp.float32, jnp.uint32, jnp.int32
LANES = 128
TOP_C = 8
INT_MIN = -(2 ** 31)
HI16 = np.uint32(0xFFFF0000)

FLAGS = {"XLA_TPU_EVENLY_DISTRIBUTE_CRITICAL_NODES": True}
PRO_PAIRS = 2
STEP_UNROLL = 2
QKV_ORDER = (1, 0, 2)
QK_LAG, PV_LAG = 3, 10
QK_START, PV_START = 0, 4
EARLY_HEADS = 24
ROUTE_SLOTS = 8
EARLY_HALVES = 6


def _dot(a, b):
    return jnp.dot(a, b, preferred_element_type=F32)


def _as_bf16(words):
    return pltpu.bitcast(words, BF16)


def _to_words(v):
    return pltpu.bitcast(v.astype(BF16), U32)


def _split_words(words):
    return pltpu.bitcast(words << 16, F32), pltpu.bitcast(words & HI16, F32)


def _sigmoid(v):
    return 1.0 / (1.0 + jnp.exp(-v))


def _mix(gate, a, b):
    return (gate * a + (1.0 - gate) * b).astype(BF16)


def _lhs_terms(a, b, c, d):
    return [c + d, a, a + b, d, a + d, c - a, b - d]


RHS_TERMS = (((0, 0),), ((0, 1), jnp.subtract, (1, 1)), ((1, 1),), ((1, 0), jnp.subtract, (0, 0)),
             ((0, 0), jnp.add, (1, 1)), ((0, 0), jnp.add, (0, 1)), ((1, 0), jnp.add, (1, 1)))


def _rhs_term(i, block):
    term = RHS_TERMS[i]
    out = block(i, *term[0])
    if len(term) > 1:
        out = term[1](out.astype(F32), block(i, *term[2]).astype(F32))
    return out.astype(BF16)


def _opaque_zero(count, i):
    return count >> (16 + i)


def _combine(m):
    return [m[3] - m[2] + m[4] + m[6], m[1] + m[2], m[0] + m[3], m[1] - m[0] + m[4] + m[5]]


def _score_fill(n_mem, seg):
    shape = (2 * (n_mem + seg), LANES)

    def decode(i):
        tail = i >= 2 * seg
        head = jnp.where(tail, (i - 2 * seg) >> 3, i >> 5)
        r = i & (seg - 1)
        pos = jnp.where(tail, n_mem + (i & 7), jnp.where(r < n_mem, r, r + n_mem))
        return head, pos

    rh, rp = decode(lax.broadcasted_iota(I32, shape, 0))
    ch, cp = decode(lax.broadcasted_iota(I32, shape, 1))
    visible = (rp < n_mem) | (rp >= cp)
    return jnp.where(rh == ch, jnp.where(visible, 0.0, -1e9), -jnp.inf).astype(F32)


def _kernel(x_hbm, mem0_hbm, wq_hbm, wk_hbm, wv_hbm, wo_hbm, wr_hbm, wg_hbm, wu_hbm,
            wd_hbm, gw_hbm, out_hbm,
            x_v, x_terms, wqkv, wo_v, qkv0, o_terms, a_v, g_v, mem, fill_v, key_v,
            mem0_ref, wr_ref, gw_ref, wg_v, wu_v, wd_v, out_v, idx_s,
            sems):
    n_seg, seg, dm = x_v.shape
    n_mem = mem.shape[0]
    n_pair = wqkv.shape[0] // 3
    n_head = 2 * n_pair
    nk = dm // LANES
    nf = wg_v.shape[0]
    scale = LANES ** -0.5
    w_hbm = (wq_hbm, wk_hbm, wv_hbm)
    first, rest = pl.ds(0, n_mem), pl.ds(n_mem, seg - n_mem)

    def lanes(n):
        return slice(n * LANES, (n + 1) * LANES)

    sem_a, sem_b = sems.at[0], sems.at[1]

    def w_copy(m, p, sem):
        return pltpu.make_async_copy(w_hbm[m].bitcast(U32).at[:, p, :], wqkv.at[3 * p + m], sem)

    def col_copy(src, dst, n, sem):
        start = n * LANES if isinstance(n, int) else pl.multiple_of(n * LANES, LANES)
        cols = pl.ds(start, LANES)
        return pltpu.make_async_copy(src.bitcast(U32).at[:, cols], dst.at[n], sem)

    def wait_whole(dst, sem):
        pltpu.make_async_copy(dst, dst, sem).wait()

    x_first = pltpu.make_async_copy(x_hbm.at[:, first, :], x_v.at[:, first, :], sem_a)
    x_rest = pltpu.make_async_copy(x_hbm.at[:, rest, :], x_v.at[:, rest, :], sem_b)

    units = [(m, j) for j in range(PRO_PAIRS) for m in range(3)]
    small = [pltpu.make_async_copy(src, dst, sem_b)
             for src, dst in ((mem0_hbm, mem0_ref), (wr_hbm, wr_ref), (gw_hbm, gw_ref))]

    def group_sem(it):
        return sems.at[2 + (it & 1)]

    x_first.start()
    for u, (m, j) in enumerate(units):
        w_copy(m, j, sems.at[4 + u]).start()
    for m, j in units:
        w_copy(m, PRO_PAIRS + j, group_sem(1)).start()

    fill_v[...] = _score_fill(n_mem, seg)
    key_v[...] = jnp.full(key_v.shape, INT_MIN, I32)
    spare = 3 * n_pair
    wqkv[spare] = jnp.zeros((dm, LANES), U32)

    half_rows = n_seg * n_mem // 2
    x_first.wait()
    for n in range(nk // 2):
        lo, hi = (x_v[:, 0:n_mem, lanes(n + i * nk // 2)].astype(F32).reshape(2, half_rows, LANES)
                  for i in range(2))
        for i, t in enumerate(_lhs_terms(lo[0], hi[0], lo[1], hi[1])):
            x_terms[i, n] = _to_words(t)

    def regroup(w, piece, n_piece):
        groups = dm // 16
        for r in range(groups * piece // n_piece * 16, groups * (piece + 1) // n_piece * 16, 16):
            even = wqkv[w, pl.ds(r, 8, stride=2), :]
            odd = wqkv[w, pl.ds(r + 1, 8, stride=2), :]
            wqkv[w, r:r + 8, :] = (even & np.uint32(0xFFFF)) | (odd << 16)
            wqkv[w, r + 8:r + 16, :] = (even >> 16) | (odd & HI16)

    def project_first(w, previous):
        def block(i, row, col):
            words = wqkv[w + _opaque_zero(w, i), row * (dm // 2):(row + 1) * (dm // 2), :]
            return _split_words(words)[col]

        prods = []
        for i in range(7):
            lhs = jnp.concatenate([_as_bf16(x_terms[i, n]) for n in range(nk // 2)], axis=1)
            prods.append(_dot(lhs, _rhs_term(i, block)))
            regroup(previous, i, 7)
        c = [t.reshape(n_seg // 2, n_mem, LANES) for t in _combine(prods)]
        for i in range(2):
            both = jnp.concatenate(c[2 * i:2 * i + 2], axis=1).reshape(2 * half_rows, LANES)
            qkv0[w, i * half_rows:(i + 1) * half_rows, :] = _to_words(both)

    n_pro = n_pair // PRO_PAIRS
    wo_per_it = nk // n_pro

    def ramp(w, carry):
        wait_whole(wqkv.at[w], sems.at[4 + w])
        project_first(w, jnp.where(w > 0, w - 1, spare))
        return carry

    lax.fori_loop(0, len(units), ramp, 0)
    for copy in small:
        copy.start()
    for n in range(wo_per_it):
        col_copy(wo_hbm, wo_v, n, sem_b).start()

    def prologue(it, carry):
        p0 = it * PRO_PAIRS

        @pl.when(it + 1 < n_pro)
        def _():
            for m, j in units:
                w_copy(m, p0 + PRO_PAIRS + j, group_sem(it + 1)).start()

        for n in range(wo_per_it):
            col_copy(wo_hbm, wo_v, it * wo_per_it + n, sem_b).start()

        @pl.when(it == n_pro // 2)
        def _():
            x_rest.start()

        wait_whole(wqkv.at[pl.ds(3 * p0, len(units))], group_sem(it))
        for u in range(len(units)):
            project_first(3 * p0 + u, 3 * p0 + u - 1)
        return carry

    lax.fori_loop(1, n_pro, prologue, 0)

    regroup(3 * n_pair - 1, 0, 1)
    x_rest.wait()
    wait_whole(wo_v, sem_b)
    for copy in small:
        copy.wait()
    mem[...] = mem0_ref[...].astype(F32)

    def row_dot(rows, w):
        acc = rows[:, lanes(0)] * w[0:1, :]
        for n in range(1, nk):
            acc = acc + rows[:, lanes(n)] * w[n:n + 1, :]
        return jnp.sum(acc, axis=-1, keepdims=True)

    def head_weights(m, hd, lo, hi):
        w = wqkv[3 * (hd // 2) + m, lo * LANES:hi * LANES, :].reshape(-1, 2, 8, LANES)
        return _as_bf16(w[:, hd % 2].reshape(-1, LANES))

    def segment(s, mem_cols, mem_is_late):
        xs = x_v[s]
        xf = xs.astype(F32)
        h_cols = [
            jnp.concatenate(
                [jnp.concatenate([mem_cols[n], xf[n_mem:2 * n_mem, lanes(n)]], axis=0).astype(BF16),
                 xs[2 * n_mem:, lanes(n)]], axis=0)
            for n in range(nk)]
        rows0 = pl.ds(pl.multiple_of(s * n_mem, n_mem), n_mem)
        pad = jnp.zeros((LANES - 2 * (seg + n_mem), LANES), F32)

        def partial_proj(m, hd, lo, hi):
            return _dot(jnp.concatenate(h_cols[lo:hi], axis=1), head_weights(m, hd, lo, hi))

        slots = [(m, 2 * p + j) for p in range(n_pair) for m in QKV_ORDER for j in range(2)]
        early = {}
        if mem_is_late:
            for m, hd in slots[:EARLY_HALVES]:
                early[m, hd] = partial_proj(m, hd, 0, nk // 2)

        def project(m, hd):
            if (m, hd) in early:
                return partial_proj(m, hd, nk // 2, nk) + early[m, hd]
            return partial_proj(m, hd, 0, nk)

        def both_heads(m, p):
            rows = [res[m, 2 * p], res[m, 2 * p + 1],
                    _as_bf16(qkv0[3 * p + m, rows0, :]).astype(F32)]
            return jnp.concatenate(rows + [pad] * (m > 0), axis=0).astype(BF16)

        def probabilities(q, k):
            sc = lax.dot_general(q, k, (((1,), (1,)), ((), ())), preferred_element_type=F32)
            fill = fill_v[...]
            sc = jnp.where(fill == 0.0, sc * scale, fill)
            e = jnp.exp(sc - jnp.max(sc, axis=-1, keepdims=True))
            den = jnp.sum(e, axis=-1, keepdims=True)
            inv = pl.reciprocal(den, approx=True)
            inv = inv * (2.0 - den * inv)
            return (e * inv).astype(BF16)

        def out_proj(lo, hi, n):
            lhs = jnp.concatenate([heads[i] for i in range(lo, hi)], axis=1)
            return _dot(lhs, _as_bf16(wo_v[n, lo * (LANES // 2):hi * (LANES // 2), :]))

        slots += [(3 + j, n) for n in range(nk) for j in range(2)]
        res, prob, heads, o_first = {}, {}, {}, {}
        for i, (m, j) in enumerate(slots):
            if m < 3:
                res[m, j] = project(m, j)
            elif m == 3:
                res[3, j] = out_proj(0, EARLY_HEADS // 2, j)
            else:
                res[3, j] = out_proj(EARLY_HEADS // 2, EARLY_HEADS, j) + res[3, j]
            for p in range(n_pair):
                ready = [slots.index((t, 2 * p + 1)) for t in range(3)]
                qk_at = max(ready[:2]) + QK_LAG
                pv_at = qk_at + PV_LAG
                if not mem_is_late:
                    qk_at += max(QK_START - 2 * p, 0)
                    pv_at += max(QK_START - 2 * p, 0) + max(PV_START - 2 * p, 0)
                if i == qk_at:
                    prob[p] = probabilities(both_heads(0, p), both_heads(1, p))
                if i == min(max(pv_at, ready[2] + 2), len(slots) - 1):
                    o = _dot(prob[p], both_heads(2, p))
                    ob = o[0:2 * seg].astype(BF16)
                    heads[2 * p], heads[2 * p + 1] = ob[0:seg], ob[seg:]
                    o_first[2 * p] = o[2 * seg:2 * seg + n_mem]
                    o_first[2 * p + 1] = o[2 * seg + n_mem:]
        gate = jnp.broadcast_to(_sigmoid(row_dot(xf, gw_ref[...].astype(F32))), (seg, LANES))
        g_v[s] = gate
        new_mem = []
        for n in range(nk):
            r = out_proj(EARLY_HEADS, n_head, n) + res[3, n]
            new_mem.append(r[0:n_mem])
            a_v[s, rest, lanes(n)] = r[n_mem:]
            out_v[s, rest, lanes(n)] = _mix(gate[n_mem:], r[n_mem:], xf[n_mem:, lanes(n)])

        score = row_dot(xf, wr_ref[...].astype(F32)).astype(BF16).astype(F32)
        score = jnp.broadcast_to(score, (seg, LANES))
        bits = pltpu.bitcast(jnp.where(score == 0.0, 0.0, score), I32)
        order = jnp.where(bits < 0, bits ^ np.int32(0x7FFFFFFF), bits)
        order = jnp.where(score != score, INT_MIN, order)
        token = s * seg + lax.broadcasted_iota(I32, (seg, LANES), 0)
        key = (order & np.int32(-65536)) | (65535 - token)
        lane = lax.broadcasted_iota(I32, (seg, LANES), 1)
        key_v[...] = jnp.where(lane == s, key, key_v[...])
        return new_mem, o_first

    n_step = n_seg // STEP_UNROLL

    def out_copy(segs, rows, cols, sem):
        return pltpu.make_async_copy(
            out_v.at[segs, rows, cols], out_hbm.at[segs, rows, cols], sem)

    every_seg, every_col = pl.ds(0, n_seg), pl.ds(0, dm)
    def step(it, carry):
        @pl.when(it > 0)
        def _():
            done = pl.ds((it - 1) * STEP_UNROLL, STEP_UNROLL)
            out_copy(done, rest, every_col, sem_b).start()

        for dst, src in ((wg_v, wg_hbm), (wu_v, wu_hbm), (wd_v, wd_hbm)):
            per_step = pl.cdiv(dst.shape[0], n_step)
            for i in range(per_step):
                @pl.when(it * per_step + i < dst.shape[0])
                def _():
                    col_copy(src, dst, it * per_step + i, sem_a).start()

        mem_cols = [mem[:, lanes(n)] for n in range(nk)]
        for u0 in range(0, STEP_UNROLL, 2):
            o = []
            for u in (u0, u0 + 1):
                mem_cols, o_first = segment(it * STEP_UNROLL + u, mem_cols, u > 0)
                o.append(o_first)
            rows = pl.ds(pl.multiple_of((it * STEP_UNROLL + u0) * 2, 4), 4)
            for hd in range(n_pair):
                a, b, c, d = (o[i][j] for i in range(2) for j in (hd, hd + n_pair))
                for i, t in enumerate(_lhs_terms(a, b, c, d)):
                    o_terms[i, hd, rows, :] = _to_words(jnp.concatenate([t, t], axis=0))[0:4]
        for n in range(nk):
            mem[:, lanes(n)] = mem_cols[n]
        return carry + 1

    steps = lax.fori_loop(0, n_step, step, 0)

    last_copy = out_copy(pl.ds(n_seg - STEP_UNROLL, STEP_UNROLL), rest, every_col, sem_a)
    first_copies = [out_copy(every_seg, first, pl.ds(0, dm - 2 * LANES), sem_a),
                    out_copy(every_seg, first, pl.ds(dm - 2 * LANES, 2 * LANES), sem_a)]

    def for_routed_segments(fn):
        segs = [idx_s[i] // seg for i in range(TOP_C)]
        for i, s in enumerate(segs):
            new = functools.reduce(jnp.logical_and, [s != t for t in segs[:i]], s < n_early)
            pl.when(new)(lambda: fn(out_copy(pl.ds(s, 1), rest, every_col, sem_b)))

    row = lax.broadcasted_iota(I32, (n_mem, dm), 0)

    def routed_ffn():
        keys = key_v[...]
        for i in range(TOP_C):
            best = jnp.max(keys)
            idx_s[i] = 65535 - (best & 65535)
            keys = jnp.where(keys == best, INT_MIN, keys)
        slot = lax.broadcasted_iota(I32, (2 * TOP_C, dm), 0)
        x_sel = jnp.zeros((2 * TOP_C, dm), F32)
        for i in range(TOP_C):
            t = idx_s[i]
            rows = pl.ds(pl.multiple_of(t & (seg - n_mem), n_mem), n_mem)
            picked = jnp.where(row == (t & (n_mem - 1)), x_v[t // seg, rows, :].astype(F32), 0.0)
            x_sel = jnp.where(slot == i, jnp.sum(picked, axis=0, keepdims=True), x_sel)
        r_sel = _sigmoid(row_dot(x_sel, wr_ref[...].astype(F32)))
        lhs = x_sel.astype(BF16)
        for _ in range(ROUTE_SLOTS):
            yield
        hidden = []
        for n in range(nf):
            gt = _dot(lhs, _as_bf16(wg_v[n]))
            yield
            up = _dot(lhs, _as_bf16(wu_v[n]))
            hidden.append((gt * _sigmoid(gt) * up).astype(BF16))
            yield
        y = [None] * nk
        for lo in range(0, nf, nk):
            hi = min(lo + nk, nf)
            lhs = jnp.concatenate(hidden[lo:hi], axis=1)
            for n in range(nk):
                part = _dot(lhs, _as_bf16(wd_v[n, lo * (LANES // 2):hi * (LANES // 2), :]))
                y[n] = part if y[n] is None else part + y[n]
                if (n + 1) * (hi - lo) % nk < hi - lo:
                    yield
        y = jnp.concatenate(y, axis=1) * r_sel
        for i in range(TOP_C):
            yield
            t = idx_s[i]
            s, r0 = t // seg, pl.multiple_of(t & (seg - n_mem), n_mem)
            rows = pl.ds(r0, n_mem)
            upd = jnp.where(row == (t & (n_mem - 1)), y[i:i + 1, :], 0.0)
            b = (x_v[s, rows, :].astype(F32) + upd).astype(BF16)
            x_v[s, rows, :] = b
            later = pl.ds(pl.multiple_of(jnp.maximum(r0, n_mem), n_mem), n_mem)
            gate, b = g_v[s, rows, :], b.astype(F32)
            for n in range(nk):
                a = a_v[s, rows if n < nk - 2 else later, lanes(n)]
                out_v[s, rows, lanes(n)] = _mix(gate, a, b[:, lanes(n)])
        yield
        first_copies[0].start()
        last_copy.start()
        for_routed_segments(lambda copy: copy.start())

    def out_first(u, filler):
        prods = []
        for i in range(7):
            acc = None
            for lo in range(0, n_pair, 4):
                lhs = jnp.concatenate(
                    [_as_bf16(o_terms[i, hd]) for hd in range(lo, lo + 4)], axis=1)

                def block(i, row, col):
                    r0 = row * (wo_v.shape[1] // 2) + lo * (LANES // 2)
                    return _as_bf16(
                        wo_v[2 * u + col + _opaque_zero(steps, i), r0:r0 + 2 * LANES, :])

                part = _dot(lhs, _rhs_term(i, block))
                acc = part if acc is None else part + acc
                next(filler, None)
            prods.append(acc)
        c = [t.reshape(n_seg // 2, 1, n_mem, LANES) for t in _combine(prods)]
        return [jnp.concatenate([c[j], c[j + 2]], axis=1).reshape(n_seg, n_mem, LANES)
                for j in range(2)]

    def mix_first(u, blocks):
        for n, a in enumerate(blocks, 2 * u):
            a_v[:, first, lanes(n)] = a
            out_v[:, first, lanes(n)] = _mix(
                g_v[:, first, :], a, x_v[:, first, lanes(n)].astype(F32))

    for w in (wg_v, wu_v, wd_v):
        wait_whole(w, sem_a)
    n_early = n_seg - STEP_UNROLL
    out_copy(pl.ds(0, n_early), rest, every_col, sem_b).wait()

    ffn = routed_ffn()
    for u in range(nk // 2):
        blocks = out_first(u, ffn)
        if u == nk // 2 - 1:
            for _ in ffn:
                pass
        mix_first(u, blocks)
    first_copies[1].start()
    for_routed_segments(lambda copy: copy.wait())
    for copy in first_copies + [last_copy]:
        copy.wait()


@functools.partial(jax.jit, static_argnames=("A_seg_len",))
def pallas_gated_mix__memory_aug_recurrent_mem_tr__moe_arch_mod__prompt_kernel(
    A_x, A_mem0, A_Wq, A_Wk, A_Wv, A_Wo, A_seg_len, B_x, B_w_r, B_w_gate, B_w_up,
    B_w_down, gate_w,
):
    del B_x
    batch, n_tok, dm = A_x.shape
    n_mem = A_mem0.shape[1]
    n_head, dh = A_Wq.shape[1:]
    d_ff = B_w_gate.shape[1]
    seg = int(A_seg_len)
    n_seg = n_tok // seg
    n_pair, nk, nf = n_head // 2, dm // LANES, d_ff // LANES
    assert (batch, n_mem, seg, dh) == (1, 8, 32, LANES)
    assert dm % (4 * LANES) == 0 and d_ff % LANES == 0 and n_pair % PRO_PAIRS == 0
    assert n_tok % (seg * STEP_UNROLL) == 0 and n_seg <= LANES
    assert nk % (n_pair // PRO_PAIRS) == 0
    assert ROUTE_SLOTS + 3 * nf > (nk // 2 - 1) * 7 * (n_pair // 4)

    hbm = pl.BlockSpec(memory_space=pl.ANY)
    out = pl.pallas_call(
        _kernel,
        out_shape=jax.ShapeDtypeStruct((n_seg, seg, dm), A_x.dtype),
        in_specs=[hbm] * 11,
        out_specs=hbm,
        scratch_shapes=[
            pltpu.VMEM((n_seg, seg, dm), BF16),
            pltpu.VMEM((7, nk // 2, n_seg * n_mem // 4, LANES), U32),
            pltpu.VMEM((3 * n_pair + 1, dm, LANES), U32),
            pltpu.VMEM((nk, n_head * dh // 2, LANES), U32),
            pltpu.VMEM((3 * n_pair, n_seg * n_mem, LANES), U32),
            pltpu.VMEM((7, n_pair, n_seg * n_mem // 4, LANES), U32),
            pltpu.VMEM((n_seg, seg, dm), F32),
            pltpu.VMEM((n_seg, seg, LANES), F32),
            pltpu.VMEM((n_mem, dm), F32),
            pltpu.VMEM((2 * (n_mem + seg), LANES), F32),
            pltpu.VMEM((seg, LANES), I32),
            pltpu.VMEM((n_mem, dm), BF16),
            pltpu.VMEM((nk, LANES), BF16),
            pltpu.VMEM((nk, LANES), BF16),
            pltpu.VMEM((nf, dm // 2, LANES), U32),
            pltpu.VMEM((nf, dm // 2, LANES), U32),
            pltpu.VMEM((nk, d_ff // 2, LANES), U32),
            pltpu.VMEM((n_seg, seg, dm), BF16),
            pltpu.SMEM((TOP_C,), I32),
            pltpu.SemaphoreType.DMA((4 + 3 * PRO_PAIRS,)),
        ],
        compiler_params=pltpu.CompilerParams(
            vmem_limit_bytes=116 * 1024 * 1024, disable_bounds_checks=True, flags=FLAGS),
        name="gated_mix_rmt_mod",
    )(
        A_x.reshape(n_seg, seg, dm), A_mem0.reshape(n_mem, dm), A_Wq, A_Wk, A_Wv,
        A_Wo.reshape(n_head * dh, dm), B_w_r.reshape(nk, LANES), B_w_gate, B_w_up, B_w_down,
        gate_w.reshape(nk, LANES),
    )
    return out.reshape(batch, n_tok, dm)
```

```python
import functools

import jax
import jax.numpy as jnp
import numpy as np
from jax import lax
from jax.experimental import pallas as pl
from jax.experimental.pallas import tpu as pltpu

BF16, F32, U32, I32 = jnp.bfloat16, jnp.float32, jnp.uint32, jnp.int32
LANES = 128
TOP_C = 8
INT_MIN = -(2 ** 31)
HI16 = np.uint32(0xFFFF0000)

FLAGS = {"XLA_TPU_EVENLY_DISTRIBUTE_CRITICAL_NODES": True}
N_DEEP = 4
STEP_UNROLL = 2
QKV_ORDER = (1, 0, 2)
QK_LAG, PV_LAG = 3, 10
QK_START, PV_START = 0, 4
EARLY_HEADS = 24
ROUTE_SLOTS = 8
EARLY_HALVES = 6


def _dot(a, b):
    return jnp.dot(a, b, preferred_element_type=F32)


def _as_bf16(words):
    return pltpu.bitcast(words, BF16)


def _to_words(v):
    return pltpu.bitcast(v.astype(BF16), U32)


def _split_words(words):
    return pltpu.bitcast(words << 16, F32), pltpu.bitcast(words & HI16, F32)


def _sigmoid(v):
    return 1.0 / (1.0 + jnp.exp(-v))


def _mix(gate, a, b):
    return (gate * a + (1.0 - gate) * b).astype(BF16)


def _lhs_terms(a, b, c, d):
    return [c + d, a, a + b, d, a + d, c - a, b - d]


RHS_TERMS = (((0, 0),), ((0, 1), jnp.subtract, (1, 1)), ((1, 1),), ((1, 0), jnp.subtract, (0, 0)),
             ((0, 0), jnp.add, (1, 1)), ((0, 0), jnp.add, (0, 1)), ((1, 0), jnp.add, (1, 1)))


def _rhs_term(i, block):
    term = RHS_TERMS[i]
    if len(term) == 1:
        return block(*term[0])
    return term[1](block(*term[0]).astype(F32), block(*term[2]).astype(F32))


def _opaque_zero(count, i):
    return count >> (16 + i)


def _combine(m):
    return [m[3] - m[2] + m[4] + m[6], m[1] + m[2], m[0] + m[3], m[1] - m[0] + m[4] + m[5]]


def _score_fill(n_mem, seg):
    shape = (2 * (n_mem + seg), LANES)

    def decode(i):
        tail = i >= 2 * seg
        head = jnp.where(tail, (i - 2 * seg) >> 3, i >> 5)
        r = i & (seg - 1)
        pos = jnp.where(tail, n_mem + (i & 7), jnp.where(r < n_mem, r, r + n_mem))
        return head, pos

    rh, rp = decode(lax.broadcasted_iota(I32, shape, 0))
    ch, cp = decode(lax.broadcasted_iota(I32, shape, 1))
    visible = (rp < n_mem) | (rp >= cp)
    return jnp.where(rh == ch, jnp.where(visible, 0.0, -1e9), -jnp.inf).astype(F32)


def _kernel(x_hbm, mem0_hbm, wq_hbm, wk_hbm, wv_hbm, wo_hbm, wr_hbm, wg_hbm, wu_hbm,
            wd_hbm, gw_hbm, out_hbm,
            x_v, x_terms, x_terms2, wqkv, wo_v, qkv0, o_terms, a_v, g_v, mem, fill_v, key_v,
            mem0_ref, wr_ref, gw_ref, wg_v, wu_v, wd_v, out_v, idx_s,
            sems):
    n_seg, seg, dm = x_v.shape
    n_mem = mem.shape[0]
    n_pair = wqkv.shape[0] // 3
    n_head = 2 * n_pair
    nk = dm // LANES
    nf = wg_v.shape[0]
    scale = LANES ** -0.5
    w_hbm = (wq_hbm, wk_hbm, wv_hbm)
    first, rest = pl.ds(0, n_mem), pl.ds(n_mem, seg - n_mem)

    def lanes(n):
        return slice(n * LANES, (n + 1) * LANES)

    sem_a, sem_b = sems.at[0], sems.at[1]

    def slot_of(m, quad, j):
        return 6 * quad + 2 * m + j

    def w_copy(m, quad, j, sem):
        return pltpu.make_async_copy(
            w_hbm[m].bitcast(U32).at[:, 2 * quad + j, :], wqkv.at[slot_of(m, quad, j)], sem)

    def col_copy(src, dst, n, sem):
        start = n * LANES if isinstance(n, int) else pl.multiple_of(n * LANES, LANES)
        cols = pl.ds(start, LANES)
        return pltpu.make_async_copy(src.bitcast(U32).at[:, cols], dst.at[n], sem)

    def wait_whole(dst, sem):
        pltpu.make_async_copy(dst, dst, sem).wait()

    x_first = pltpu.make_async_copy(x_hbm.at[:, first, :], x_v.at[:, first, :], sem_a)
    x_rest = pltpu.make_async_copy(x_hbm.at[:, rest, :], x_v.at[:, rest, :], sem_b)

    units = [(m, j) for m in range(3) for j in range(2)]
    small = [pltpu.make_async_copy(src, dst, sem_b)
             for src, dst in ((mem0_hbm, mem0_ref), (wr_hbm, wr_ref), (gw_hbm, gw_ref))]

    def group_sem(it):
        return sems.at[2 + (it & 1)]

    x_first.start()
    for m, j in units:
        w_copy(m, 0, j, sems.at[4 + m]).start()
    for m, j in units:
        w_copy(m, 1, j, group_sem(1)).start()

    fill_v[...] = _score_fill(n_mem, seg)
    key_v[...] = jnp.full(key_v.shape, INT_MIN, I32)
    spare = 3 * n_pair
    wqkv[spare:spare + 2] = jnp.zeros((2, dm, LANES), U32)

    quarter = n_seg * n_mem // 4
    x_first.wait()
    for n in range(nk // 4):
        x0 = [x_v[:, 0:n_mem, lanes(n + k * nk // 4)].astype(F32).reshape(2, 2, quarter, LANES)
              for k in range(4)]
        terms = [_lhs_terms(x0[k][0], x0[k + 2][0], x0[k][1], x0[k + 2][1]) for k in range(2)]
        for j in range(7):
            left, right = terms[0][j], terms[1][j]
            if j < N_DEEP:
                for i, t in enumerate(_lhs_terms(left[0], right[0], left[1], right[1])):
                    x_terms2[7 * j + i, n] = _to_words(t)
            else:
                for k, t in enumerate((left, right)):
                    x_terms[j - N_DEEP, n + k * nk // 4] = _to_words(t.reshape(-1, LANES))

    def regroup(w, piece, n_piece):
        groups = dm // 16
        for r in range(groups * piece // n_piece * 16, groups * (piece + 1) // n_piece * 16, 16):
            even = wqkv[w, pl.ds(r, 8, stride=2), :]
            odd = wqkv[w, pl.ds(r + 1, 8, stride=2), :]
            wqkv[w, r:r + 8, :] = (even & np.uint32(0xFFFF)) | (odd << 16)
            wqkv[w, r + 8:r + 16, :] = (even >> 16) | (odd & HI16)

    def project_first(w, previous):
        def rhs_term(j, head, r0, rn, tag):
            def block(row, pair):
                rows = slice(row * (dm // 2) + r0, row * (dm // 2) + r0 + rn)
                return _split_words(wqkv[w + pair + _opaque_zero(w, tag), rows, :])[head]
            return _rhs_term(j, block)

        def small_product(j, i):
            lhs = jnp.concatenate(
                [_as_bf16(x_terms2[7 * j + i, n]) for n in range(nk // 4)], axis=1)
            rhs = _rhs_term(i, lambda row, head: rhs_term(j, head, row * (dm // 4), dm // 4, i))
            return _dot(lhs, rhs.astype(BF16))

        def large_product(j, head):
            lhs = jnp.concatenate(
                [_as_bf16(x_terms[j - N_DEEP, n]) for n in range(nk // 2)], axis=1)
            return _dot(lhs, rhs_term(j, head, 0, dm // 2, 2 * j + head).astype(BF16))

        cheap = [(j, i) for j in range(N_DEEP) if len(RHS_TERMS[j]) == 1 for i in range(7)]
        dear = [(j, i) for j in range(N_DEEP) if len(RHS_TERMS[j]) > 1 for i in range(7)]
        large = [(j, head) for j in range(N_DEEP, 7) for head in range(2)]
        order = [cheap[k:k + 2] for k in range(0, len(cheap), 2)]
        dear = [dear[k:k + 2] for k in range(0, len(dear), 2)]
        for k, at in enumerate(large):
            order += dear[len(dear) * k // len(large):len(dear) * (k + 1) // len(large)] + [[at]]
        prods, n_piece = {}, len(order) // 2
        for k, group in enumerate(order):
            for j, i in group:
                prods[j, i] = small_product(j, i) if j < N_DEEP else large_product(j, i)
            if k < 2 * n_piece:
                regroup(previous + k // n_piece, k % n_piece, n_piece)
        blocks = [_combine([prods[j, i] for i in range(7)]) for j in range(N_DEEP)]
        blocks += [[prods[j, head][q * quarter:(q + 1) * quarter]
                    for q in range(2) for head in range(2)] for j in range(N_DEEP, 7)]
        for q in range(2):
            both = zip(*(_combine([b[2 * q + head] for b in blocks]) for head in range(2)))
            for i, heads in enumerate(both):
                rows = jnp.concatenate([t.reshape(-1, n_mem, LANES) for t in heads], axis=1)
                r0 = (2 * (i // 2) + q) * quarter
                qkv0[w + i % 2, r0:r0 + quarter, :] = _to_words(rows.reshape(-1, LANES))

    n_pro = n_pair // 2
    wo_per_it = nk // n_pro

    def ramp(m, carry):
        wait_whole(wqkv.at[pl.ds(2 * m, 2)], sems.at[4 + m])
        project_first(2 * m, jnp.where(m > 0, 2 * m - 2, spare))
        return carry

    lax.fori_loop(0, 3, ramp, 0)
    for copy in small:
        copy.start()
    for n in range(wo_per_it):
        col_copy(wo_hbm, wo_v, n, sem_b).start()

    def prologue(it, carry):
        @pl.when(it + 1 < n_pro)
        def _():
            for m, j in units:
                w_copy(m, it + 1, j, group_sem(it + 1)).start()

        for n in range(wo_per_it):
            col_copy(wo_hbm, wo_v, it * wo_per_it + n, sem_b).start()

        @pl.when(it == n_pro // 2)
        def _():
            x_rest.start()

        wait_whole(wqkv.at[pl.ds(slot_of(0, it, 0), len(units))], group_sem(it))
        for m in range(3):
            project_first(slot_of(m, it, 0), slot_of(m, it, 0) - 2)
        return carry

    lax.fori_loop(1, n_pro, prologue, 0)

    for w in (spare - 2, spare - 1):
        regroup(w, 0, 1)
    x_rest.wait()
    wait_whole(wo_v, sem_b)
    for copy in small:
        copy.wait()
    mem[...] = mem0_ref[...].astype(F32)

    def row_dot(rows, w):
        acc = rows[:, lanes(0)] * w[0:1, :]
        for n in range(1, nk):
            acc = acc + rows[:, lanes(n)] * w[n:n + 1, :]
        return jnp.sum(acc, axis=-1, keepdims=True)

    def head_weights(m, hd, lo, hi):
        w = wqkv[slot_of(m, hd // 4, hd // 2 % 2), lo * LANES:hi * LANES, :]
        w = w.reshape(-1, 2, 8, LANES)
        return _as_bf16(w[:, hd % 2].reshape(-1, LANES))

    def segment(s, mem_cols, mem_is_late):
        xs = x_v[s]
        xf = xs.astype(F32)
        h_cols = [
            jnp.concatenate(
                [jnp.concatenate([mem_cols[n], xf[n_mem:2 * n_mem, lanes(n)]], axis=0).astype(BF16),
                 xs[2 * n_mem:, lanes(n)]], axis=0)
            for n in range(nk)]
        rows0 = pl.ds(pl.multiple_of(s * n_mem, n_mem), n_mem)
        pad = jnp.zeros((LANES - 2 * (seg + n_mem), LANES), F32)

        def partial_proj(m, hd, lo, hi):
            return _dot(jnp.concatenate(h_cols[lo:hi], axis=1), head_weights(m, hd, lo, hi))

        slots = [(m, 2 * p + j) for p in range(n_pair) for m in QKV_ORDER for j in range(2)]
        early = {}
        if mem_is_late:
            for m, hd in slots[:EARLY_HALVES]:
                early[m, hd] = partial_proj(m, hd, 0, nk // 2)

        def project(m, hd):
            if (m, hd) in early:
                return partial_proj(m, hd, nk // 2, nk) + early[m, hd]
            return partial_proj(m, hd, 0, nk)

        def both_heads(m, p):
            rows = [res[m, 2 * p], res[m, 2 * p + 1],
                    _as_bf16(qkv0[slot_of(m, p // 2, p % 2), rows0, :]).astype(F32)]
            return jnp.concatenate(rows + [pad] * (m > 0), axis=0).astype(BF16)

        def probabilities(q, k):
            sc = lax.dot_general(q, k, (((1,), (1,)), ((), ())), preferred_element_type=F32)
            fill = fill_v[...]
            sc = jnp.where(fill == 0.0, sc * scale, fill)
            e = jnp.exp(sc - jnp.max(sc, axis=-1, keepdims=True))
            den = jnp.sum(e, axis=-1, keepdims=True)
            inv = pl.reciprocal(den, approx=True)
            inv = inv * (2.0 - den * inv)
            return (e * inv).astype(BF16)

        def out_proj(lo, hi, n):
            lhs = jnp.concatenate([heads[i] for i in range(lo, hi)], axis=1)
            return _dot(lhs, _as_bf16(wo_v[n, lo * (LANES // 2):hi * (LANES // 2), :]))

        slots += [(3 + j, n) for n in range(nk) for j in range(2)]
        res, prob, heads, o_first = {}, {}, {}, {}
        for i, (m, j) in enumerate(slots):
            if m < 3:
                res[m, j] = project(m, j)
            elif m == 3:
                res[3, j] = out_proj(0, EARLY_HEADS // 2, j)
            else:
                res[3, j] = out_proj(EARLY_HEADS // 2, EARLY_HEADS, j) + res[3, j]
            for p in range(n_pair):
                ready = [slots.index((t, 2 * p + 1)) for t in range(3)]
                qk_at = max(ready[:2]) + QK_LAG
                pv_at = qk_at + PV_LAG
                if not mem_is_late:
                    qk_at += max(QK_START - 2 * p, 0)
                    pv_at += max(QK_START - 2 * p, 0) + max(PV_START - 2 * p, 0)
                if i == qk_at:
                    prob[p] = probabilities(both_heads(0, p), both_heads(1, p))
                if i == min(max(pv_at, ready[2] + 2), len(slots) - 1):
                    o = _dot(prob[p], both_heads(2, p))
                    ob = o[0:2 * seg].astype(BF16)
                    heads[2 * p], heads[2 * p + 1] = ob[0:seg], ob[seg:]
                    o_first[2 * p] = o[2 * seg:2 * seg + n_mem]
                    o_first[2 * p + 1] = o[2 * seg + n_mem:]
        gate = jnp.broadcast_to(_sigmoid(row_dot(xf, gw_ref[...].astype(F32))), (seg, LANES))
        g_v[s] = gate
        new_mem = []
        for n in range(nk):
            r = out_proj(EARLY_HEADS, n_head, n) + res[3, n]
            new_mem.append(r[0:n_mem])
            a_v[s, rest, lanes(n)] = r[n_mem:]
            out_v[s, rest, lanes(n)] = _mix(gate[n_mem:], r[n_mem:], xf[n_mem:, lanes(n)])

        score = row_dot(xf, wr_ref[...].astype(F32)).astype(BF16).astype(F32)
        score = jnp.broadcast_to(score, (seg, LANES))
        bits = pltpu.bitcast(jnp.where(score == 0.0, 0.0, score), I32)
        order = jnp.where(bits < 0, bits ^ np.int32(0x7FFFFFFF), bits)
        order = jnp.where(score != score, INT_MIN, order)
        token = s * seg + lax.broadcasted_iota(I32, (seg, LANES), 0)
        key = (order & np.int32(-65536)) | (65535 - token)
        lane = lax.broadcasted_iota(I32, (seg, LANES), 1)
        key_v[...] = jnp.where(lane == s, key, key_v[...])
        return new_mem, o_first

    n_step = n_seg // STEP_UNROLL

    def out_copy(segs, rows, cols, sem):
        return pltpu.make_async_copy(
            out_v.at[segs, rows, cols], out_hbm.at[segs, rows, cols], sem)

    every_seg, every_col = pl.ds(0, n_seg), pl.ds(0, dm)
    def step(it, carry):
        @pl.when(it > 0)
        def _():
            done = pl.ds((it - 1) * STEP_UNROLL, STEP_UNROLL)
            out_copy(done, rest, every_col, sem_b).start()

        for dst, src in ((wg_v, wg_hbm), (wu_v, wu_hbm), (wd_v, wd_hbm)):
            per_step = pl.cdiv(dst.shape[0], n_step)
            for i in range(per_step):
                @pl.when(it * per_step + i < dst.shape[0])
                def _():
                    col_copy(src, dst, it * per_step + i, sem_a).start()

        mem_cols = [mem[:, lanes(n)] for n in range(nk)]
        for u0 in range(0, STEP_UNROLL, 2):
            o = []
            for u in (u0, u0 + 1):
                mem_cols, o_first = segment(it * STEP_UNROLL + u, mem_cols, u > 0)
                o.append(o_first)
            rows = pl.ds(pl.multiple_of((it * STEP_UNROLL + u0) * 2, 4), 4)
            for hd in range(n_pair):
                a, b, c, d = (o[i][j] for i in range(2) for j in (hd, hd + n_pair))
                for i, t in enumerate(_lhs_terms(a, b, c, d)):
                    o_terms[i, hd, rows, :] = _to_words(jnp.concatenate([t, t], axis=0))[0:4]
        for n in range(nk):
            mem[:, lanes(n)] = mem_cols[n]
        return carry + 1

    steps = lax.fori_loop(0, n_step, step, 0)

    last_copy = out_copy(pl.ds(n_seg - STEP_UNROLL, STEP_UNROLL), rest, every_col, sem_a)
    first_copies = [out_copy(every_seg, first, pl.ds(0, dm - 2 * LANES), sem_a),
                    out_copy(every_seg, first, pl.ds(dm - 2 * LANES, 2 * LANES), sem_a)]

    def for_routed_segments(fn):
        segs = [idx_s[i] // seg for i in range(TOP_C)]
        for i, s in enumerate(segs):
            new = functools.reduce(jnp.logical_and, [s != t for t in segs[:i]], s < n_early)
            pl.when(new)(lambda: fn(out_copy(pl.ds(s, 1), rest, every_col, sem_b)))

    row = lax.broadcasted_iota(I32, (n_mem, dm), 0)

    def routed_ffn():
        keys = key_v[...]
        for i in range(TOP_C):
            best = jnp.max(keys)
            idx_s[i] = 65535 - (best & 65535)
            keys = jnp.where(keys == best, INT_MIN, keys)
        slot = lax.broadcasted_iota(I32, (2 * TOP_C, dm), 0)
        x_sel = jnp.zeros((2 * TOP_C, dm), F32)
        for i in range(TOP_C):
            t = idx_s[i]
            rows = pl.ds(pl.multiple_of(t & (seg - n_mem), n_mem), n_mem)
            picked = jnp.where(row == (t & (n_mem - 1)), x_v[t // seg, rows, :].astype(F32), 0.0)
            x_sel = jnp.where(slot == i, jnp.sum(picked, axis=0, keepdims=True), x_sel)
        r_sel = _sigmoid(row_dot(x_sel, wr_ref[...].astype(F32)))
        lhs = x_sel.astype(BF16)
        for _ in range(ROUTE_SLOTS):
            yield
        hidden = []
        for n in range(nf):
            gt = _dot(lhs, _as_bf16(wg_v[n]))
            yield
            up = _dot(lhs, _as_bf16(wu_v[n]))
            hidden.append((gt * _sigmoid(gt) * up).astype(BF16))
            yield
        y = [None] * nk
        for lo in range(0, nf, nk):
            hi = min(lo + nk, nf)
            lhs = jnp.concatenate(hidden[lo:hi], axis=1)
            for n in range(nk):
                part = _dot(lhs, _as_bf16(wd_v[n, lo * (LANES // 2):hi * (LANES // 2), :]))
                y[n] = part if y[n] is None else part + y[n]
                if (n + 1) * (hi - lo) % nk < hi - lo:
                    yield
        y = jnp.concatenate(y, axis=1) * r_sel
        for i in range(TOP_C):
            yield
            t = idx_s[i]
            s, r0 = t // seg, pl.multiple_of(t & (seg - n_mem), n_mem)
            rows = pl.ds(r0, n_mem)
            upd = jnp.where(row == (t & (n_mem - 1)), y[i:i + 1, :], 0.0)
            b = (x_v[s, rows, :].astype(F32) + upd).astype(BF16)
            x_v[s, rows, :] = b
            later = pl.ds(pl.multiple_of(jnp.maximum(r0, n_mem), n_mem), n_mem)
            gate, b = g_v[s, rows, :], b.astype(F32)
            for n in range(nk):
                a = a_v[s, rows if n < nk - 2 else later, lanes(n)]
                out_v[s, rows, lanes(n)] = _mix(gate, a, b[:, lanes(n)])
        yield
        first_copies[0].start()
        last_copy.start()
        for_routed_segments(lambda copy: copy.start())

    def out_first(u, filler):
        prods = []
        for i in range(7):
            acc = None
            for lo in range(0, n_pair, 4):
                lhs = jnp.concatenate(
                    [_as_bf16(o_terms[i, hd]) for hd in range(lo, lo + 4)], axis=1)

                def block(row, col):
                    r0 = row * (wo_v.shape[1] // 2) + lo * (LANES // 2)
                    return _as_bf16(
                        wo_v[2 * u + col + _opaque_zero(steps, i), r0:r0 + 2 * LANES, :])

                part = _dot(lhs, _rhs_term(i, block).astype(BF16))
                acc = part if acc is None else part + acc
                next(filler, None)
            prods.append(acc)
        c = [t.reshape(n_seg // 2, 1, n_mem, LANES) for t in _combine(prods)]
        return [jnp.concatenate([c[j], c[j + 2]], axis=1).reshape(n_seg, n_mem, LANES)
                for j in range(2)]

    def mix_first(u, blocks):
        for n, a in enumerate(blocks, 2 * u):
            a_v[:, first, lanes(n)] = a
            out_v[:, first, lanes(n)] = _mix(
                g_v[:, first, :], a, x_v[:, first, lanes(n)].astype(F32))

    for w in (wg_v, wu_v, wd_v):
        wait_whole(w, sem_a)
    n_early = n_seg - STEP_UNROLL
    out_copy(pl.ds(0, n_early), rest, every_col, sem_b).wait()

    ffn = routed_ffn()
    for u in range(nk // 2):
        blocks = out_first(u, ffn)
        if u == nk // 2 - 1:
            for _ in ffn:
                pass
        mix_first(u, blocks)
    first_copies[1].start()
    for_routed_segments(lambda copy: copy.wait())
    for copy in first_copies + [last_copy]:
        copy.wait()


@functools.partial(jax.jit, static_argnames=("A_seg_len",))
def pallas_gated_mix__memory_aug_recurrent_mem_tr__moe_arch_mod__prompt_kernel(
    A_x, A_mem0, A_Wq, A_Wk, A_Wv, A_Wo, A_seg_len, B_x, B_w_r, B_w_gate, B_w_up,
    B_w_down, gate_w,
):
    del B_x
    batch, n_tok, dm = A_x.shape
    n_mem = A_mem0.shape[1]
    n_head, dh = A_Wq.shape[1:]
    d_ff = B_w_gate.shape[1]
    seg = int(A_seg_len)
    n_seg = n_tok // seg
    n_pair, nk, nf = n_head // 2, dm // LANES, d_ff // LANES
    assert (batch, n_mem, seg, dh) == (1, 8, 32, LANES)
    assert dm % (4 * LANES) == 0 and d_ff % LANES == 0 and n_pair % 4 == 0
    assert n_tok % (8 * seg) == 0 and n_seg <= LANES
    assert nk % (n_pair // 2) == 0
    assert ROUTE_SLOTS + 3 * nf > (nk // 2 - 1) * 7 * (n_pair // 4)

    hbm = pl.BlockSpec(memory_space=pl.ANY)
    out = pl.pallas_call(
        _kernel,
        out_shape=jax.ShapeDtypeStruct((n_seg, seg, dm), A_x.dtype),
        in_specs=[hbm] * 11,
        out_specs=hbm,
        scratch_shapes=[
            pltpu.VMEM((n_seg, seg, dm), BF16),
            pltpu.VMEM((7 - N_DEEP, nk // 2, n_seg * n_mem // 4, LANES), U32),
            pltpu.VMEM((7 * N_DEEP, nk // 4, n_seg * n_mem // 8, LANES), U32),
            pltpu.VMEM((3 * n_pair + 2, dm, LANES), U32),
            pltpu.VMEM((nk, n_head * dh // 2, LANES), U32),
            pltpu.VMEM((3 * n_pair, n_seg * n_mem, LANES), U32),
            pltpu.VMEM((7, n_pair, n_seg * n_mem // 4, LANES), U32),
            pltpu.VMEM((n_seg, seg, dm), F32),
            pltpu.VMEM((n_seg, seg, LANES), F32),
            pltpu.VMEM((n_mem, dm), F32),
            pltpu.VMEM((2 * (n_mem + seg), LANES), F32),
            pltpu.VMEM((seg, LANES), I32),
            pltpu.VMEM((n_mem, dm), BF16),
            pltpu.VMEM((nk, LANES), BF16),
            pltpu.VMEM((nk, LANES), BF16),
            pltpu.VMEM((nf, dm // 2, LANES), U32),
            pltpu.VMEM((nf, dm // 2, LANES), U32),
            pltpu.VMEM((nk, d_ff // 2, LANES), U32),
            pltpu.VMEM((n_seg, seg, dm), BF16),
            pltpu.SMEM((TOP_C,), I32),
            pltpu.SemaphoreType.DMA((7,)),
        ],
        compiler_params=pltpu.CompilerParams(
            vmem_limit_bytes=116 * 1024 * 1024, disable_bounds_checks=True, flags=FLAGS),
        name="gated_mix_rmt_mod",
    )(
        A_x.reshape(n_seg, seg, dm), A_mem0.reshape(n_mem, dm), A_Wq, A_Wk, A_Wv,
        A_Wo.reshape(n_head * dh, dm), B_w_r.reshape(nk, LANES), B_w_gate, B_w_up, B_w_down,
        gate_w.reshape(nk, LANES),
    )
    return out.reshape(batch, n_tok, dm)
```

```python
import functools

import jax
import jax.numpy as jnp
import numpy as np
from jax import lax
from jax.experimental import pallas as pl
from jax.experimental.pallas import tpu as pltpu

BF16, F32, U32, I32 = jnp.bfloat16, jnp.float32, jnp.uint32, jnp.int32
LANES = 128
TOP_C = 8
INT_MIN = -(2 ** 31)
HI16 = np.uint32(0xFFFF0000)

N_DEEP = 4
STEP_UNROLL = 2
QKV_ORDER = (1, 0, 2)
QK_LAG, PV_LAG = 3, 11
QK_START, PV_START = 0, 2
EARLY_HEADS = 16
ROUTE_SLOTS = 8
EARLY_HALVES = 6


def _dot(a, b):
    return jnp.dot(a, b, preferred_element_type=F32)


def _as_bf16(words):
    return pltpu.bitcast(words, BF16)


def _to_words(v):
    return pltpu.bitcast(v.astype(BF16), U32)


def _split_words(words):
    return pltpu.bitcast(words << 16, F32), pltpu.bitcast(words & HI16, F32)


def _sigmoid(v):
    return 1.0 / (1.0 + jnp.exp(-v))


def _mix(gate, a, b):
    return (gate * a + (1.0 - gate) * b).astype(BF16)


def _lhs_terms(a, b, c, d):
    return [c + d, a, a + b, d, a + d, c - a, b - d]


RHS_TERMS = (((0, 0),), ((0, 1), jnp.subtract, (1, 1)), ((1, 1),), ((1, 0), jnp.subtract, (0, 0)),
             ((0, 0), jnp.add, (1, 1)), ((0, 0), jnp.add, (0, 1)), ((1, 0), jnp.add, (1, 1)))


def _rhs_term(i, block):
    term = RHS_TERMS[i]
    if len(term) == 1:
        return block(*term[0])
    return term[1](block(*term[0]).astype(F32), block(*term[2]).astype(F32))


def _opaque_zero(count, i):
    return count >> (16 + i)


def _combine(m):
    return [m[3] - m[2] + m[4] + m[6], m[1] + m[2], m[0] + m[3], m[1] - m[0] + m[4] + m[5]]


def _score_fill(n_mem, seg):
    shape = (2 * (n_mem + seg), LANES)

    def decode(i):
        tail = i >= 2 * seg
        head = jnp.where(tail, (i - 2 * seg) >> 3, i >> 5)
        r = i & (seg - 1)
        pos = jnp.where(tail, n_mem + (i & 7), jnp.where(r < n_mem, r, r + n_mem))
        return head, pos

    rh, rp = decode(lax.broadcasted_iota(I32, shape, 0))
    ch, cp = decode(lax.broadcasted_iota(I32, shape, 1))
    visible = (rp < n_mem) | (rp >= cp)
    return jnp.where(rh == ch, jnp.where(visible, 0.0, -1e9), -jnp.inf).astype(F32)


def _kernel(x_hbm, mem0_hbm, wq_hbm, wk_hbm, wv_hbm, wo_hbm, wr_hbm, wg_hbm, wu_hbm,
            wd_hbm, gw_hbm, out_hbm,
            x_v, x_terms, x_terms2, wqkv, wo_v, qkv0, o_terms, a_v, g_v, mem, fill_v, key_v,
            mem0_ref, wr_ref, gw_ref, wg_v, wu_v, wd_v, out_v, idx_s,
            sems):
    n_seg, seg, dm = x_v.shape
    n_mem = mem.shape[0]
    n_pair = wqkv.shape[0] // 3
    n_head = 2 * n_pair
    nk = dm // LANES
    nf = wg_v.shape[0]
    scale = LANES ** -0.5
    w_hbm = (wq_hbm, wk_hbm, wv_hbm)
    first, rest = pl.ds(0, n_mem), pl.ds(n_mem, seg - n_mem)

    def lanes(n):
        return slice(n * LANES, (n + 1) * LANES)

    sem_a, sem_b = sems.at[0], sems.at[1]

    def slot_of(m, quad, j):
        return 6 * quad + 2 * m + j

    def w_copy(m, quad, j, sem):
        return pltpu.make_async_copy(
            w_hbm[m].bitcast(U32).at[:, 2 * quad + j, :], wqkv.at[slot_of(m, quad, j)], sem)

    def col_copy(src, dst, n, sem):
        start = n * LANES if isinstance(n, int) else pl.multiple_of(n * LANES, LANES)
        cols = pl.ds(start, LANES)
        return pltpu.make_async_copy(src.bitcast(U32).at[:, cols], dst.at[n], sem)

    def wait_whole(dst, sem):
        pltpu.make_async_copy(dst, dst, sem).wait()

    x_first = pltpu.make_async_copy(x_hbm.at[:, first, :], x_v.at[:, first, :], sem_a)
    x_rest = pltpu.make_async_copy(x_hbm.at[:, rest, :], x_v.at[:, rest, :], sem_b)

    units = [(m, j) for m in range(3) for j in range(2)]
    small = [pltpu.make_async_copy(src, dst, sem_b)
             for src, dst in ((mem0_hbm, mem0_ref), (wr_hbm, wr_ref), (gw_hbm, gw_ref))]

    def group_sem(it):
        return sems.at[2 + (it & 1)]

    x_first.start()
    for m, j in units:
        w_copy(m, 0, j, sems.at[4 + m]).start()
    for m, j in units:
        w_copy(m, 1, j, group_sem(1)).start()

    fill_v[...] = _score_fill(n_mem, seg)
    key_v[...] = jnp.full(key_v.shape, INT_MIN, I32)
    spare = 3 * n_pair
    wqkv[spare:spare + 2] = jnp.zeros((2, dm, LANES), U32)

    quarter = n_seg * n_mem // 4
    x_first.wait()
    for n in range(nk // 4):
        x0 = [x_v[:, 0:n_mem, lanes(n + k * nk // 4)].astype(F32).reshape(2, 2, quarter, LANES)
              for k in range(4)]
        terms = [_lhs_terms(x0[k][0], x0[k + 2][0], x0[k][1], x0[k + 2][1]) for k in range(2)]
        for j in range(7):
            left, right = terms[0][j], terms[1][j]
            if j < N_DEEP:
                for i, t in enumerate(_lhs_terms(left[0], right[0], left[1], right[1])):
                    x_terms2[7 * j + i, n] = _to_words(t)
            else:
                for k, t in enumerate((left, right)):
                    x_terms[j - N_DEEP, n + k * nk // 4] = _to_words(t.reshape(-1, LANES))

    def regroup(w, piece, n_piece):
        groups = dm // 16
        for r in range(groups * piece // n_piece * 16, groups * (piece + 1) // n_piece * 16, 16):
            even = wqkv[w, pl.ds(r, 8, stride=2), :]
            odd = wqkv[w, pl.ds(r + 1, 8, stride=2), :]
            wqkv[w, r:r + 8, :] = (even & np.uint32(0xFFFF)) | (odd << 16)
            wqkv[w, r + 8:r + 16, :] = (even >> 16) | (odd & HI16)

    def project_first(w, previous):
        def rhs_term(j, head, r0, rn, tag):
            def block(row, pair):
                rows = slice(row * (dm // 2) + r0, row * (dm // 2) + r0 + rn)
                return _split_words(wqkv[w + pair + _opaque_zero(w, tag), rows, :])[head]
            return _rhs_term(j, block)

        def small_product(j, i):
            lhs = jnp.concatenate(
                [_as_bf16(x_terms2[7 * j + i, n]) for n in range(nk // 4)], axis=1)
            rhs = _rhs_term(i, lambda row, head: rhs_term(j, head, row * (dm // 4), dm // 4, i))
            return _dot(lhs, rhs.astype(BF16))

        def large_product(j, head):
            lhs = jnp.concatenate(
                [_as_bf16(x_terms[j - N_DEEP, n]) for n in range(nk // 2)], axis=1)
            return _dot(lhs, rhs_term(j, head, 0, dm // 2, 2 * j + head).astype(BF16))

        def cost(at):
            return len(RHS_TERMS[at[0]]) * len(RHS_TERMS[at[1]])

        small = [(j, i) for j in range(N_DEEP) for i in range(7)]
        cheap = [at for at in small if cost(at) < 9]
        dear = [at for at in small if cost(at) == 9]
        large = [(j, head) for j in range(N_DEEP, 7) for head in range(2)]
        order, dear = ([t[k:k + 2] for k in range(0, len(t), 2)] for t in (cheap, dear))
        for k, at in enumerate(large):
            order += [[at]] + dear[k:k + 1]
        order += dear[len(large):]
        prods, n_piece = {}, len(order) // 2
        for k, group in enumerate(order):
            for j, i in group:
                prods[j, i] = small_product(j, i) if j < N_DEEP else large_product(j, i)
            if k < 2 * n_piece:
                regroup(previous + k // n_piece, k % n_piece, n_piece)
        blocks = [_combine([prods[j, i] for i in range(7)]) for j in range(N_DEEP)]
        blocks += [[prods[j, head][q * quarter:(q + 1) * quarter]
                    for q in range(2) for head in range(2)] for j in range(N_DEEP, 7)]
        for q in range(2):
            for head in range(2):
                for i, t in enumerate(_combine([b[2 * q + head] for b in blocks])):
                    segs = pl.ds((2 * (i // 2) + q) * (n_seg // 4), n_seg // 4)
                    qkv0[w >> 1, segs, 2 * (i % 2) + head] = t.reshape(-1, n_mem, LANES)

    n_pro = n_pair // 2
    wo_per_it = nk // n_pro

    def ramp(m, carry):
        wait_whole(wqkv.at[pl.ds(2 * m, 2)], sems.at[4 + m])
        project_first(2 * m, jnp.where(m > 0, 2 * m - 2, spare))
        return carry

    lax.fori_loop(0, 3, ramp, 0)
    for copy in small:
        copy.start()
    for n in range(wo_per_it):
        col_copy(wo_hbm, wo_v, n, sem_b).start()

    def prologue(it, carry):
        @pl.when(it + 1 < n_pro)
        def _():
            for m, j in units:
                w_copy(m, it + 1, j, group_sem(it + 1)).start()

        for n in range(wo_per_it):
            col_copy(wo_hbm, wo_v, it * wo_per_it + n, sem_b).start()

        @pl.when(it + 1 == n_pro)
        def _():
            x_rest.start()

        wait_whole(wqkv.at[pl.ds(slot_of(0, it, 0), len(units))], group_sem(it))
        for m in range(3):
            project_first(slot_of(m, it, 0), slot_of(m, it, 0) - 2)
        return carry

    lax.fori_loop(1, n_pro, prologue, 0)

    for w in (spare - 2, spare - 1):
        regroup(w, 0, 1)
    x_rest.wait()
    wait_whole(wo_v, sem_b)
    for copy in small:
        copy.wait()
    mem[...] = mem0_ref[...].astype(F32)

    def row_dot(rows, w):
        acc = rows[:, lanes(0)] * w[0:1, :]
        for n in range(1, nk):
            acc = acc + rows[:, lanes(n)] * w[n:n + 1, :]
        return jnp.sum(acc, axis=-1, keepdims=True)

    def head_weights(m, hd, lo, hi):
        w = wqkv[slot_of(m, hd // 4, hd // 2 % 2), lo * LANES:hi * LANES, :]
        w = w.reshape(-1, 2, 8, LANES)
        return _as_bf16(w[:, hd % 2].reshape(-1, LANES))

    def segment(s, mem_cols, mem_is_late):
        xs = x_v[s]
        xf = xs.astype(F32)
        h_cols = [
            jnp.concatenate(
                [jnp.concatenate([mem_cols[n], xf[n_mem:2 * n_mem, lanes(n)]], axis=0).astype(BF16),
                 xs[2 * n_mem:, lanes(n)]], axis=0)
            for n in range(nk)]
        pad = jnp.zeros((LANES - 2 * (seg + n_mem), LANES), F32)

        def partial_proj(m, hd, lo, hi):
            return _dot(jnp.concatenate(h_cols[lo:hi], axis=1), head_weights(m, hd, lo, hi))

        slots = [(m, 2 * p + j) for p in range(n_pair) for m in QKV_ORDER for j in range(2)]
        early = {}
        if mem_is_late:
            for m, hd in slots[:EARLY_HALVES]:
                early[m, hd] = partial_proj(m, hd, 0, nk // 2)

        def project(m, hd):
            if (m, hd) in early:
                return partial_proj(m, hd, nk // 2, nk) + early[m, hd]
            return partial_proj(m, hd, 0, nk)

        def both_heads(m, p):
            rows = [res[m, 2 * p], res[m, 2 * p + 1]]
            rows += [qkv0[3 * (p // 2) + m, s, 2 * (p % 2) + j] for j in range(2)]
            return jnp.concatenate(rows + [pad] * (m > 0), axis=0).astype(BF16)

        def probabilities(q, k):
            sc = lax.dot_general(q, k, (((1,), (1,)), ((), ())), preferred_element_type=F32)
            fill = fill_v[...]
            sc = jnp.where(fill == 0.0, sc * scale, fill)
            e = jnp.exp(sc - jnp.max(sc, axis=-1, keepdims=True))
            den = jnp.sum(e, axis=-1, keepdims=True)
            inv = pl.reciprocal(den, approx=True)
            inv = inv * (2.0 - den * inv)
            return (e * inv).astype(BF16)

        def out_proj(lo, hi, n):
            lhs = jnp.concatenate([heads[i] for i in range(lo, hi)], axis=1)
            return _dot(lhs, _as_bf16(wo_v[n, lo * (LANES // 2):hi * (LANES // 2), :]))

        slots += [(3 + j, n) for n in range(nk) for j in range(2)]
        res, prob, heads, o_first = {}, {}, {}, {}
        for i, (m, j) in enumerate(slots):
            if m < 3:
                res[m, j] = project(m, j)
            elif m == 3:
                res[3, j] = out_proj(0, EARLY_HEADS // 2, j)
            else:
                res[3, j] = out_proj(EARLY_HEADS // 2, EARLY_HEADS, j) + res[3, j]
            for p in range(n_pair):
                ready = [slots.index((t, 2 * p + 1)) for t in range(3)]
                qk_at = max(ready[:2]) + QK_LAG
                pv_at = qk_at + PV_LAG
                if not mem_is_late:
                    qk_at += max(QK_START - 2 * p, 0)
                    pv_at += max(QK_START - 2 * p, 0) + max(PV_START - 2 * p, 0)
                if i == qk_at:
                    prob[p] = probabilities(both_heads(0, p), both_heads(1, p))
                if i == min(max(pv_at, ready[2] + 2), len(slots) - 1):
                    o = _dot(prob[p], both_heads(2, p))
                    ob = o[0:2 * seg].astype(BF16)
                    heads[2 * p], heads[2 * p + 1] = ob[0:seg], ob[seg:]
                    o_first[2 * p] = o[2 * seg:2 * seg + n_mem]
                    o_first[2 * p + 1] = o[2 * seg + n_mem:]
        gate = jnp.broadcast_to(_sigmoid(row_dot(xf, gw_ref[...].astype(F32))), (seg, LANES))
        g_v[s] = gate
        new_mem = []
        for n in range(nk):
            r = out_proj(EARLY_HEADS, n_head, n) + res[3, n]
            new_mem.append(r[0:n_mem])
            a_v[s, rest, lanes(n)] = r[n_mem:]
            out_v[s, rest, lanes(n)] = _mix(gate[n_mem:], r[n_mem:], xf[n_mem:, lanes(n)])

        score = row_dot(xf, wr_ref[...].astype(F32)).astype(BF16).astype(F32)
        score = jnp.broadcast_to(score, (seg, LANES))
        bits = pltpu.bitcast(jnp.where(score == 0.0, 0.0, score), I32)
        order = jnp.where(bits < 0, bits ^ np.int32(0x7FFFFFFF), bits)
        order = jnp.where(score != score, INT_MIN, order)
        token = s * seg + lax.broadcasted_iota(I32, (seg, LANES), 0)
        key = (order & np.int32(-65536)) | (65535 - token)
        lane = lax.broadcasted_iota(I32, (seg, LANES), 1)
        key_v[...] = jnp.where(lane == s, key, key_v[...])
        return new_mem, o_first

    n_step = n_seg // STEP_UNROLL

    def out_copy(segs, rows, cols, sem):
        return pltpu.make_async_copy(
            out_v.at[segs, rows, cols], out_hbm.at[segs, rows, cols], sem)

    every_seg, every_col = pl.ds(0, n_seg), pl.ds(0, dm)
    def step(it, carry):
        @pl.when(it > 0)
        def _():
            done = pl.ds((it - 1) * STEP_UNROLL, STEP_UNROLL)
            out_copy(done, rest, every_col, sem_b).start()

        for dst, src in ((wg_v, wg_hbm), (wu_v, wu_hbm), (wd_v, wd_hbm)):
            per_step = pl.cdiv(dst.shape[0], n_step)
            for i in range(per_step):
                @pl.when(it * per_step + i < dst.shape[0])
                def _():
                    col_copy(src, dst, it * per_step + i, sem_a).start()

        mem_cols = [mem[:, lanes(n)] for n in range(nk)]
        for u0 in range(0, STEP_UNROLL, 2):
            o = []
            for u in (u0, u0 + 1):
                mem_cols, o_first = segment(it * STEP_UNROLL + u, mem_cols, u > 0)
                o.append(o_first)
            s0 = it * STEP_UNROLL + u0
            rows = pl.ds(pl.multiple_of((s0 & 2) * 2, 4), 4)
            for hd in range(n_pair):
                a, b, c, d = (o[i][j] for i in range(2) for j in (hd, hd + n_pair))
                for i, t in enumerate(_lhs_terms(a, b, c, d)):
                    o_terms[s0 >> 2, i, hd, rows, :] = _to_words(jnp.concatenate([t, t], axis=0))[0:4]
        for n in range(nk):
            mem[:, lanes(n)] = mem_cols[n]
        return carry + 1

    steps = lax.fori_loop(0, n_step, step, 0)

    last_copy = out_copy(pl.ds(n_seg - STEP_UNROLL, STEP_UNROLL), rest, every_col, sem_a)
    first_copies = [out_copy(every_seg, first, pl.ds(0, dm - 2 * LANES), sem_a),
                    out_copy(every_seg, first, pl.ds(dm - 2 * LANES, 2 * LANES), sem_a)]

    def for_routed_segments(fn):
        segs = [idx_s[i] // seg for i in range(TOP_C)]
        for i, s in enumerate(segs):
            new = functools.reduce(jnp.logical_and, [s != t for t in segs[:i]], s < n_early)
            pl.when(new)(lambda: fn(out_copy(pl.ds(s, 1), rest, every_col, sem_b)))

    row = lax.broadcasted_iota(I32, (n_mem, dm), 0)

    def routed_ffn():
        keys = key_v[...]
        for i in range(TOP_C):
            best = jnp.max(keys)
            idx_s[i] = 65535 - (best & 65535)
            keys = jnp.where(keys == best, INT_MIN, keys)
        slot = lax.broadcasted_iota(I32, (2 * TOP_C, dm), 0)
        x_sel = jnp.zeros((2 * TOP_C, dm), F32)
        for i in range(TOP_C):
            t = idx_s[i]
            rows = pl.ds(pl.multiple_of(t & (seg - n_mem), n_mem), n_mem)
            picked = jnp.where(row == (t & (n_mem - 1)), x_v[t // seg, rows, :].astype(F32), 0.0)
            x_sel = jnp.where(slot == i, jnp.sum(picked, axis=0, keepdims=True), x_sel)
        r_sel = _sigmoid(row_dot(x_sel, wr_ref[...].astype(F32)))
        lhs = x_sel.astype(BF16)
        for _ in range(ROUTE_SLOTS):
            yield
        hidden = []
        for n in range(nf):
            gt = _dot(lhs, _as_bf16(wg_v[n]))
            yield
            up = _dot(lhs, _as_bf16(wu_v[n]))
            hidden.append((gt * _sigmoid(gt) * up).astype(BF16))
            yield
        y = [None] * nk
        for lo in range(0, nf, nk):
            hi = min(lo + nk, nf)
            lhs = jnp.concatenate(hidden[lo:hi], axis=1)
            for n in range(nk):
                part = _dot(lhs, _as_bf16(wd_v[n, lo * (LANES // 2):hi * (LANES // 2), :]))
                y[n] = part if y[n] is None else part + y[n]
                if (n + 1) * (hi - lo) % nk < hi - lo:
                    yield
        y = jnp.concatenate(y, axis=1) * r_sel
        for i in range(TOP_C):
            yield
            t = idx_s[i]
            s, r0 = t // seg, pl.multiple_of(t & (seg - n_mem), n_mem)
            rows = pl.ds(r0, n_mem)
            upd = jnp.where(row == (t & (n_mem - 1)), y[i:i + 1, :], 0.0)
            b = (x_v[s, rows, :].astype(F32) + upd).astype(BF16)
            x_v[s, rows, :] = b
            later = pl.ds(pl.multiple_of(jnp.maximum(r0, n_mem), n_mem), n_mem)
            gate, b = g_v[s, rows, :], b.astype(F32)
            for n in range(nk):
                a = a_v[s, rows if n < nk - 2 else later, lanes(n)]
                out_v[s, rows, lanes(n)] = _mix(gate, a, b[:, lanes(n)])
        yield
        first_copies[0].start()
        last_copy.start()
        for_routed_segments(lambda copy: copy.start())

    def out_first(u, filler):
        prods = []
        for i in range(7):
            acc = None
            for lo in range(0, n_pair, 4):
                lhs = jnp.concatenate(
                    [_as_bf16(o_terms[:, i, hd].reshape(-1, LANES)) for hd in range(lo, lo + 4)],
                    axis=1)

                def block(row, col):
                    r0 = row * (wo_v.shape[1] // 2) + lo * (LANES // 2)
                    return _as_bf16(
                        wo_v[2 * u + col + _opaque_zero(steps, i), r0:r0 + 2 * LANES, :])

                part = _dot(lhs, _rhs_term(i, block).astype(BF16))
                acc = part if acc is None else part + acc
                next(filler, None)
            prods.append(acc)
        c = [t.reshape(n_seg // 2, 1, n_mem, LANES) for t in _combine(prods)]
        return [jnp.concatenate([c[j], c[j + 2]], axis=1).reshape(n_seg, n_mem, LANES)
                for j in range(2)]

    def mix_first(u, blocks):
        for n, a in enumerate(blocks, 2 * u):
            a_v[:, first, lanes(n)] = a
            out_v[:, first, lanes(n)] = _mix(
                g_v[:, first, :], a, x_v[:, first, lanes(n)].astype(F32))

    for w in (wg_v, wu_v, wd_v):
        wait_whole(w, sem_a)
    n_early = n_seg - STEP_UNROLL
    out_copy(pl.ds(0, n_early), rest, every_col, sem_b).wait()

    ffn = routed_ffn()
    for u in range(nk // 2):
        blocks = out_first(u, ffn)
        if u == nk // 2 - 1:
            for _ in ffn:
                pass
        mix_first(u, blocks)
    first_copies[1].start()
    for_routed_segments(lambda copy: copy.wait())
    for copy in first_copies + [last_copy]:
        copy.wait()


@functools.partial(jax.jit, static_argnames=("A_seg_len",))
def pallas_gated_mix__memory_aug_recurrent_mem_tr__moe_arch_mod__prompt_kernel(
    A_x, A_mem0, A_Wq, A_Wk, A_Wv, A_Wo, A_seg_len, B_x, B_w_r, B_w_gate, B_w_up,
    B_w_down, gate_w,
):
    del B_x
    batch, n_tok, dm = A_x.shape
    n_mem = A_mem0.shape[1]
    n_head, dh = A_Wq.shape[1:]
    d_ff = B_w_gate.shape[1]
    seg = int(A_seg_len)
    n_seg = n_tok // seg
    n_pair, nk, nf = n_head // 2, dm // LANES, d_ff // LANES
    assert (batch, n_mem, seg, dh) == (1, 8, 32, LANES)
    assert dm % (4 * LANES) == 0 and d_ff % LANES == 0 and n_pair % 4 == 0
    assert n_tok % (8 * seg) == 0 and n_seg <= LANES
    assert nk % (n_pair // 2) == 0
    assert ROUTE_SLOTS + 3 * nf > (nk // 2 - 1) * 7 * (n_pair // 4)

    hbm = pl.BlockSpec(memory_space=pl.ANY)
    out = pl.pallas_call(
        _kernel,
        out_shape=jax.ShapeDtypeStruct((n_seg, seg, dm), A_x.dtype),
        in_specs=[hbm] * 11,
        out_specs=hbm,
        scratch_shapes=[
            pltpu.VMEM((n_seg, seg, dm), BF16),
            pltpu.VMEM((7 - N_DEEP, nk // 2, n_seg * n_mem // 4, LANES), U32),
            pltpu.VMEM((7 * N_DEEP, nk // 4, n_seg * n_mem // 8, LANES), U32),
            pltpu.VMEM((3 * n_pair + 2, dm, LANES), U32),
            pltpu.VMEM((nk, n_head * dh // 2, LANES), U32),
            pltpu.VMEM((3 * n_pair // 2, n_seg, 4, n_mem, LANES), F32),
            pltpu.VMEM((n_seg // 4, 7, n_pair, 8, LANES), U32),
            pltpu.VMEM((n_seg, seg, dm), F32),
            pltpu.VMEM((n_seg, seg, LANES), F32),
            pltpu.VMEM((n_mem, dm), F32),
            pltpu.VMEM((2 * (n_mem + seg), LANES), F32),
            pltpu.VMEM((seg, LANES), I32),
            pltpu.VMEM((n_mem, dm), BF16),
            pltpu.VMEM((nk, LANES), BF16),
            pltpu.VMEM((nk, LANES), BF16),
            pltpu.VMEM((nf, dm // 2, LANES), U32),
            pltpu.VMEM((nf, dm // 2, LANES), U32),
            pltpu.VMEM((nk, d_ff // 2, LANES), U32),
            pltpu.VMEM((n_seg, seg, dm), BF16),
            pltpu.SMEM((TOP_C,), I32),
            pltpu.SemaphoreType.DMA((7,)),
        ],
        compiler_params=pltpu.CompilerParams(
            vmem_limit_bytes=116 * 1024 * 1024, disable_bounds_checks=True),
        name="gated_mix_rmt_mod",
    )(
        A_x.reshape(n_seg, seg, dm), A_mem0.reshape(n_mem, dm), A_Wq, A_Wk, A_Wv,
        A_Wo.reshape(n_head * dh, dm), B_w_r.reshape(nk, LANES), B_w_gate, B_w_up, B_w_down,
        gate_w.reshape(nk, LANES),
    )
    return out.reshape(batch, n_tok, dm)
```

```python
import functools

import jax
import jax.numpy as jnp
import numpy as np
from jax import lax
from jax.experimental import pallas as pl
from jax.experimental.pallas import tpu as pltpu

BF16, F32, U32, I32 = jnp.bfloat16, jnp.float32, jnp.uint32, jnp.int32
LANES = 128
TOP_C = 8
INT_MIN = -(2 ** 31)
HI16 = np.uint32(0xFFFF0000)

RAW = 2
N_DEEP = 4
STEP_UNROLL = 2
QKV_ORDER = (1, 0, 2)
QK_LAG, PV_LAG = 3, 11
QK_START, PV_START = 0, 2
EARLY_HEADS = 16
ROUTE_SLOTS = 8
EARLY_HALVES = 6


def _dot(a, b):
    return jnp.dot(a, b, preferred_element_type=F32)


def _as_bf16(words):
    return pltpu.bitcast(words, BF16)


def _to_words(v):
    return pltpu.bitcast(v.astype(BF16), U32)


def _split_words(words):
    return pltpu.bitcast(words << 16, F32), pltpu.bitcast(words & HI16, F32)


def _sigmoid(v):
    return 1.0 / (1.0 + jnp.exp(-v))


def _mix(gate, a, b):
    return (gate * a + (1.0 - gate) * b).astype(BF16)


def _lhs_terms(a, b, c, d):
    return [c + d, a, a + b, d, a + d, c - a, b - d]


RHS_TERMS = (((0, 0),), ((0, 1), jnp.subtract, (1, 1)), ((1, 1),), ((1, 0), jnp.subtract, (0, 0)),
             ((0, 0), jnp.add, (1, 1)), ((0, 0), jnp.add, (0, 1)), ((1, 0), jnp.add, (1, 1)))


def _rhs_term(i, block):
    term = RHS_TERMS[i]
    if len(term) == 1:
        return block(*term[0])
    return term[1](block(*term[0]).astype(F32), block(*term[2]).astype(F32))


def _opaque_zero(count, i):
    return count >> (16 + i)


def _combine(m):
    return [m[3] - m[2] + m[4] + m[6], m[1] + m[2], m[0] + m[3], m[1] - m[0] + m[4] + m[5]]


def _score_fill(n_mem, seg):
    shape = (2 * (n_mem + seg), LANES)

    def decode(i):
        tail = i >= 2 * seg
        head = jnp.where(tail, (i - 2 * seg) >> 3, i >> 5)
        r = i & (seg - 1)
        pos = jnp.where(tail, n_mem + (i & 7), jnp.where(r < n_mem, r, r + n_mem))
        return head, pos

    rh, rp = decode(lax.broadcasted_iota(I32, shape, 0))
    ch, cp = decode(lax.broadcasted_iota(I32, shape, 1))
    visible = (rp < n_mem) | (rp >= cp)
    return jnp.where(rh == ch, jnp.where(visible, 0.0, -1e9), -jnp.inf).astype(F32)


def _kernel(x_hbm, mem0_hbm, wq_hbm, wk_hbm, wv_hbm, wo_hbm, wr_hbm, wg_hbm, wu_hbm,
            wd_hbm, gw_hbm, out_hbm,
            x_v, x_terms, x_terms2, wqkv, wo_v, qkv0, o_terms, a_v, g_v, mem, fill_v, key_v,
            mem0_ref, wr_ref, gw_ref, wg_v, wu_v, wd_v, out_v, idx_s,
            sems):
    n_seg, seg, dm = x_v.shape
    n_mem = mem.shape[0]
    n_pair = wqkv.shape[0] // 3
    n_head = 2 * n_pair
    nk = dm // LANES
    nf = wg_v.shape[0]
    scale = LANES ** -0.5
    w_hbm = (wq_hbm, wk_hbm, wv_hbm)
    first, rest = pl.ds(0, n_mem), pl.ds(n_mem, seg - n_mem)

    def lanes(n):
        return slice(n * LANES, (n + 1) * LANES)

    sem_a, sem_b = sems.at[0], sems.at[1]

    def slot_of(m, quad, j):
        return 6 * quad + 2 * m + j

    def w_copy(m, quad, j, sem):
        return pltpu.make_async_copy(
            w_hbm[m].bitcast(U32).at[:, 2 * quad + j, :], wqkv.at[slot_of(m, quad, j) + RAW], sem)

    def col_copy(src, dst, n, sem):
        start = n * LANES if isinstance(n, int) else pl.multiple_of(n * LANES, LANES)
        cols = pl.ds(start, LANES)
        return pltpu.make_async_copy(src.bitcast(U32).at[:, cols], dst.at[n], sem)

    def wait_whole(dst, sem):
        pltpu.make_async_copy(dst, dst, sem).wait()

    x_first = pltpu.make_async_copy(x_hbm.at[:, first, :], x_v.at[:, first, :], sem_a)
    x_rest = pltpu.make_async_copy(x_hbm.at[:, rest, :], x_v.at[:, rest, :], sem_b)

    units = [(m, j) for m in range(3) for j in range(2)]
    small = [pltpu.make_async_copy(src, dst, sem_b)
             for src, dst in ((mem0_hbm, mem0_ref), (wr_hbm, wr_ref), (gw_hbm, gw_ref))]

    def group_sem(it):
        return sems.at[2 + (it & 1)]

    x_first.start()
    for m, j in units:
        w_copy(m, 0, j, sems.at[4 + m]).start()
    for m, j in units:
        w_copy(m, 1, j, group_sem(1)).start()

    fill_v[...] = _score_fill(n_mem, seg)
    key_v[...] = jnp.full(key_v.shape, INT_MIN, I32)

    quarter = n_seg * n_mem // 4
    x_first.wait()
    for n in range(nk // 4):
        x0 = [x_v[:, 0:n_mem, lanes(n + k * nk // 4)].astype(F32).reshape(2, 2, quarter, LANES)
              for k in range(4)]
        terms = [_lhs_terms(x0[k][0], x0[k + 2][0], x0[k][1], x0[k + 2][1]) for k in range(2)]
        for j in range(7):
            left, right = terms[0][j], terms[1][j]
            if j < N_DEEP:
                for i, t in enumerate(_lhs_terms(left[0], right[0], left[1], right[1])):
                    x_terms2[7 * j + i, n] = _to_words(t)
            else:
                for k, t in enumerate((left, right)):
                    x_terms[j - N_DEEP, n + k * nk // 4] = _to_words(t.reshape(-1, LANES))

    def regroup(w, piece, n_piece):
        groups = dm // 16
        for r in range(groups * piece // n_piece * 16, groups * (piece + 1) // n_piece * 16, 16):
            even = wqkv[w + RAW, pl.ds(r, 8, stride=2), :]
            odd = wqkv[w + RAW, pl.ds(r + 1, 8, stride=2), :]
            wqkv[w, r:r + 8, :] = (even & np.uint32(0xFFFF)) | (odd << 16)
            wqkv[w, r + 8:r + 16, :] = (even >> 16) | (odd & HI16)

    def project_first(w):
        def rhs_term(j, head, r0, rn, tag):
            def block(row, pair):
                rows = slice(row * (dm // 2) + r0, row * (dm // 2) + r0 + rn)
                words = wqkv[w + RAW + pair + _opaque_zero(w, tag), rows, :]
                return _split_words(words)[head]
            return _rhs_term(j, block)

        def small_product(j, i):
            lhs = jnp.concatenate(
                [_as_bf16(x_terms2[7 * j + i, n]) for n in range(nk // 4)], axis=1)
            rhs = _rhs_term(i, lambda row, head: rhs_term(j, head, row * (dm // 4), dm // 4, i))
            return _dot(lhs, rhs.astype(BF16))

        def large_product(j, head):
            lhs = jnp.concatenate(
                [_as_bf16(x_terms[j - N_DEEP, n]) for n in range(nk // 2)], axis=1)
            return _dot(lhs, rhs_term(j, head, 0, dm // 2, 2 * j + head).astype(BF16))

        def cost(at):
            return len(RHS_TERMS[at[0]]) * len(RHS_TERMS[at[1]])

        small = [(j, i) for j in range(N_DEEP) for i in range(7)]
        cheap = [at for at in small if cost(at) < 9]
        dear = [at for at in small if cost(at) == 9]
        large = [(j, head) for j in range(N_DEEP, 7) for head in range(2)]
        order, dear = ([t[k:k + 2] for k in range(0, len(t), 2)] for t in (cheap, dear))
        for k, at in enumerate(large):
            order += [[at]] + dear[k:k + 1]
        order += dear[len(large):]
        prods, n_piece = {}, len(order) // 2
        for k, group in enumerate(order):
            for j, i in group:
                prods[j, i] = small_product(j, i) if j < N_DEEP else large_product(j, i)
            if k < 2 * n_piece:
                regroup(w + k // n_piece, k % n_piece, n_piece)
        blocks = [_combine([prods[j, i] for i in range(7)]) for j in range(N_DEEP)]
        blocks += [[prods[j, head][q * quarter:(q + 1) * quarter]
                    for q in range(2) for head in range(2)] for j in range(N_DEEP, 7)]
        for q in range(2):
            for head in range(2):
                for i, t in enumerate(_combine([b[2 * q + head] for b in blocks])):
                    segs = pl.ds((2 * (i // 2) + q) * (n_seg // 4), n_seg // 4)
                    qkv0[w >> 1, segs, 2 * (i % 2) + head] = t.reshape(-1, n_mem, LANES)

    n_pro = n_pair // 2
    wo_per_it = nk // n_pro

    def ramp(m, carry):
        wait_whole(wqkv.at[pl.ds(2 * m + RAW, 2)], sems.at[4 + m])
        project_first(2 * m)
        return carry

    lax.fori_loop(0, 3, ramp, 0)
    for copy in small:
        copy.start()
    for n in range(wo_per_it):
        col_copy(wo_hbm, wo_v, n, sem_b).start()

    def prologue(it, carry):
        @pl.when(it + 1 < n_pro)
        def _():
            for m, j in units:
                w_copy(m, it + 1, j, group_sem(it + 1)).start()

        for n in range(wo_per_it):
            col_copy(wo_hbm, wo_v, it * wo_per_it + n, sem_b).start()

        @pl.when(it + 1 == n_pro)
        def _():
            x_rest.start()

        wait_whole(wqkv.at[pl.ds(slot_of(0, it, 0) + RAW, len(units))], group_sem(it))
        for m in range(3):
            project_first(slot_of(m, it, 0))
        return carry

    lax.fori_loop(1, n_pro, prologue, 0)

    x_rest.wait()
    wait_whole(wo_v, sem_b)
    for copy in small:
        copy.wait()
    mem[...] = mem0_ref[...].astype(F32)

    def row_dot(rows, w):
        acc = rows[:, lanes(0)] * w[0:1, :]
        for n in range(1, nk):
            acc = acc + rows[:, lanes(n)] * w[n:n + 1, :]
        return jnp.sum(acc, axis=-1, keepdims=True)

    def head_weights(m, hd, lo, hi):
        w = wqkv[slot_of(m, hd // 4, hd // 2 % 2), lo * LANES:hi * LANES, :]
        w = w.reshape(-1, 2, 8, LANES)
        return _as_bf16(w[:, hd % 2].reshape(-1, LANES))

    def segment(s, mem_cols, mem_is_late):
        xs = x_v[s]
        xf = xs.astype(F32)
        h_cols = [
            jnp.concatenate(
                [jnp.concatenate([mem_cols[n], xf[n_mem:2 * n_mem, lanes(n)]], axis=0).astype(BF16),
                 xs[2 * n_mem:, lanes(n)]], axis=0)
            for n in range(nk)]
        pad = jnp.zeros((LANES - 2 * (seg + n_mem), LANES), F32)

        def partial_proj(m, hd, lo, hi):
            return _dot(jnp.concatenate(h_cols[lo:hi], axis=1), head_weights(m, hd, lo, hi))

        slots = [(m, 2 * p + j) for p in range(n_pair) for m in QKV_ORDER for j in range(2)]
        early = {}
        if mem_is_late:
            for m, hd in slots[:EARLY_HALVES]:
                early[m, hd] = partial_proj(m, hd, 0, nk // 2)

        def project(m, hd):
            if (m, hd) in early:
                return partial_proj(m, hd, nk // 2, nk) + early[m, hd]
            return partial_proj(m, hd, 0, nk)

        def both_heads(m, p):
            rows = [res[m, 2 * p], res[m, 2 * p + 1]]
            rows += [qkv0[3 * (p // 2) + m, s, 2 * (p % 2) + j] for j in range(2)]
            return jnp.concatenate(rows + [pad] * (m > 0), axis=0).astype(BF16)

        def probabilities(q, k):
            sc = lax.dot_general(q, k, (((1,), (1,)), ((), ())), preferred_element_type=F32)
            fill = fill_v[...]
            sc = jnp.where(fill == 0.0, sc * scale, fill)
            e = jnp.exp(sc - jnp.max(sc, axis=-1, keepdims=True))
            den = jnp.sum(e, axis=-1, keepdims=True)
            inv = pl.reciprocal(den, approx=True)
            inv = inv * (2.0 - den * inv)
            return (e * inv).astype(BF16)

        def out_proj(lo, hi, n):
            lhs = jnp.concatenate([heads[i] for i in range(lo, hi)], axis=1)
            return _dot(lhs, _as_bf16(wo_v[n, lo * (LANES // 2):hi * (LANES // 2), :]))

        slots += [(3 + j, n) for n in range(nk) for j in range(2)]
        res, prob, heads, o_first = {}, {}, {}, {}
        for i, (m, j) in enumerate(slots):
            if m < 3:
                res[m, j] = project(m, j)
            elif m == 3:
                res[3, j] = out_proj(0, EARLY_HEADS // 2, j)
            else:
                res[3, j] = out_proj(EARLY_HEADS // 2, EARLY_HEADS, j) + res[3, j]
            for p in range(n_pair):
                ready = [slots.index((t, 2 * p + 1)) for t in range(3)]
                qk_at = max(ready[:2]) + QK_LAG
                pv_at = qk_at + PV_LAG
                if not mem_is_late:
                    qk_at += max(QK_START - 2 * p, 0)
                    pv_at += max(QK_START - 2 * p, 0) + max(PV_START - 2 * p, 0)
                if i == qk_at:
                    prob[p] = probabilities(both_heads(0, p), both_heads(1, p))
                if i == min(max(pv_at, ready[2] + 2), len(slots) - 1):
                    o = _dot(prob[p], both_heads(2, p))
                    ob = o[0:2 * seg].astype(BF16)
                    heads[2 * p], heads[2 * p + 1] = ob[0:seg], ob[seg:]
                    o_first[2 * p] = o[2 * seg:2 * seg + n_mem]
                    o_first[2 * p + 1] = o[2 * seg + n_mem:]
        gate = jnp.broadcast_to(_sigmoid(row_dot(xf, gw_ref[...].astype(F32))), (seg, LANES))
        g_v[s] = gate
        new_mem = []
        for n in range(nk):
            r = out_proj(EARLY_HEADS, n_head, n) + res[3, n]
            new_mem.append(r[0:n_mem])
            a_v[s, rest, lanes(n)] = r[n_mem:]
            out_v[s, rest, lanes(n)] = _mix(gate[n_mem:], r[n_mem:], xf[n_mem:, lanes(n)])

        score = row_dot(xf, wr_ref[...].astype(F32)).astype(BF16).astype(F32)
        score = jnp.broadcast_to(score, (seg, LANES))
        bits = pltpu.bitcast(jnp.where(score == 0.0, 0.0, score), I32)
        order = jnp.where(bits < 0, bits ^ np.int32(0x7FFFFFFF), bits)
        order = jnp.where(score != score, INT_MIN, order)
        token = s * seg + lax.broadcasted_iota(I32, (seg, LANES), 0)
        key = (order & np.int32(-65536)) | (65535 - token)
        lane = lax.broadcasted_iota(I32, (seg, LANES), 1)
        key_v[...] = jnp.where(lane == s, key, key_v[...])
        return new_mem, o_first

    n_step = n_seg // STEP_UNROLL

    def out_copy(segs, rows, cols, sem):
        return pltpu.make_async_copy(
            out_v.at[segs, rows, cols], out_hbm.at[segs, rows, cols], sem)

    every_seg, every_col = pl.ds(0, n_seg), pl.ds(0, dm)
    def step(it, carry):
        @pl.when(it > 0)
        def _():
            done = pl.ds((it - 1) * STEP_UNROLL, STEP_UNROLL)
            out_copy(done, rest, every_col, sem_b).start()

        for dst, src in ((wg_v, wg_hbm), (wu_v, wu_hbm), (wd_v, wd_hbm)):
            per_step = pl.cdiv(dst.shape[0], n_step)
            for i in range(per_step):
                @pl.when(it * per_step + i < dst.shape[0])
                def _():
                    col_copy(src, dst, it * per_step + i, sem_a).start()

        mem_cols = [mem[:, lanes(n)] for n in range(nk)]
        for u0 in range(0, STEP_UNROLL, 2):
            o = []
            for u in (u0, u0 + 1):
                mem_cols, o_first = segment(it * STEP_UNROLL + u, mem_cols, u > 0)
                o.append(o_first)
            s0 = it * STEP_UNROLL + u0
            rows = pl.ds(pl.multiple_of((s0 & 2) * 2, 4), 4)
            for hd in range(n_pair):
                a, b, c, d = (o[i][j] for i in range(2) for j in (hd, hd + n_pair))
                for i, t in enumerate(_lhs_terms(a, b, c, d)):
                    o_terms[s0 >> 2, i, hd, rows, :] = _to_words(jnp.concatenate([t, t], axis=0))[0:4]
        for n in range(nk):
            mem[:, lanes(n)] = mem_cols[n]
        return carry + 1

    steps = lax.fori_loop(0, n_step, step, 0)

    last_copy = out_copy(pl.ds(n_seg - STEP_UNROLL, STEP_UNROLL), rest, every_col, sem_a)
    first_copies = [out_copy(every_seg, first, pl.ds(0, dm - 2 * LANES), sem_a),
                    out_copy(every_seg, first, pl.ds(dm - 2 * LANES, 2 * LANES), sem_a)]

    def for_routed_segments(fn):
        segs = [idx_s[i] // seg for i in range(TOP_C)]
        for i, s in enumerate(segs):
            new = functools.reduce(jnp.logical_and, [s != t for t in segs[:i]], s < n_early)
            pl.when(new)(lambda: fn(out_copy(pl.ds(s, 1), rest, every_col, sem_b)))

    row = lax.broadcasted_iota(I32, (n_mem, dm), 0)

    def routed_ffn():
        keys = key_v[...]
        for i in range(TOP_C):
            best = jnp.max(keys)
            idx_s[i] = 65535 - (best & 65535)
            keys = jnp.where(keys == best, INT_MIN, keys)
        slot = lax.broadcasted_iota(I32, (2 * TOP_C, dm), 0)
        x_sel = jnp.zeros((2 * TOP_C, dm), F32)
        for i in range(TOP_C):
            t = idx_s[i]
            rows = pl.ds(pl.multiple_of(t & (seg - n_mem), n_mem), n_mem)
            picked = jnp.where(row == (t & (n_mem - 1)), x_v[t // seg, rows, :].astype(F32), 0.0)
            x_sel = jnp.where(slot == i, jnp.sum(picked, axis=0, keepdims=True), x_sel)
        r_sel = _sigmoid(row_dot(x_sel, wr_ref[...].astype(F32)))
        lhs = x_sel.astype(BF16)
        for _ in range(ROUTE_SLOTS):
            yield
        hidden = []
        for n in range(nf):
            gt = _dot(lhs, _as_bf16(wg_v[n]))
            yield
            up = _dot(lhs, _as_bf16(wu_v[n]))
            hidden.append((gt * _sigmoid(gt) * up).astype(BF16))
            yield
        y = [None] * nk
        for lo in range(0, nf, nk):
            hi = min(lo + nk, nf)
            lhs = jnp.concatenate(hidden[lo:hi], axis=1)
            for n in range(nk):
                part = _dot(lhs, _as_bf16(wd_v[n, lo * (LANES // 2):hi * (LANES // 2), :]))
                y[n] = part if y[n] is None else part + y[n]
                if (n + 1) * (hi - lo) % nk < hi - lo:
                    yield
        y = jnp.concatenate(y, axis=1) * r_sel
        for i in range(TOP_C):
            yield
            t = idx_s[i]
            s, r0 = t // seg, pl.multiple_of(t & (seg - n_mem), n_mem)
            rows = pl.ds(r0, n_mem)
            upd = jnp.where(row == (t & (n_mem - 1)), y[i:i + 1, :], 0.0)
            b = (x_v[s, rows, :].astype(F32) + upd).astype(BF16)
            x_v[s, rows, :] = b
            later = pl.ds(pl.multiple_of(jnp.maximum(r0, n_mem), n_mem), n_mem)
            gate, b = g_v[s, rows, :], b.astype(F32)
            for n in range(nk):
                a = a_v[s, rows if n < nk - 2 else later, lanes(n)]
                out_v[s, rows, lanes(n)] = _mix(gate, a, b[:, lanes(n)])
        yield
        first_copies[0].start()
        last_copy.start()
        for_routed_segments(lambda copy: copy.start())

    def out_first(u, filler):
        prods = []
        for i in range(7):
            acc = None
            for lo in range(0, n_pair, 4):
                lhs = jnp.concatenate(
                    [_as_bf16(o_terms[:, i, hd].reshape(-1, LANES)) for hd in range(lo, lo + 4)],
                    axis=1)

                def block(row, col):
                    r0 = row * (wo_v.shape[1] // 2) + lo * (LANES // 2)
                    return _as_bf16(
                        wo_v[2 * u + col + _opaque_zero(steps, i), r0:r0 + 2 * LANES, :])

                part = _dot(lhs, _rhs_term(i, block).astype(BF16))
                acc = part if acc is None else part + acc
                next(filler, None)
            prods.append(acc)
        c = [t.reshape(n_seg // 2, 1, n_mem, LANES) for t in _combine(prods)]
        return [jnp.concatenate([c[j], c[j + 2]], axis=1).reshape(n_seg, n_mem, LANES)
                for j in range(2)]

    def mix_first(u, blocks):
        for n, a in enumerate(blocks, 2 * u):
            a_v[:, first, lanes(n)] = a
            out_v[:, first, lanes(n)] = _mix(
                g_v[:, first, :], a, x_v[:, first, lanes(n)].astype(F32))

    for w in (wg_v, wu_v, wd_v):
        wait_whole(w, sem_a)
    n_early = n_seg - STEP_UNROLL
    out_copy(pl.ds(0, n_early), rest, every_col, sem_b).wait()

    ffn = routed_ffn()
    for u in range(nk // 2):
        blocks = out_first(u, ffn)
        if u == nk // 2 - 1:
            for _ in ffn:
                pass
        mix_first(u, blocks)
    first_copies[1].start()
    for_routed_segments(lambda copy: copy.wait())
    for copy in first_copies + [last_copy]:
        copy.wait()


@functools.partial(jax.jit, static_argnames=("A_seg_len",))
def pallas_gated_mix__memory_aug_recurrent_mem_tr__moe_arch_mod__prompt_kernel(
    A_x, A_mem0, A_Wq, A_Wk, A_Wv, A_Wo, A_seg_len, B_x, B_w_r, B_w_gate, B_w_up,
    B_w_down, gate_w,
):
    del B_x
    batch, n_tok, dm = A_x.shape
    n_mem = A_mem0.shape[1]
    n_head, dh = A_Wq.shape[1:]
    d_ff = B_w_gate.shape[1]
    seg = int(A_seg_len)
    n_seg = n_tok // seg
    n_pair, nk, nf = n_head // 2, dm // LANES, d_ff // LANES
    assert (batch, n_mem, seg, dh) == (1, 8, 32, LANES)
    assert dm % (4 * LANES) == 0 and d_ff % LANES == 0 and n_pair % 4 == 0
    assert n_tok % (8 * seg) == 0 and n_seg <= LANES
    assert nk % (n_pair // 2) == 0
    assert ROUTE_SLOTS + 3 * nf > (nk // 2 - 1) * 7 * (n_pair // 4)

    hbm = pl.BlockSpec(memory_space=pl.ANY)
    out = pl.pallas_call(
        _kernel,
        out_shape=jax.ShapeDtypeStruct((n_seg, seg, dm), A_x.dtype),
        in_specs=[hbm] * 11,
        out_specs=hbm,
        scratch_shapes=[
            pltpu.VMEM((n_seg, seg, dm), BF16),
            pltpu.VMEM((7 - N_DEEP, nk // 2, n_seg * n_mem // 4, LANES), U32),
            pltpu.VMEM((7 * N_DEEP, nk // 4, n_seg * n_mem // 8, LANES), U32),
            pltpu.VMEM((3 * n_pair + RAW, dm, LANES), U32),
            pltpu.VMEM((nk, n_head * dh // 2, LANES), U32),
            pltpu.VMEM((3 * n_pair // 2, n_seg, 4, n_mem, LANES), F32),
            pltpu.VMEM((n_seg // 4, 7, n_pair, 8, LANES), U32),
            pltpu.VMEM((n_seg, seg, dm), F32),
            pltpu.VMEM((n_seg, seg, LANES), F32),
            pltpu.VMEM((n_mem, dm), F32),
            pltpu.VMEM((2 * (n_mem + seg), LANES), F32),
            pltpu.VMEM((seg, LANES), I32),
            pltpu.VMEM((n_mem, dm), BF16),
            pltpu.VMEM((nk, LANES), BF16),
            pltpu.VMEM((nk, LANES), BF16),
            pltpu.VMEM((nf, dm // 2, LANES), U32),
            pltpu.VMEM((nf, dm // 2, LANES), U32),
            pltpu.VMEM((nk, d_ff // 2, LANES), U32),
            pltpu.VMEM((n_seg, seg, dm), BF16),
            pltpu.SMEM((TOP_C,), I32),
            pltpu.SemaphoreType.DMA((7,)),
        ],
        compiler_params=pltpu.CompilerParams(
            vmem_limit_bytes=116 * 1024 * 1024, disable_bounds_checks=True),
        name="gated_mix_rmt_mod",
    )(
        A_x.reshape(n_seg, seg, dm), A_mem0.reshape(n_mem, dm), A_Wq, A_Wk, A_Wv,
        A_Wo.reshape(n_head * dh, dm), B_w_r.reshape(nk, LANES), B_w_gate, B_w_up, B_w_down,
        gate_w.reshape(nk, LANES),
    )
    return out.reshape(batch, n_tok, dm)
```

```python
import functools

import jax
import jax.numpy as jnp
import numpy as np
from jax import lax
from jax.experimental import pallas as pl
from jax.experimental.pallas import tpu as pltpu

BF16, F32, U32, I32 = jnp.bfloat16, jnp.float32, jnp.uint32, jnp.int32
LANES = 128
TOP_C = 8
INT_MIN = -(2 ** 31)
HI16 = np.uint32(0xFFFF0000)

RAW = 2
N_DEEP = 4
STEP_UNROLL = 2
QKV_ORDER = (1, 0, 2)
QK_LAG = ("3233333373333332", "3333336333343343")
PV_LAG = ("dcbbbbbbdbbba9be", "bbbbbb9bbbbabbab")
EARLY_HEADS = 16
ROUTE_SLOTS = 18
EARLY_HALVES = 6


def _dot(a, b):
    return jnp.dot(a, b, preferred_element_type=F32)


def _as_bf16(words):
    return pltpu.bitcast(words, BF16)


def _to_words(v):
    return pltpu.bitcast(v.astype(BF16), U32)


def _split_words(words):
    return pltpu.bitcast(words << 16, F32), pltpu.bitcast(words & HI16, F32)


def _sigmoid(v):
    return 1.0 / (1.0 + jnp.exp(-v))


def _mix(gate, a, b):
    return (gate * a + (1.0 - gate) * b).astype(BF16)


def _lhs_terms(a, b, c, d):
    return [c + d, a, a + b, d, a + d, c - a, b - d]


RHS_TERMS = (((0, 0),), ((0, 1), jnp.subtract, (1, 1)), ((1, 1),), ((1, 0), jnp.subtract, (0, 0)),
             ((0, 0), jnp.add, (1, 1)), ((0, 0), jnp.add, (0, 1)), ((1, 0), jnp.add, (1, 1)))


def _rhs_term(i, block):
    term = RHS_TERMS[i]
    if len(term) == 1:
        return block(*term[0])
    return term[1](block(*term[0]).astype(F32), block(*term[2]).astype(F32))


def _opaque_zero(count, i):
    return count >> (16 + i)


def _combine(m):
    return [m[3] - m[2] + m[4] + m[6], m[1] + m[2], m[0] + m[3], m[1] - m[0] + m[4] + m[5]]


def _score_fill(n_mem, seg):
    shape = (2 * (n_mem + seg), LANES)

    def decode(i):
        tail = i >= 2 * seg
        head = jnp.where(tail, (i - 2 * seg) >> 3, i >> 5)
        r = i & (seg - 1)
        pos = jnp.where(tail, n_mem + (i & 7), jnp.where(r < n_mem, r, r + n_mem))
        return head, pos

    rh, rp = decode(lax.broadcasted_iota(I32, shape, 0))
    ch, cp = decode(lax.broadcasted_iota(I32, shape, 1))
    visible = (rp < n_mem) | (rp >= cp)
    return jnp.where(rh == ch, jnp.where(visible, 0.0, -1e9), -jnp.inf).astype(F32)


def _kernel(x_hbm, mem0_hbm, wq_hbm, wk_hbm, wv_hbm, wo_hbm, wr_hbm, wg_hbm, wu_hbm,
            wd_hbm, gw_hbm, out_hbm,
            x_v, x_terms, x_terms2, wqkv, wo_v, qkv0, o_terms, a_v, g_v, mem, fill_v, key_v,
            mem0_ref, wr_ref, gw_ref, wg_v, wu_v, wd_v, out_v, idx_s,
            sems):
    n_seg, seg, dm = x_v.shape
    n_mem = mem.shape[0]
    n_pair = wqkv.shape[0] // 3
    n_head = 2 * n_pair
    nk = dm // LANES
    nf = wg_v.shape[0]
    scale = LANES ** -0.5
    w_hbm = (wq_hbm, wk_hbm, wv_hbm)
    first, rest = pl.ds(0, n_mem), pl.ds(n_mem, seg - n_mem)

    def lanes(n):
        return slice(n * LANES, (n + 1) * LANES)

    sem_a, sem_b = sems.at[0], sems.at[1]

    def slot_of(m, quad, j):
        return 6 * quad + 2 * m + j

    def w_copy(m, quad, j, sem):
        return pltpu.make_async_copy(
            w_hbm[m].bitcast(U32).at[:, 2 * quad + j, :], wqkv.at[slot_of(m, quad, j) + RAW], sem)

    def col_copy(src, dst, n, sem):
        start = n * LANES if isinstance(n, int) else pl.multiple_of(n * LANES, LANES)
        cols = pl.ds(start, LANES)
        return pltpu.make_async_copy(src.bitcast(U32).at[:, cols], dst.at[n], sem)

    def wait_whole(dst, sem):
        pltpu.make_async_copy(dst, dst, sem).wait()

    x_first = pltpu.make_async_copy(x_hbm.at[:, first, :], x_v.at[:, first, :], sem_a)
    x_rest = pltpu.make_async_copy(x_hbm.at[:, rest, :], x_v.at[:, rest, :], sem_b)

    units = [(m, j) for m in range(3) for j in range(2)]
    small = [pltpu.make_async_copy(src, dst, sem_b)
             for src, dst in ((mem0_hbm, mem0_ref), (wr_hbm, wr_ref), (gw_hbm, gw_ref))]

    def group_sem(it):
        return sems.at[2 + (it & 1)]

    x_first.start()
    for m, j in units:
        w_copy(m, 0, j, sems.at[4 + m]).start()
    for m, j in units:
        w_copy(m, 1, j, group_sem(1)).start()

    fill_v[...] = _score_fill(n_mem, seg)
    key_v[...] = jnp.full(key_v.shape, INT_MIN, I32)

    quarter = n_seg * n_mem // 4
    x_first.wait()
    for n in range(nk // 4):
        x0 = [x_v[:, 0:n_mem, lanes(n + k * nk // 4)].astype(F32).reshape(2, 2, quarter, LANES)
              for k in range(4)]
        terms = [_lhs_terms(x0[k][0], x0[k + 2][0], x0[k][1], x0[k + 2][1]) for k in range(2)]
        for j in range(7):
            left, right = terms[0][j], terms[1][j]
            if j < N_DEEP:
                for i, t in enumerate(_lhs_terms(left[0], right[0], left[1], right[1])):
                    x_terms2[7 * j + i, n] = _to_words(t)
            else:
                for k, t in enumerate((left, right)):
                    x_terms[j - N_DEEP, n + k * nk // 4] = _to_words(t.reshape(-1, LANES))

    def regroup(w, piece, n_piece):
        groups = dm // 16
        for r in range(groups * piece // n_piece * 16, groups * (piece + 1) // n_piece * 16, 16):
            even = wqkv[w + RAW, pl.ds(r, 8, stride=2), :]
            odd = wqkv[w + RAW, pl.ds(r + 1, 8, stride=2), :]
            wqkv[w, r:r + 8, :] = (even & np.uint32(0xFFFF)) | (odd << 16)
            wqkv[w, r + 8:r + 16, :] = (even >> 16) | (odd & HI16)

    def project_first(w):
        def rhs_term(j, head, r0, rn, tag):
            def block(row, pair):
                rows = slice(row * (dm // 2) + r0, row * (dm // 2) + r0 + rn)
                words = wqkv[w + RAW + pair + _opaque_zero(w, tag), rows, :]
                return _split_words(words)[head]
            return _rhs_term(j, block)

        def small_product(j, i):
            lhs = jnp.concatenate(
                [_as_bf16(x_terms2[7 * j + i, n]) for n in range(nk // 4)], axis=1)
            rhs = _rhs_term(i, lambda row, head: rhs_term(j, head, row * (dm // 4), dm // 4, i))
            return _dot(lhs, rhs.astype(BF16))

        def large_product(j, head):
            lhs = jnp.concatenate(
                [_as_bf16(x_terms[j - N_DEEP, n]) for n in range(nk // 2)], axis=1)
            return _dot(lhs, rhs_term(j, head, 0, dm // 2, 2 * j + head).astype(BF16))

        def cost(at):
            return len(RHS_TERMS[at[0]]) * len(RHS_TERMS[at[1]])

        small = [(j, i) for j in range(N_DEEP) for i in range(7)]
        cheap = [at for at in small if cost(at) < 9]
        dear = [at for at in small if cost(at) == 9]
        large = [(j, head) for j in range(N_DEEP, 7) for head in range(2)]
        order, dear = ([t[k:k + 2] for k in range(0, len(t), 2)] for t in (cheap, dear))
        for k, at in enumerate(large):
            order += [[at]] + dear[k:k + 1]
        order += dear[len(large):]
        prods, n_piece = {}, len(order) // 2
        for k, group in enumerate(order):
            for j, i in group:
                prods[j, i] = small_product(j, i) if j < N_DEEP else large_product(j, i)
            if k < 2 * n_piece:
                regroup(w + k // n_piece, k % n_piece, n_piece)
        blocks = [_combine([prods[j, i] for i in range(7)]) for j in range(N_DEEP)]
        blocks += [[prods[j, head][q * quarter:(q + 1) * quarter]
                    for q in range(2) for head in range(2)] for j in range(N_DEEP, 7)]
        for q in range(2):
            for head in range(2):
                for i, t in enumerate(_combine([b[2 * q + head] for b in blocks])):
                    segs = pl.ds((2 * (i // 2) + q) * (n_seg // 4), n_seg // 4)
                    qkv0[w >> 1, segs, 2 * (i % 2) + head] = t.reshape(-1, n_mem, LANES)

    n_pro = n_pair // 2
    wo_per_it = nk // n_pro

    def ramp(m, carry):
        wait_whole(wqkv.at[pl.ds(2 * m + RAW, 2)], sems.at[4 + m])
        project_first(2 * m)
        return carry

    lax.fori_loop(0, 3, ramp, 0)
    for copy in small:
        copy.start()
    for n in range(wo_per_it):
        col_copy(wo_hbm, wo_v, n, sem_b).start()

    def prologue(it, carry):
        @pl.when(it + 1 < n_pro)
        def _():
            for m, j in units:
                w_copy(m, it + 1, j, group_sem(it + 1)).start()

        for n in range(wo_per_it):
            col_copy(wo_hbm, wo_v, it * wo_per_it + n, sem_b).start()

        @pl.when(it + 1 == n_pro)
        def _():
            x_rest.start()

        wait_whole(wqkv.at[pl.ds(slot_of(0, it, 0) + RAW, len(units))], group_sem(it))
        for m in range(3):
            project_first(slot_of(m, it, 0))
        return carry

    lax.fori_loop(1, n_pro, prologue, 0)

    x_rest.wait()
    wait_whole(wo_v, sem_b)
    for copy in small:
        copy.wait()
    mem[...] = mem0_ref[...].astype(F32)

    def row_dot(rows, w):
        acc = rows[:, lanes(0)] * w[0:1, :]
        for n in range(1, nk):
            acc = acc + rows[:, lanes(n)] * w[n:n + 1, :]
        return jnp.sum(acc, axis=-1, keepdims=True)

    def head_weights(m, hd, lo, hi):
        w = wqkv[slot_of(m, hd // 4, hd // 2 % 2), lo * LANES:hi * LANES, :]
        w = w.reshape(-1, 2, 8, LANES)
        return _as_bf16(w[:, hd % 2].reshape(-1, LANES))

    def segment(s, mem_cols, mem_is_late):
        xs = x_v[s]
        xf = xs.astype(F32)
        h_cols = [
            jnp.concatenate(
                [jnp.concatenate([mem_cols[n], xf[n_mem:2 * n_mem, lanes(n)]], axis=0).astype(BF16),
                 xs[2 * n_mem:, lanes(n)]], axis=0)
            for n in range(nk)]
        pad = jnp.zeros((LANES - 2 * (seg + n_mem), LANES), F32)

        def partial_proj(m, hd, lo, hi):
            return _dot(jnp.concatenate(h_cols[lo:hi], axis=1), head_weights(m, hd, lo, hi))

        slots = [(m, 2 * p + j) for p in range(n_pair) for m in QKV_ORDER for j in range(2)]
        early = {}
        if mem_is_late:
            for m, hd in slots[:EARLY_HALVES]:
                early[m, hd] = partial_proj(m, hd, 0, nk // 2)

        def project(m, hd):
            if (m, hd) in early:
                return partial_proj(m, hd, nk // 2, nk) + early[m, hd]
            return partial_proj(m, hd, 0, nk)

        def both_heads(m, p):
            rows = [res[m, 2 * p], res[m, 2 * p + 1]]
            rows += [qkv0[3 * (p // 2) + m, s, 2 * (p % 2) + j] for j in range(2)]
            return jnp.concatenate(rows + [pad] * (m > 0), axis=0).astype(BF16)

        def probabilities(q, k):
            sc = lax.dot_general(q, k, (((1,), (1,)), ((), ())), preferred_element_type=F32)
            fill = fill_v[...]
            sc = jnp.where(fill == 0.0, sc * scale, fill)
            e = jnp.exp(sc - jnp.max(sc, axis=-1, keepdims=True))
            den = jnp.sum(e, axis=-1, keepdims=True)
            inv = pl.reciprocal(den, approx=True)
            inv = inv * (2.0 - den * inv)
            return (e * inv).astype(BF16)

        def out_proj(lo, hi, n):
            lhs = jnp.concatenate([heads[i] for i in range(lo, hi)], axis=1)
            return _dot(lhs, _as_bf16(wo_v[n, lo * (LANES // 2):hi * (LANES // 2), :]))

        slots += [(3 + j, n) for n in range(nk) for j in range(2)]
        res, prob, heads, o_first = {}, {}, {}, {}
        for i, (m, j) in enumerate(slots):
            if m < 3:
                res[m, j] = project(m, j)
            elif m == 3:
                res[3, j] = out_proj(0, EARLY_HEADS // 2, j)
            else:
                res[3, j] = out_proj(EARLY_HEADS // 2, EARLY_HEADS, j) + res[3, j]
            for p in range(n_pair):
                ready = [slots.index((t, 2 * p + 1)) for t in range(3)]
                qk_at = max(ready[:2]) + int(QK_LAG[mem_is_late][p % 16], 36)
                pv_at = qk_at + int(PV_LAG[mem_is_late][p % 16], 36)
                if i == qk_at:
                    prob[p] = probabilities(both_heads(0, p), both_heads(1, p))
                if i == min(max(pv_at, ready[2] + 2), len(slots) - 1):
                    o = _dot(prob[p], both_heads(2, p))
                    ob = o[0:2 * seg].astype(BF16)
                    heads[2 * p], heads[2 * p + 1] = ob[0:seg], ob[seg:]
                    o_first[2 * p] = o[2 * seg:2 * seg + n_mem]
                    o_first[2 * p + 1] = o[2 * seg + n_mem:]
        gate = jnp.broadcast_to(_sigmoid(row_dot(xf, gw_ref[...].astype(F32))), (seg, LANES))
        g_v[s] = gate
        new_mem = []
        for n in range(nk):
            r = out_proj(EARLY_HEADS, n_head, n) + res[3, n]
            new_mem.append(r[0:n_mem])
            a_v[s, rest, lanes(n)] = r[n_mem:]
            out_v[s, rest, lanes(n)] = _mix(gate[n_mem:], r[n_mem:], xf[n_mem:, lanes(n)])

        score = row_dot(xf, wr_ref[...].astype(F32)).astype(BF16).astype(F32)
        score = jnp.broadcast_to(score, (seg, LANES))
        bits = pltpu.bitcast(jnp.where(score == 0.0, 0.0, score), I32)
        order = jnp.where(bits < 0, bits ^ np.int32(0x7FFFFFFF), bits)
        order = jnp.where(score != score, INT_MIN, order)
        token = s * seg + lax.broadcasted_iota(I32, (seg, LANES), 0)
        key = (order & np.int32(-65536)) | (65535 - token)
        lane = lax.broadcasted_iota(I32, (seg, LANES), 1)
        key_v[...] = jnp.where(lane == s, key, key_v[...])
        return new_mem, o_first

    n_step = n_seg // STEP_UNROLL

    def out_copy(segs, rows, cols, sem):
        return pltpu.make_async_copy(
            out_v.at[segs, rows, cols], out_hbm.at[segs, rows, cols], sem)

    every_seg, every_col = pl.ds(0, n_seg), pl.ds(0, dm)
    def step(it, carry):
        @pl.when(it > 0)
        def _():
            done = pl.ds((it - 1) * STEP_UNROLL, STEP_UNROLL)
            out_copy(done, rest, every_col, sem_b).start()

        for dst, src in ((wg_v, wg_hbm), (wu_v, wu_hbm), (wd_v, wd_hbm)):
            per_step = pl.cdiv(dst.shape[0], n_step)
            for i in range(per_step):
                @pl.when(it * per_step + i < dst.shape[0])
                def _():
                    col_copy(src, dst, it * per_step + i, sem_a).start()

        mem_cols = [mem[:, lanes(n)] for n in range(nk)]
        for u0 in range(0, STEP_UNROLL, 2):
            o = []
            for u in (u0, u0 + 1):
                mem_cols, o_first = segment(it * STEP_UNROLL + u, mem_cols, u > 0)
                o.append(o_first)
            s0 = it * STEP_UNROLL + u0
            rows = pl.ds(pl.multiple_of((s0 & 2) * 2, 4), 4)
            for hd in range(n_pair):
                a, b, c, d = (o[i][j] for i in range(2) for j in (hd, hd + n_pair))
                for i, t in enumerate(_lhs_terms(a, b, c, d)):
                    o_terms[s0 >> 2, i, hd, rows, :] = _to_words(jnp.concatenate([t, t], axis=0))[0:4]
        for n in range(nk):
            mem[:, lanes(n)] = mem_cols[n]
        return carry + 1

    steps = lax.fori_loop(0, n_step, step, 0)

    last_copy = out_copy(pl.ds(n_seg - STEP_UNROLL, STEP_UNROLL), rest, every_col, sem_a)
    first_copies = [out_copy(every_seg, first, pl.ds(0, dm - 2 * LANES), sem_a),
                    out_copy(every_seg, first, pl.ds(dm - 2 * LANES, 2 * LANES), sem_a)]

    def for_routed_segments(fn):
        segs = [idx_s[i] // seg for i in range(TOP_C)]
        for i, s in enumerate(segs):
            new = functools.reduce(jnp.logical_and, [s != t for t in segs[:i]], s < n_early)
            pl.when(new)(lambda: fn(out_copy(pl.ds(s, 1), rest, every_col, sem_b)))

    row = lax.broadcasted_iota(I32, (n_mem, dm), 0)

    def routed_ffn():
        keys = key_v[...]
        for i in range(TOP_C):
            best = jnp.max(keys)
            idx_s[i] = 65535 - (best & 65535)
            keys = jnp.where(keys == best, INT_MIN, keys)
        x_sel = jnp.zeros((TOP_C, dm), F32)
        for i in range(TOP_C):
            t = idx_s[i]
            rows = pl.ds(pl.multiple_of(t & (seg - n_mem), n_mem), n_mem)
            picked = jnp.where(row == (t & (n_mem - 1)), x_v[t // seg, rows, :].astype(F32), 0.0)
            x_sel = jnp.where(row == i, jnp.sum(picked, axis=0, keepdims=True), x_sel)
        r_sel = _sigmoid(row_dot(x_sel, wr_ref[...].astype(F32)))
        for _ in range(ROUTE_SLOTS):
            yield

        def ffn_dot(lhs, w, n):
            acc = None
            for k in range(0, lhs.shape[1], 4 * LANES):
                part = lax.dot_general(
                    lhs[:, k:k + 4 * LANES], _as_bf16(w[n, k // 2:k // 2 + 2 * LANES, :]),
                    (((1,), (0,)), ((), ())), preferred_element_type=F32)
                acc = part if acc is None else part + acc
                yield
            return acc

        hidden, y = [], []
        for n in range(nf):
            gt = yield from ffn_dot(x_sel, wg_v, n)
            up = yield from ffn_dot(x_sel, wu_v, n)
            hidden.append((gt * _sigmoid(gt) * up).astype(BF16).astype(F32))
        hidden = jnp.concatenate(hidden, axis=1)
        for n in range(nk):
            y.append((yield from ffn_dot(hidden, wd_v, n)))
        y = jnp.concatenate(y, axis=1) * r_sel
        for i in range(TOP_C):
            yield
            yield
            t = idx_s[i]
            s, r0 = t // seg, pl.multiple_of(t & (seg - n_mem), n_mem)
            rows = pl.ds(r0, n_mem)
            upd = jnp.where(row == (t & (n_mem - 1)), y[i:i + 1, :], 0.0)
            b = (x_v[s, rows, :].astype(F32) + upd).astype(BF16)
            x_v[s, rows, :] = b
            later = pl.ds(pl.multiple_of(jnp.maximum(r0, n_mem), n_mem), n_mem)
            gate, b = g_v[s, rows, :], b.astype(F32)
            for n in range(nk):
                a = a_v[s, rows if n < nk - 2 else later, lanes(n)]
                out_v[s, rows, lanes(n)] = _mix(gate, a, b[:, lanes(n)])
        yield
        first_copies[0].start()
        last_copy.start()
        for_routed_segments(lambda copy: copy.start())

    def out_first(u, filler):
        prods = []
        for i in range(7):
            acc = [None, None]
            for lo in range(0, n_pair, 4):
                def block(row, col):
                    r0 = row * (wo_v.shape[1] // 2) + lo * (LANES // 2)
                    return _as_bf16(
                        wo_v[2 * u + col + _opaque_zero(steps, i), r0:r0 + 2 * LANES, :])

                rhs = _rhs_term(i, block).astype(BF16)
                for j in range(2):
                    groups = slice(j * n_seg // 8, (j + 1) * n_seg // 8)
                    lhs = jnp.concatenate(
                        [_as_bf16(o_terms[groups, i, hd].reshape(-1, LANES))
                         for hd in range(lo, lo + 4)], axis=1)
                    part = _dot(lhs, rhs)
                    acc[j] = part if acc[j] is None else part + acc[j]
                    next(filler, None)
            prods.append(jnp.concatenate(acc, axis=0))
        c = [t.reshape(n_seg // 2, 1, n_mem, LANES) for t in _combine(prods)]
        return [jnp.concatenate([c[j], c[j + 2]], axis=1).reshape(n_seg, n_mem, LANES)
                for j in range(2)]

    def mix_first(u, blocks):
        for n, a in enumerate(blocks, 2 * u):
            a_v[:, first, lanes(n)] = a
            out_v[:, first, lanes(n)] = _mix(
                g_v[:, first, :], a, x_v[:, first, lanes(n)].astype(F32))

    for w in (wg_v, wu_v, wd_v):
        wait_whole(w, sem_a)
    n_early = n_seg - STEP_UNROLL
    out_copy(pl.ds(0, n_early), rest, every_col, sem_b).wait()

    ffn = routed_ffn()
    for u in range(nk // 2):
        blocks = out_first(u, ffn)
        if u == nk // 2 - 1:
            for _ in ffn:
                pass
        mix_first(u, blocks)
    first_copies[1].start()
    for_routed_segments(lambda copy: copy.wait())
    for copy in first_copies + [last_copy]:
        copy.wait()


@functools.partial(jax.jit, static_argnames=("A_seg_len",))
def pallas_gated_mix__memory_aug_recurrent_mem_tr__moe_arch_mod__prompt_kernel(
    A_x, A_mem0, A_Wq, A_Wk, A_Wv, A_Wo, A_seg_len, B_x, B_w_r, B_w_gate, B_w_up,
    B_w_down, gate_w,
):
    del B_x
    batch, n_tok, dm = A_x.shape
    n_mem = A_mem0.shape[1]
    n_head, dh = A_Wq.shape[1:]
    d_ff = B_w_gate.shape[1]
    seg = int(A_seg_len)
    n_seg = n_tok // seg
    n_pair, nk, nf = n_head // 2, dm // LANES, d_ff // LANES
    assert (batch, n_mem, seg, dh) == (1, 8, 32, LANES)
    assert dm % (4 * LANES) == 0 and d_ff % (4 * LANES) == 0 and n_pair % 4 == 0
    assert n_tok % (8 * seg) == 0 and n_seg <= LANES
    assert nk % (n_pair // 2) == 0
    assert ROUTE_SLOTS + 3 * nf * nk // 4 > (nk // 2 - 1) * 7 * (n_pair // 2)

    hbm = pl.BlockSpec(memory_space=pl.ANY)
    out = pl.pallas_call(
        _kernel,
        out_shape=jax.ShapeDtypeStruct((n_seg, seg, dm), A_x.dtype),
        in_specs=[hbm] * 11,
        out_specs=hbm,
        scratch_shapes=[
            pltpu.VMEM((n_seg, seg, dm), BF16),
            pltpu.VMEM((7 - N_DEEP, nk // 2, n_seg * n_mem // 4, LANES), U32),
            pltpu.VMEM((7 * N_DEEP, nk // 4, n_seg * n_mem // 8, LANES), U32),
            pltpu.VMEM((3 * n_pair + RAW, dm, LANES), U32),
            pltpu.VMEM((nk, n_head * dh // 2, LANES), U32),
            pltpu.VMEM((3 * n_pair // 2, n_seg, 4, n_mem, LANES), F32),
            pltpu.VMEM((n_seg // 4, 7, n_pair, 8, LANES), U32),
            pltpu.VMEM((n_seg, seg, dm), F32),
            pltpu.VMEM((n_seg, seg, LANES), F32),
            pltpu.VMEM((n_mem, dm), F32),
            pltpu.VMEM((2 * (n_mem + seg), LANES), F32),
            pltpu.VMEM((seg, LANES), I32),
            pltpu.VMEM((n_mem, dm), BF16),
            pltpu.VMEM((nk, LANES), BF16),
            pltpu.VMEM((nk, LANES), BF16),
            pltpu.VMEM((nf, dm // 2, LANES), U32),
            pltpu.VMEM((nf, dm // 2, LANES), U32),
            pltpu.VMEM((nk, d_ff // 2, LANES), U32),
            pltpu.VMEM((n_seg, seg, dm), BF16),
            pltpu.SMEM((TOP_C,), I32),
            pltpu.SemaphoreType.DMA((7,)),
        ],
        compiler_params=pltpu.CompilerParams(
            vmem_limit_bytes=116 * 1024 * 1024, disable_bounds_checks=True),
        name="gated_mix_rmt_mod",
    )(
        A_x.reshape(n_seg, seg, dm), A_mem0.reshape(n_mem, dm), A_Wq, A_Wk, A_Wv,
        A_Wo.reshape(n_head * dh, dm), B_w_r.reshape(nk, LANES), B_w_gate, B_w_up, B_w_down,
        gate_w.reshape(nk, LANES),
    )
    return out.reshape(batch, n_tok, dm)
```

```python
import functools

import jax
import jax.numpy as jnp
import numpy as np
from jax import lax
from jax.experimental import pallas as pl
from jax.experimental.pallas import tpu as pltpu

BF16, F32, U32, I32 = jnp.bfloat16, jnp.float32, jnp.uint32, jnp.int32
LANES = 128
TOP_C = 8
INT_MIN = -(2 ** 31)
HI16 = np.uint32(0xFFFF0000)

RAW = 2
N_DEEP = 4
STEP_UNROLL = 2
ROUTE_SLOTS = 18
EARLY_HALVES = 6
QK_LAG = ((3, 2, 3, 3, 3, 3, 3, 3, 7, 3, 3, 3, 3, 3, 3, 2),
          (3, 3, 3, 3, 3, 3, 6, 3, 3, 3, 3, 4, 3, 3, 4, 3))
PV_LAG = ((13, 12, 11, 11, 11, 11, 11, 11, 13, 11, 11, 11, 10, 9, 11, 14),
          (11, 11, 11, 11, 11, 11, 9, 11, 11, 11, 11, 10, 11, 11, 10, 11))


def _dot(a, b):
    return jnp.dot(a, b, preferred_element_type=F32)


def _as_bf16(words):
    return pltpu.bitcast(words, BF16)


def _to_words(v):
    return pltpu.bitcast(v.astype(BF16), U32)


def _split_words(words):
    return pltpu.bitcast(words << 16, F32), pltpu.bitcast(words & HI16, F32)


def _sigmoid(v):
    return 1.0 / (1.0 + jnp.exp(-v))


def _mix(gate, a, b):
    return (gate * a + (1.0 - gate) * b).astype(BF16)


def _lhs_terms(a, b, c, d):
    return [c + d, a, a + b, d, a + d, c - a, b - d]


RHS_TERMS = (((0, 0),), ((0, 1), jnp.subtract, (1, 1)), ((1, 1),), ((1, 0), jnp.subtract, (0, 0)),
             ((0, 0), jnp.add, (1, 1)), ((0, 0), jnp.add, (0, 1)), ((1, 0), jnp.add, (1, 1)))


def _rhs_term(i, block):
    term = RHS_TERMS[i]
    if len(term) == 1:
        return block(*term[0])
    return term[1](block(*term[0]).astype(F32), block(*term[2]).astype(F32))


def _opaque_zero(count, i):
    return count >> (16 + i)


def _combine(m):
    return [m[3] - m[2] + m[4] + m[6], m[1] + m[2], m[0] + m[3], m[1] - m[0] + m[4] + m[5]]


def _score_fill(n_mem, seg):
    shape = (2 * (n_mem + seg), LANES)

    def decode(i):
        tail = i >= 2 * seg
        head = jnp.where(tail, (i - 2 * seg) >> 3, i >> 5)
        r = i & (seg - 1)
        pos = jnp.where(tail, n_mem + (i & 7), jnp.where(r < n_mem, r, r + n_mem))
        return head, pos

    rh, rp = decode(lax.broadcasted_iota(I32, shape, 0))
    ch, cp = decode(lax.broadcasted_iota(I32, shape, 1))
    visible = (rp < n_mem) | (rp >= cp)
    return jnp.where(rh == ch, jnp.where(visible, 0.0, -1e9), -jnp.inf).astype(F32)


def _kernel(x_hbm, mem0_hbm, wq_hbm, wk_hbm, wv_hbm, wo_hbm, wr_hbm, wg_hbm, wu_hbm,
            wd_hbm, gw_hbm, out_hbm,
            x_v, x_terms, x_terms2, wqkv, wo_v, qkv0, o_terms, a_v, g_v, mem, fill_v, key_v,
            mem0_ref, wr_ref, gw_ref, wg_v, wu_v, wd_v, out_v, idx_s, sems):
    n_seg, seg, dm = x_v.shape
    n_mem = mem.shape[0]
    n_pair = wqkv.shape[0] // 3
    n_head = 2 * n_pair
    nk = dm // LANES
    nf = wg_v.shape[0]
    scale = LANES ** -0.5
    w_hbm = (wq_hbm, wk_hbm, wv_hbm)
    first, rest = pl.ds(0, n_mem), pl.ds(n_mem, seg - n_mem)

    def lanes(n):
        return slice(n * LANES, (n + 1) * LANES)

    sem_a, sem_b = sems.at[0], sems.at[1]

    def slot_of(m, quad, j):
        return 6 * quad + 2 * m + j

    def w_copy(m, quad, j, sem):
        return pltpu.make_async_copy(
            w_hbm[m].bitcast(U32).at[:, 2 * quad + j, :], wqkv.at[slot_of(m, quad, j) + RAW], sem)

    def col_copy(src, dst, n, sem):
        start = n * LANES if isinstance(n, int) else pl.multiple_of(n * LANES, LANES)
        cols = pl.ds(start, LANES)
        return pltpu.make_async_copy(src.bitcast(U32).at[:, cols], dst.at[n], sem)

    def wait_whole(dst, sem):
        pltpu.make_async_copy(dst, dst, sem).wait()

    x_first = pltpu.make_async_copy(x_hbm.at[:, first, :], x_v.at[:, first, :], sem_a)
    x_rest = pltpu.make_async_copy(x_hbm.at[:, rest, :], x_v.at[:, rest, :], sem_b)

    units = [(m, j) for m in range(3) for j in range(2)]
    small = [pltpu.make_async_copy(src, dst, sem_b)
             for src, dst in ((mem0_hbm, mem0_ref), (wr_hbm, wr_ref), (gw_hbm, gw_ref))]

    def group_sem(it):
        return sems.at[2 + (it & 1)]

    x_first.start()
    for m, j in units:
        w_copy(m, 0, j, sems.at[4 + m]).start()
    for m, j in units:
        w_copy(m, 1, j, group_sem(1)).start()

    fill_v[...] = _score_fill(n_mem, seg)
    key_v[...] = jnp.full(key_v.shape, INT_MIN, I32)

    quarter = n_seg * n_mem // 4
    x_first.wait()
    for n in range(nk // 4):
        x0 = [x_v[:, 0:n_mem, lanes(n + k * nk // 4)].astype(F32).reshape(2, 2, quarter, LANES)
              for k in range(4)]
        terms = [_lhs_terms(x0[k][0], x0[k + 2][0], x0[k][1], x0[k + 2][1]) for k in range(2)]
        for j in range(7):
            left, right = terms[0][j], terms[1][j]
            if j < N_DEEP:
                for i, t in enumerate(_lhs_terms(left[0], right[0], left[1], right[1])):
                    x_terms2[7 * j + i, n] = _to_words(t)
            else:
                for k, t in enumerate((left, right)):
                    x_terms[j - N_DEEP, n + k * nk // 4] = _to_words(t.reshape(-1, LANES))

    def regroup(w, piece, n_piece):
        groups = dm // 16
        for r in range(groups * piece // n_piece * 16, groups * (piece + 1) // n_piece * 16, 16):
            even = wqkv[w + RAW, pl.ds(r, 8, stride=2), :]
            odd = wqkv[w + RAW, pl.ds(r + 1, 8, stride=2), :]
            wqkv[w, r:r + 8, :] = (even & np.uint32(0xFFFF)) | (odd << 16)
            wqkv[w, r + 8:r + 16, :] = (even >> 16) | (odd & HI16)

    def project_first(w):
        def rhs_term(j, head, r0, rn, tag):
            def block(row, pair):
                rows = slice(row * (dm // 2) + r0, row * (dm // 2) + r0 + rn)
                words = wqkv[w + RAW + pair + _opaque_zero(w, tag), rows, :]
                return _split_words(words)[head]
            return _rhs_term(j, block)

        def small_product(j, i):
            lhs = jnp.concatenate(
                [_as_bf16(x_terms2[7 * j + i, n]) for n in range(nk // 4)], axis=1)
            rhs = _rhs_term(i, lambda row, head: rhs_term(j, head, row * (dm // 4), dm // 4, i))
            return _dot(lhs, rhs.astype(BF16))

        def large_product(j, head):
            lhs = jnp.concatenate(
                [_as_bf16(x_terms[j - N_DEEP, n]) for n in range(nk // 2)], axis=1)
            return _dot(lhs, rhs_term(j, head, 0, dm // 2, 2 * j + head).astype(BF16))

        def cost(at):
            return len(RHS_TERMS[at[0]]) * len(RHS_TERMS[at[1]])

        deep = [(j, i) for j in range(N_DEEP) for i in range(7)]
        cheap = [at for at in deep if cost(at) < 9]
        dear = [at for at in deep if cost(at) == 9]
        large = [(j, head) for j in range(N_DEEP, 7) for head in range(2)]
        order, dear = ([t[k:k + 2] for k in range(0, len(t), 2)] for t in (cheap, dear))
        for k, at in enumerate(large):
            order += [[at]] + dear[k:k + 1]
        order += dear[len(large):]
        prods, n_piece = {}, len(order) // 2
        for k, group in enumerate(order):
            for j, i in group:
                prods[j, i] = small_product(j, i) if j < N_DEEP else large_product(j, i)
            if k < 2 * n_piece:
                regroup(w + k // n_piece, k % n_piece, n_piece)
        blocks = [_combine([prods[j, i] for i in range(7)]) for j in range(N_DEEP)]
        blocks += [[prods[j, head][q * quarter:(q + 1) * quarter]
                    for q in range(2) for head in range(2)] for j in range(N_DEEP, 7)]
        for q in range(2):
            for head in range(2):
                for i, t in enumerate(_combine([b[2 * q + head] for b in blocks])):
                    segs = pl.ds((2 * (i // 2) + q) * (n_seg // 4), n_seg // 4)
                    qkv0[w >> 1, segs, 2 * (i % 2) + head] = t.reshape(-1, n_mem, LANES)

    n_pro = n_pair // 2
    wo_per_it = nk // n_pro

    def ramp(m, carry):
        wait_whole(wqkv.at[pl.ds(2 * m + RAW, 2)], sems.at[4 + m])
        project_first(2 * m)
        return carry

    lax.fori_loop(0, 3, ramp, 0)
    for copy in small:
        copy.start()
    for n in range(wo_per_it):
        col_copy(wo_hbm, wo_v, n, sem_b).start()

    def prologue(it, carry):
        @pl.when(it + 1 < n_pro)
        def _():
            for m, j in units:
                w_copy(m, it + 1, j, group_sem(it + 1)).start()

        for n in range(wo_per_it):
            col_copy(wo_hbm, wo_v, it * wo_per_it + n, sem_b).start()

        @pl.when(it + 1 == n_pro)
        def _():
            x_rest.start()

        wait_whole(wqkv.at[pl.ds(slot_of(0, it, 0) + RAW, len(units))], group_sem(it))
        for m in range(3):
            project_first(slot_of(m, it, 0))
        return carry

    lax.fori_loop(1, n_pro, prologue, 0)

    x_rest.wait()
    wait_whole(wo_v, sem_b)
    for copy in small:
        copy.wait()
    mem[...] = mem0_ref[...].astype(F32)

    def row_dot(rows, w):
        acc = rows[:, lanes(0)] * w[0:1, :]
        for n in range(1, nk):
            acc = acc + rows[:, lanes(n)] * w[n:n + 1, :]
        return jnp.sum(acc, axis=-1, keepdims=True)

    def head_weights(m, hd, lo, hi):
        w = wqkv[slot_of(m, hd // 4, hd // 2 % 2), lo * LANES:hi * LANES, :]
        w = w.reshape(-1, 2, 8, LANES)
        return _as_bf16(w[:, hd % 2].reshape(-1, LANES))

    def segment(s, mem_cols, mem_is_late):
        xs = x_v[s]
        xf = xs.astype(F32)
        h_cols = [
            jnp.concatenate(
                [jnp.concatenate([mem_cols[n], xf[n_mem:2 * n_mem, lanes(n)]], axis=0).astype(BF16),
                 xs[2 * n_mem:, lanes(n)]], axis=0)
            for n in range(nk)]
        pad = jnp.zeros((LANES - 2 * (seg + n_mem), LANES), F32)

        def partial_proj(m, hd, lo, hi):
            return _dot(jnp.concatenate(h_cols[lo:hi], axis=1), head_weights(m, hd, lo, hi))

        slots = [(m, 2 * p + j) for p in range(n_pair) for m in (1, 0, 2) for j in range(2)]
        early = {}
        if mem_is_late:
            for m, hd in slots[:EARLY_HALVES]:
                early[m, hd] = partial_proj(m, hd, 0, nk // 2)

        def project(m, hd):
            if (m, hd) in early:
                return partial_proj(m, hd, nk // 2, nk) + early[m, hd]
            return partial_proj(m, hd, 0, nk)

        def both_heads(m, p):
            rows = [res[m, 2 * p], res[m, 2 * p + 1]]
            rows += [qkv0[3 * (p // 2) + m, s, 2 * (p % 2) + j] for j in range(2)]
            return jnp.concatenate(rows + [pad] * (m > 0), axis=0).astype(BF16)

        def probabilities(q, k):
            sc = lax.dot_general(q, k, (((1,), (1,)), ((), ())), preferred_element_type=F32)
            fill = fill_v[...]
            sc = jnp.where(fill == 0.0, sc * scale, fill)
            e = jnp.exp(sc - jnp.max(sc, axis=-1, keepdims=True))
            den = jnp.sum(e, axis=-1, keepdims=True)
            inv = pl.reciprocal(den, approx=True)
            inv = inv * (2.0 - den * inv)
            return (e * inv).astype(BF16)

        def out_proj(lo, hi, n):
            lhs = jnp.concatenate([heads[i] for i in range(lo, hi)], axis=1)
            return _dot(lhs, _as_bf16(wo_v[n, lo * (LANES // 2):hi * (LANES // 2), :]))

        slots += [(3 + j, n) for n in range(nk) for j in range(2)]
        res, prob, heads, o_first = {}, {}, {}, {}
        for i, (m, j) in enumerate(slots):
            if m < 3:
                res[m, j] = project(m, j)
            elif m == 3:
                res[3, j] = out_proj(0, n_head // 4, j)
            else:
                res[3, j] = out_proj(n_head // 4, n_head // 2, j) + res[3, j]
            for p in range(n_pair):
                qk_at = slots.index((0, 2 * p + 1)) + QK_LAG[mem_is_late][p]
                if i == qk_at:
                    prob[p] = probabilities(both_heads(0, p), both_heads(1, p))
                if i == min(qk_at + PV_LAG[mem_is_late][p], len(slots) - 1):
                    o = _dot(prob[p], both_heads(2, p))
                    ob = o[0:2 * seg].astype(BF16)
                    heads[2 * p], heads[2 * p + 1] = ob[0:seg], ob[seg:]
                    o_first[2 * p] = o[2 * seg:2 * seg + n_mem]
                    o_first[2 * p + 1] = o[2 * seg + n_mem:]
        gate = jnp.broadcast_to(_sigmoid(row_dot(xf, gw_ref[...].astype(F32))), (seg, LANES))
        g_v[s] = gate
        new_mem = []
        for n in range(nk):
            r = out_proj(n_head // 2, n_head, n) + res[3, n]
            new_mem.append(r[0:n_mem])
            a_v[s, rest, lanes(n)] = r[n_mem:]
            out_v[s, rest, lanes(n)] = _mix(gate[n_mem:], r[n_mem:], xf[n_mem:, lanes(n)])

        score = row_dot(xf, wr_ref[...].astype(F32)).astype(BF16).astype(F32)
        score = jnp.broadcast_to(score, (seg, LANES))
        bits = pltpu.bitcast(jnp.where(score == 0.0, 0.0, score), I32)
        order = jnp.where(bits < 0, bits ^ np.int32(0x7FFFFFFF), bits)
        order = jnp.where(score != score, INT_MIN, order)
        token = s * seg + lax.broadcasted_iota(I32, (seg, LANES), 0)
        key = (order & np.int32(-65536)) | (65535 - token)
        lane = lax.broadcasted_iota(I32, (seg, LANES), 1)
        key_v[...] = jnp.where(lane == s, key, key_v[...])
        return new_mem, o_first

    n_step = n_seg // STEP_UNROLL

    def out_copy(segs, rows, cols, sem):
        return pltpu.make_async_copy(
            out_v.at[segs, rows, cols], out_hbm.at[segs, rows, cols], sem)

    every_seg, every_col = pl.ds(0, n_seg), pl.ds(0, dm)

    def step(it, carry):
        @pl.when(jnp.logical_and(it > 0, it + 1 < n_step))
        def _():
            done = pl.ds((it - 1) * STEP_UNROLL, STEP_UNROLL)
            out_copy(done, rest, every_col, sem_b).start()

        for dst, src in ((wg_v, wg_hbm), (wu_v, wu_hbm), (wd_v, wd_hbm)):
            per_step = pl.cdiv(dst.shape[0], n_step)
            for i in range(per_step):
                @pl.when(it * per_step + i < dst.shape[0])
                def _():
                    col_copy(src, dst, it * per_step + i, sem_a).start()

        mem_cols = [mem[:, lanes(n)] for n in range(nk)]
        o = []
        for u in range(STEP_UNROLL):
            mem_cols, o_first = segment(it * STEP_UNROLL + u, mem_cols, u > 0)
            o.append(o_first)
        rows = pl.ds(pl.multiple_of((it & 1) * 4, 4), 4)
        for hd in range(n_pair):
            a, b, c, d = (o[i][j] for i in range(2) for j in (hd, hd + n_pair))
            for i, t in enumerate(_lhs_terms(a, b, c, d)):
                o_terms[it >> 1, i, hd, rows, :] = _to_words(jnp.concatenate([t, t], axis=0))[0:4]
        for n in range(nk):
            mem[:, lanes(n)] = mem_cols[n]
        return carry + 1

    steps = lax.fori_loop(0, n_step, step, 0)

    n_early = n_seg - 2 * STEP_UNROLL
    last_copy = out_copy(pl.ds(n_early, n_seg - n_early), rest, every_col, sem_a)
    first_copies = [out_copy(every_seg, first, pl.ds(0, dm - 2 * LANES), sem_a),
                    out_copy(every_seg, first, pl.ds(dm - 2 * LANES, 2 * LANES), sem_a)]

    def for_routed_segments(fn):
        segs = [idx_s[i] // seg for i in range(TOP_C)]
        for i, s in enumerate(segs):
            new = functools.reduce(jnp.logical_and, [s != t for t in segs[:i]], s < n_early)
            pl.when(new)(lambda: fn(out_copy(pl.ds(s, 1), rest, every_col, sem_b)))

    row = lax.broadcasted_iota(I32, (n_mem, dm), 0)

    def routed_ffn():
        keys = key_v[...]
        for i in range(TOP_C):
            best = jnp.max(keys)
            idx_s[i] = 65535 - (best & 65535)
            keys = jnp.where(keys == best, INT_MIN, keys)
        x_sel = jnp.zeros((TOP_C, dm), F32)
        for i in range(TOP_C):
            t = idx_s[i]
            rows = pl.ds(pl.multiple_of(t & (seg - n_mem), n_mem), n_mem)
            picked = jnp.where(row == (t & (n_mem - 1)), x_v[t // seg, rows, :].astype(F32), 0.0)
            x_sel = jnp.where(row == i, jnp.sum(picked, axis=0, keepdims=True), x_sel)
        r_sel = _sigmoid(row_dot(x_sel, wr_ref[...].astype(F32)))
        for _ in range(ROUTE_SLOTS):
            yield

        def ffn_dot(lhs, w, n):
            acc = None
            for k in range(0, lhs.shape[1], 4 * LANES):
                part = lax.dot_general(
                    lhs[:, k:k + 4 * LANES], _as_bf16(w[n, k // 2:k // 2 + 2 * LANES, :]),
                    (((1,), (0,)), ((), ())), preferred_element_type=F32)
                acc = part if acc is None else part + acc
                yield
            return acc

        hidden, y = [], []
        for n in range(nf):
            gt = yield from ffn_dot(x_sel, wg_v, n)
            up = yield from ffn_dot(x_sel, wu_v, n)
            hidden.append((gt * _sigmoid(gt) * up).astype(BF16).astype(F32))
        hidden = jnp.concatenate(hidden, axis=1)
        for n in range(nk):
            y.append((yield from ffn_dot(hidden, wd_v, n)))
        y = jnp.concatenate(y, axis=1) * r_sel
        for i in range(TOP_C):
            yield
            yield
            t = idx_s[i]
            s, r0 = t // seg, pl.multiple_of(t & (seg - n_mem), n_mem)
            rows = pl.ds(r0, n_mem)
            upd = jnp.where(row == (t & (n_mem - 1)), y[i:i + 1, :], 0.0)
            b = (x_v[s, rows, :].astype(F32) + upd).astype(BF16)
            x_v[s, rows, :] = b
            later = pl.ds(pl.multiple_of(jnp.maximum(r0, n_mem), n_mem), n_mem)
            gate, b = g_v[s, rows, :], b.astype(F32)
            for n in range(nk):
                a = a_v[s, rows if n < nk - 2 else later, lanes(n)]
                out_v[s, rows, lanes(n)] = _mix(gate, a, b[:, lanes(n)])
        yield
        first_copies[0].start()
        last_copy.start()
        for_routed_segments(lambda copy: copy.start())

    def out_first(u, filler):
        prods = []
        for i in range(7):
            acc = [None, None]
            for lo in range(0, n_pair, 4):
                def block(row, col):
                    r0 = row * (wo_v.shape[1] // 2) + lo * (LANES // 2)
                    return _as_bf16(
                        wo_v[2 * u + col + _opaque_zero(steps, i), r0:r0 + 2 * LANES, :])

                rhs = _rhs_term(i, block).astype(BF16)
                for j in range(2):
                    groups = slice(j * n_seg // 8, (j + 1) * n_seg // 8)
                    lhs = jnp.concatenate(
                        [_as_bf16(o_terms[groups, i, hd].reshape(-1, LANES))
                         for hd in range(lo, lo + 4)], axis=1)
                    part = _dot(lhs, rhs)
                    acc[j] = part if acc[j] is None else part + acc[j]
                    next(filler, None)
            prods.append(jnp.concatenate(acc, axis=0))
        c = [t.reshape(n_seg // 2, 1, n_mem, LANES) for t in _combine(prods)]
        return [jnp.concatenate([c[j], c[j + 2]], axis=1).reshape(n_seg, n_mem, LANES)
                for j in range(2)]

    def mix_first(u, blocks):
        for n, a in enumerate(blocks, 2 * u):
            a_v[:, first, lanes(n)] = a
            out_v[:, first, lanes(n)] = _mix(
                g_v[:, first, :], a, x_v[:, first, lanes(n)].astype(F32))

    for w in (wg_v, wu_v, wd_v):
        wait_whole(w, sem_a)
    out_copy(pl.ds(0, n_early), rest, every_col, sem_b).wait()

    ffn = routed_ffn()
    for u in range(nk // 2):
        blocks = out_first(u, ffn)
        if u == nk // 2 - 1:
            for _ in ffn:
                pass
        mix_first(u, blocks)
    first_copies[1].start()
    for_routed_segments(lambda copy: copy.wait())
    for copy in first_copies + [last_copy]:
        copy.wait()


@functools.partial(jax.jit, static_argnames=("A_seg_len",))
def pallas_gated_mix__memory_aug_recurrent_mem_tr__moe_arch_mod__prompt_kernel(
    A_x, A_mem0, A_Wq, A_Wk, A_Wv, A_Wo, A_seg_len, B_x, B_w_r, B_w_gate, B_w_up,
    B_w_down, gate_w,
):
    del B_x
    batch, n_tok, dm = A_x.shape
    n_mem = A_mem0.shape[1]
    n_head, dh = A_Wq.shape[1:]
    d_ff = B_w_gate.shape[1]
    seg = int(A_seg_len)
    n_seg = n_tok // seg
    n_pair, nk, nf = n_head // 2, dm // LANES, d_ff // LANES
    assert (batch, n_mem, seg, dm, n_head, dh) == (1, 8, 32, 1024, 32, LANES)
    assert n_tok % (8 * seg) == 0 and n_seg <= LANES and d_ff % (4 * LANES) == 0
    assert ROUTE_SLOTS + 3 * nf * nk // 4 > (nk // 2 - 1) * 7 * (n_pair // 2)

    hbm = pl.BlockSpec(memory_space=pl.ANY)
    out = pl.pallas_call(
        _kernel,
        out_shape=jax.ShapeDtypeStruct((n_seg, seg, dm), A_x.dtype),
        in_specs=[hbm] * 11,
        out_specs=hbm,
        scratch_shapes=[
            pltpu.VMEM((n_seg, seg, dm), BF16),
            pltpu.VMEM((7 - N_DEEP, nk // 2, n_seg * n_mem // 4, LANES), U32),
            pltpu.VMEM((7 * N_DEEP, nk // 4, n_seg * n_mem // 8, LANES), U32),
            pltpu.VMEM((3 * n_pair + RAW, dm, LANES), U32),
            pltpu.VMEM((nk, n_head * dh // 2, LANES), U32),
            pltpu.VMEM((3 * n_pair // 2, n_seg, 4, n_mem, LANES), F32),
            pltpu.VMEM((n_seg // 4, 7, n_pair, 8, LANES), U32),
            pltpu.VMEM((n_seg, seg, dm), F32),
            pltpu.VMEM((n_seg, seg, LANES), F32),
            pltpu.VMEM((n_mem, dm), F32),
            pltpu.VMEM((2 * (n_mem + seg), LANES), F32),
            pltpu.VMEM((seg, LANES), I32),
            pltpu.VMEM((n_mem, dm), BF16),
            pltpu.VMEM((nk, LANES), BF16),
            pltpu.VMEM((nk, LANES), BF16),
            pltpu.VMEM((nf, dm // 2, LANES), U32),
            pltpu.VMEM((nf, dm // 2, LANES), U32),
            pltpu.VMEM((nk, d_ff // 2, LANES), U32),
            pltpu.VMEM((n_seg, seg, dm), BF16),
            pltpu.SMEM((TOP_C,), I32),
            pltpu.SemaphoreType.DMA((7,)),
        ],
        compiler_params=pltpu.CompilerParams(
            vmem_limit_bytes=116 * 1024 * 1024, disable_bounds_checks=True),
        name="gated_mix_rmt_mod",
    )(
        A_x.reshape(n_seg, seg, dm), A_mem0.reshape(n_mem, dm), A_Wq, A_Wk, A_Wv,
        A_Wo.reshape(n_head * dh, dm), B_w_r.reshape(nk, LANES), B_w_gate, B_w_up, B_w_down,
        gate_w.reshape(nk, LANES),
    )
    return out.reshape(batch, n_tok, dm)
```
